```python
import jax
import jax.numpy as jnp

def _softmax(x, axis=-1):
    return jax.nn.softmax(x, axis=axis)

def _gelu(x):
    return jax.nn.gelu(x, approximate=True)

def _silu(x):
    return jax.nn.silu(x)

def _sigmoid(x):
    return jax.nn.sigmoid(x)

def _layernorm(x, axis=-1, eps=1e-05):
    m = jnp.mean(x, axis=axis, keepdims=True)
    v = jnp.var(x, axis=axis, keepdims=True)
    return (x - m) / jnp.sqrt(v + eps)

def _scatter_add(tgt, idx, src, axis=0):
    return tgt.at[idx].add(src)

def _segment_sum(src, seg, n):
    return jax.ops.segment_sum(src, seg, n)

class _Rng:

    def __init__(self, key):
        self._k = key

    def _next(self):
        self._k, sub = jax.random.split(self._k)
        return sub

    def normal(self, shape):
        return jax.random.normal(self._next(), shape, dtype=jnp.bfloat16)

    def randint(self, lo, hi, shape):
        return jax.random.randint(self._next(), shape, lo, hi, dtype=jnp.int32)

    def uniform(self, shape, lo=0.0, hi=1.0):
        return jax.random.uniform(self._next(), shape, jnp.bfloat16, lo, hi)

    def permutation(self, n):
        return jax.random.permutation(self._next(), n)
kernel_name = 'concat_heads__memory_aug_recurrent_mem_tr__sliding_local_dilated__prompt'

def setup_inputs():
    _rng = _Rng(jax.random.key(int.from_bytes(__import__("os").urandom(4), "little")))
    _w = lambda a: (lambda t: t.astype(jnp.bfloat16) if jnp.issubdtype(t.dtype, jnp.floating) else t)(jnp.asarray(a))

    def _A_setup():
        B, S, Dm = (1, 2048, 1024)
        H, Dh = (32, 128)
        M, seg = (8, 32)
        seg = min(seg, S)
        S = S // seg * seg
        return {'x': _w((lambda *s: _rng.normal(s) * 0.05)(B, S, Dm)), 'mem0': _w((lambda *s: _rng.normal(s) * 0.05)(B, M, Dm)), 'Wq': _w((lambda *s: _rng.normal(s) * 0.05)(Dm, H, Dh) * Dm ** (-0.5)), 'Wk': _w((lambda *s: _rng.normal(s) * 0.05)(Dm, H, Dh) * Dm ** (-0.5)), 'Wv': _w((lambda *s: _rng.normal(s) * 0.05)(Dm, H, Dh) * Dm ** (-0.5)), 'Wo': _w((lambda *s: _rng.normal(s) * 0.05)(H, Dh, Dm) * (H * Dh) ** (-0.5)), 'seg_len': seg}
    _A_in = _A_setup()

    def _B_setup():
        B, S, D = (1, 2048, 1024)
        return {'x': _w((lambda *s: _rng.normal(s) * 0.05)(B, S, D)), 'wqkv': _w((lambda *s: _rng.normal(s) * 0.05)(D, 3 * D)), 'wo': _w((lambda *s: _rng.normal(s) * 0.05)(D, D))}
    _B_in = _B_setup()
    return {'A_x': _A_in['x'], 'A_mem0': _A_in['mem0'], 'A_Wq': _A_in['Wq'], 'A_Wk': _A_in['Wk'], 'A_Wv': _A_in['Wv'], 'A_Wo': _A_in['Wo'], 'A_seg_len': _A_in['seg_len'], 'B_x': _B_in['x'], 'B_wqkv': _B_in['wqkv'], 'B_wo': _B_in['wo']}

def reference(A_x, A_mem0, A_Wq, A_Wk, A_Wv, A_Wo, A_seg_len, B_x, B_wqkv, B_wo):

    def _A_ref(x, mem0, Wq, Wk, Wv, Wo, seg_len):
        B, S, Dm = x.shape
        H, Dh = (Wq.shape[1], Wq.shape[2])
        M = mem0.shape[1]
        scale = Dh ** (-0.5)
        n_seg = S // seg_len
        L = M + seg_len
        idx = jnp.arange(L)
        mask = (idx[:, None] < M) | (idx[:, None] >= idx[None, :])
        mem = mem0
        outs = []
        for s in range(n_seg):
            xs = x[:, s * seg_len:(s + 1) * seg_len, :].copy()
            h = jnp.concatenate([mem, xs], axis=1)
            q = jnp.einsum('btd,dhe->bhte', h, Wq)
            k = jnp.einsum('btd,dhe->bhte', h, Wk)
            v = jnp.einsum('btd,dhe->bhte', h, Wv)
            scores = jnp.einsum('bhqe,bhke->bhqk', q, k) * scale
            scores = jnp.where(mask[None, None], scores, -1000000000.0)
            p = _softmax(scores, axis=-1)
            o = jnp.einsum('bhqk,bhke->bhqe', p, v)
            o = jnp.einsum('bhte,hed->btd', o, Wo)
            mem = o[:, :M, :].copy()
            outs.append(o[:, M:, :])
        return jnp.concatenate(outs, axis=1)

    def _B_ref(x, wqkv, wo):
        B, S, D = x.shape
        H = 32
        Dh = D // H
        W, dil = (8, 2)
        qkv = (lambda x, *d: x.transpose(*d))((x @ wqkv).reshape(B, S, 3, H, Dh), 2, 0, 3, 1, 4)
        q, k, v = (qkv[0], qkv[1], qkv[2])
        scale = Dh ** (-0.5)
        pos = jnp.arange(S)
        off = jnp.arange(W) * dil
        idx = pos[:, None] - off[None, :]
        mask = idx >= 0
        idx_c = jnp.where(mask, idx, 0).reshape(-1)
        kg = k[:, :, idx_c, :].reshape(B, H, S, W, Dh)
        vg = v[:, :, idx_c, :].reshape(B, H, S, W, Dh)
        logits = jnp.einsum('bhsd,bhswd->bhsw', q, kg) * scale
        logits = jnp.where(mask[None, None, :, :], logits, -1000000000.0)
        attn = _softmax(logits, axis=-1)
        o = jnp.einsum('bhsw,bhswd->bhsd', attn, vg)
        return (lambda x, *d: x.transpose(*d))(o, 0, 2, 1, 3).reshape(B, S, D) @ wo
    a = _A_ref(A_x, A_mem0, A_Wq, A_Wk, A_Wv, A_Wo, A_seg_len)
    b = _B_ref(B_x, B_wqkv, B_wo)
    return jnp.concatenate([a, b], axis=-1)
```

```python
import functools

import jax
import jax.numpy as jnp
from jax import lax
import jax.experimental.pallas as pl
import jax.experimental.pallas.tpu as pltpu

BF = jnp.bfloat16
F32 = jnp.float32
U32 = jnp.uint32

S = 2048
D = 1024
H = 32
E = 128
MEM = 8
SEG = 32
L = MEM + SEG
NSEG = S // SEG
XR = 24
PRE = S - NSEG * XR
NS = 17
NB = 4
PAIR = 2 * L
SLOT = (H // 2 // NB) * PAIR
SPLIT = 24
OLROWS = NSEG * 32 + PRE
WIN = 8
DIL = 2
HIST = 16
NCH = 12
NEG = -1000000000.0


def _rcp(d):
    r = pl.reciprocal(d, approx=True)
    return r * (2.0 - d * r)


def _dot(a, b):
    return jnp.dot(a, b, preferred_element_type=F32)


def _kernel(xa, mem0, wq, wk, wv, wo, xb, wqkv, wob, out,
            xpre, hx, xbb, wst, wa0, wa1, woa, bst, wb, wobst, wobp,
            r0, r1, r2, r3, ola, olb, acc, fill, qb, kb, vb, ob, outa, outb,
            sem_misc, sem_w, sem_b, sem_wob, sem_woa, sem_hx, sem_xb, sem_out):
    rings = (r0, r1, r2, r3)
    was = (wa0, wa1)
    wsrc = (wq, wk, wv)

    def w_copy(t, g, slot):
        return pltpu.make_async_copy(
            wsrc[t].at[:, pl.ds(pl.multiple_of(g * 8, 8), 8), :], wst.at[slot], sem_w.at[slot])

    def w_start(c):
        if isinstance(c, int):
            w_copy(c // 4, c % 4, c % 3).start()
        else:
            for t in range(3):
                @pl.when(c // 4 == t)
                def _():
                    w_copy(t, c % 4, c % 3).start()

    def w_wait(c):
        w_copy(0, 0, c % 3).wait()

    def b_copy(b):
        return pltpu.make_async_copy(
            wqkv.at[pl.ds(pl.multiple_of((b % 4) * 256, 256), 256),
                    pl.ds(pl.multiple_of((b // 4) * D, D), D)],
            bst.at[b % 2], sem_b.at[b % 2])

    def wob_copy(j):
        return pltpu.make_async_copy(
            wob.at[:, pl.ds(pl.multiple_of(j * 128, 128), 128)], wobst.at[j % 2], sem_wob.at[j % 2])

    def woa_copy(j):
        return pltpu.make_async_copy(
            wo.at[:, pl.ds(pl.multiple_of(j * 128, 128), 128)], woa.at[j], sem_woa.at[j])

    def hx_copy(s):
        return pltpu.make_async_copy(
            xa.at[pl.ds(pl.multiple_of(PRE + s * XR, 8), XR), :],
            hx.at[s % 4, pl.ds(MEM, XR), :], sem_hx.at[s % 4])

    def xb_copy(s):
        return pltpu.make_async_copy(
            xb.at[pl.ds(pl.multiple_of(s * SEG, SEG), SEG), :], xbb.at[s % 4], sem_xb.at[s % 4])

    xpre_copy = pltpu.make_async_copy(xa.at[pl.ds(0, PRE), :], xpre, sem_misc.at[0])
    mem_copy = pltpu.make_async_copy(mem0, hx.at[0, pl.ds(0, MEM), :], sem_misc.at[1])

    w_start(0)
    xpre_copy.start()
    w_start(1)
    b_copy(0).start()
    wob_copy(0).start()
    w_start(2)
    mem_copy.start()

    ri = lax.broadcasted_iota(jnp.int32, (PAIR, PAIR), 0)
    ci = lax.broadcasted_iota(jnp.int32, (PAIR, PAIR), 1)
    rb = ri >= L
    cb = ci >= L
    rl = jnp.where(rb, ri - L, ri)
    cl = jnp.where(cb, ci - L, ci)
    allowed = (rl < MEM) | (rl >= cl)
    fill[...] = jnp.where(rb == cb, jnp.where(allowed, 0.0, NEG), -jnp.inf).astype(F32)
    kb[...] = jnp.zeros(kb.shape, F32)
    vb[...] = jnp.zeros(vb.shape, F32)
    ob[...] = jnp.zeros(ob.shape, BF)

    def wa_index(c):
        return (c // 2) * 8

    def relayout(c, par):
        base = wa_index(c)
        slot = c % 3
        for kt in range(D // 128):
            v = wst[slot, kt * 128:(kt + 1) * 128]
            v = jnp.swapaxes(v, 0, 1)
            for hh in range(8):
                was[par][base + hh, kt * 64:(kt + 1) * 64, :] = pltpu.bitcast(v[hh], U32)

    def pre_matmul(c, par, heads):
        base = wa_index(c)
        t = c // 4
        g = c % 4
        for hh in heads:
            r = _dot(xpre[...], pltpu.bitcast(was[par][base + hh], BF)).astype(BF)
            ring = rings[hh // 2]
            off = pl.multiple_of(g * PAIR, 8)
            for sg in range(PRE // SEG):
                ring[t, pl.ds(off + sg * SLOT + (hh % 2) * L + MEM, SEG), :] = r[sg * SEG:(sg + 1) * SEG]

    def b_prep(b):
        x32 = pltpu.bitcast(bst[b % 2], U32)
        y = jnp.swapaxes(x32.T.reshape(H, 32, 128), 0, 1).reshape(D, 128)
        z = y.T
        row = pl.multiple_of((b % 4) * 128, 128)
        for cc in range(8):
            wb[(b // 4) * 8 + cc, pl.ds(row, 128), :] = z[:, cc * 128:(cc + 1) * 128]

    def wob_prep(j):
        v = wobst[j % 2].reshape(H, 32, 128)
        v = jnp.swapaxes(v, 0, 1).reshape(D, 128)
        wobp[j] = pltpu.bitcast(v, U32)

    def half(c, par):
        @pl.when(c + 1 < NCH)
        def _():
            w_wait(c + 1)

        @pl.when(c + 3 < NCH)
        def _():
            w_start(c + 3)

        @pl.when(c + 1 < NCH)
        def _():
            b_copy(c + 1).start()

        @pl.when(c + 1 < 8)
        def _():
            wob_copy(c + 1).start()

        @pl.when(c >= 4)
        def _():
            woa_copy(c - 4).start()

        @pl.when(c >= NCH - 2)
        def _():
            hx_copy(c - (NCH - 2)).start()
            xb_copy(c - (NCH - 2)).start()

        relayout(jnp.where(c + 1 < NCH, c + 1, NCH - 2), 1 - par)
        pre_matmul(c, par, range(0, 4))
        b_copy(c).wait()

        @pl.when(c < 8)
        def _():
            wob_copy(c).wait()

        b_prep(c)
        wob_prep(jnp.minimum(c, 7))
        pre_matmul(c, par, range(4, 8))

    w_wait(0)
    relayout(0, 0)
    xpre_copy.wait()

    def phase1(i, carry):
        half(2 * i, 0)
        half(2 * i + 1, 1)
        return carry

    lax.fori_loop(0, NCH // 2, phase1, 0)
    mem_copy.wait()
    for j in range(8):
        woa_copy(j).wait()

    def wa_ref(t, h):
        g = h // 8
        return pltpu.bitcast(was[g % 2][(2 * t + g // 2) * 8 + h % 8], BF)

    def ol_ref(h):
        return (ola, h) if h < SPLIT else (olb, h - SPLIT)

    def ol_lhs(row, n, h0, h1):
        return jnp.concatenate(
            [ol_ref(h)[0][ol_ref(h)[1], pl.ds(row, n), :] for h in range(h0, h1)], axis=1)

    a_scale = E ** -0.5
    b_scale = (D // H) ** -0.5

    def b_out(s):
        o = ob[...]
        row = pl.multiple_of(s * SEG, SEG)
        for j in range(8):
            outb[pl.ds(row, SEG), j * 128:(j + 1) * 128] = _dot(o, pltpu.bitcast(wobp[j], BF)).astype(BF)

    def outb_copy(s):
        row = pl.multiple_of(s * SEG, SEG)
        return pltpu.make_async_copy(
            outb.at[pl.ds(row, SEG), :], out.at[pl.ds(row, SEG), pl.ds(D, D)], sem_out.at[1])

    def outa_copy(row, n):
        return pltpu.make_async_copy(
            outa.at[pl.ds(row, n), :], out.at[pl.ds(row, n), pl.ds(0, D)], sem_out.at[0])

    def step(s, carry):
        @pl.when(s + 2 < NSEG)
        def _():
            hx_copy(s + 2).start()
            xb_copy(s + 2).start()

        hx_copy(s).wait()
        xb_copy(s).wait()

        b_out(jnp.maximum(s - 1, 0))

        xrows = xbb[s % 4]
        for cc in range(8):
            kb[cc, 0:HIST, :] = kb[cc, SEG:SEG + HIST, :]
            vb[cc, 0:HIST, :] = vb[cc, SEG:SEG + HIST, :]
        for cc in range(8):
            qb[cc] = _dot(xrows, pltpu.bitcast(wb[cc], BF)) * b_scale
            kb[cc, HIST:HIST + SEG, :] = _dot(xrows, pltpu.bitcast(wb[8 + cc], BF))
            vb[cc, HIST:HIST + SEG, :] = _dot(xrows, pltpu.bitcast(wb[16 + cc], BF))

        def b_attn(i):
            q = [qb[cc, 8 * i:8 * i + 8, :] for cc in range(8)]
            pos = s * SEG + 8 * i + lax.broadcasted_iota(jnp.int32, (8, 128), 0)
            logits = []
            for w in range(WIN):
                lo = HIST + 8 * i - DIL * w
                t = q[0] * kb[0, lo:lo + 8, :]
                for cc in range(1, 8):
                    t = t + q[cc] * kb[cc, lo:lo + 8, :]
                t = t + pltpu.roll(t, 64, 1)
                t = t + pltpu.roll(t, 32, 1)
                if w > 0:
                    t = jnp.where(pos >= DIL * w, t, NEG)
                logits.append(t)
            m = functools.reduce(jnp.maximum, logits)
            ex = [jnp.exp(t - m) for t in logits]
            r = _rcp(functools.reduce(lambda a, b: a + b, ex))
            p = [e * r for e in ex]
            for cc in range(8):
                t = p[0] * vb[cc, HIST + 8 * i:HIST + 8 * i + 8, :]
                for w in range(1, WIN):
                    lo = HIST + 8 * i - DIL * w
                    t = t + p[w] * vb[cc, lo:lo + 8, :]
                ob[8 * i:8 * i + 8, cc * 128:(cc + 1) * 128] = t.astype(BF)

        lhs = hx[s % 4]
        slot = pl.multiple_of((s % NS) * SLOT, 16)
        offs = [slot]
        for i in range(3):
            g = PRE // 8 + 3 * s + i
            offs.append(pl.multiple_of(((g // 4) % NS) * SLOT + MEM + 8 * (g % 4), 8))
        oofs = [pl.multiple_of(s * 32, 32)]
        for i in range(4):
            g = 4 * s + i
            oofs.append(pl.multiple_of(
                jnp.where(g < 3 * NSEG, (g // 3) * 32 + MEM + 8 * (g % 3),
                          NSEG * 32 + (g - 3 * NSEG) * 8), 8))

        def proj(h):
            p = h // 2
            ring = rings[p % NB]
            ro = (p // NB) * PAIR + (h % 2) * L
            for t in range(3):
                r = _dot(lhs, wa_ref(t, h)).astype(BF)
                for i in range(4):
                    ring[t, pl.ds(offs[i] + ro, 8), :] = r[8 * i:8 * i + 8]

        probs = {}

        def att1(p):
            ring = rings[p % NB]
            ro = (p // NB) * PAIR
            q = ring[0, pl.ds(slot + ro, PAIR), :]
            k = ring[1, pl.ds(slot + ro, PAIR), :]
            sc = lax.dot_general(q, k, (((1,), (1,)), ((), ())), preferred_element_type=F32) * a_scale
            fl = fill[...]
            sc = jnp.where(fl == 0.0, sc, fl)
            e = jnp.exp(sc - jnp.max(sc, axis=1, keepdims=True))
            probs[p] = (e * _rcp(jnp.sum(e, axis=1, keepdims=True))).astype(BF)

        def att2(p):
            ring = rings[p % NB]
            ro = (p // NB) * PAIR
            o = _dot(probs.pop(p), ring[2, pl.ds(slot + ro, PAIR), :]).astype(BF)
            for hh in range(2):
                ol, hi = ol_ref(2 * p + hh)
                for i in range(5):
                    ol[hi, pl.ds(oofs[i], 8), :] = o[hh * L + 8 * i:hh * L + 8 * i + 8]

        for p in range(H // 2):
            proj(2 * p)
            if p >= 1:
                att1(p - 1)
            proj(2 * p + 1)
            if p >= 2:
                att2(p - 2)
            if p % 3 == 2 and p // 3 < 4:
                b_attn(p // 3)
        pend = [lambda: att1(15), lambda: att2(14), lambda: att2(15)]
        l1 = ol_lhs(oofs[0], 32, 0, SPLIT)
        for j in range(8):
            acc[j] = _dot(l1, woa[j, :SPLIT * 128, :])
            if pend and j % 2 == 0:
                pend.pop(0)()
        l2 = ol_lhs(oofs[0], 32, SPLIT, H)
        orow = pl.multiple_of(s * XR, 8)
        for j in range(8):
            res = (acc[j] + _dot(l2, woa[j, SPLIT * 128:, :])).astype(BF)
            hx[(s + 1) % 4, 0:MEM, j * 128:(j + 1) * 128] = res[0:MEM]
            outa[pl.ds(orow, XR), j * 128:(j + 1) * 128] = res[MEM:]

        outa_copy(orow, XR).start()

        @pl.when(s >= 1)
        def _():
            outb_copy(s - 1).start()

        return carry

    lax.fori_loop(0, NSEG, step, 0)

    b_out(NSEG - 1)
    outb_copy(NSEG - 1).start()

    def post(i, carry):
        lhs = ol_lhs(pl.multiple_of(NSEG * 32 + i * 128, 128), 128, 0, H)
        row = pl.multiple_of(NSEG * XR + i * 128, 128)
        for j in range(8):
            outa[pl.ds(row, 128), j * 128:(j + 1) * 128] = _dot(lhs, woa[j]).astype(BF)
        outa_copy(row, 128).start()
        return carry

    lax.fori_loop(0, PRE // 128, post, 0)

    pltpu.make_async_copy(outb, out.at[:, pl.ds(D, D)], sem_out.at[1]).wait()
    pltpu.make_async_copy(outa, out.at[:, pl.ds(0, D)], sem_out.at[0]).wait()


@jax.jit
def _run(A_x, A_mem0, A_Wq, A_Wk, A_Wv, A_Wo, B_x, B_wqkv, B_wo):
    assert A_x.shape == (1, S, D) and A_mem0.shape == (1, MEM, D)
    assert A_Wq.shape == (D, H, E) and A_Wo.shape == (H, E, D)
    assert B_x.shape == (1, S, D) and B_wqkv.shape == (D, 3 * D) and B_wo.shape == (D, D)
    vm = pltpu.VMEM
    dma = pltpu.SemaphoreType.DMA
    scratch = [
        vm((PRE, D), BF),
        vm((4, 32, D), BF),
        vm((4, SEG, D), BF),
        vm((3, D, 8, E), BF),
        vm((48, D // 2, E), U32),
        vm((48, D // 2, E), U32),
        vm((8, H * E, 128), BF),
        vm((2, 256, D), BF),
        vm((24, D // 2, 128), U32),
        vm((2, D, 128), BF),
        vm((8, D // 2, 128), U32),
    ] + [vm((3, NS * SLOT, E), BF)] * NB + [
        vm((SPLIT, OLROWS, E), BF),
        vm((H - SPLIT, OLROWS, E), BF),
        vm((8, 32, 128), F32),
        vm((PAIR, PAIR), F32),
        vm((8, SEG, 128), F32),
        vm((8, HIST + SEG, 128), F32),
        vm((8, HIST + SEG, 128), F32),
        vm((SEG, D), BF),
        vm((S, D), BF),
        vm((S, D), BF),
        dma((2,)), dma((3,)), dma((2,)), dma((2,)), dma((8,)), dma((4,)), dma((4,)), dma((2,)),
    ]
    out = pl.pallas_call(
        _kernel,
        out_shape=jax.ShapeDtypeStruct((S, 2 * D), BF),
        in_specs=[pl.BlockSpec(memory_space=pl.ANY)] * 9,
        out_specs=pl.BlockSpec(memory_space=pl.ANY),
        scratch_shapes=scratch,
        compiler_params=pltpu.CompilerParams(vmem_limit_bytes=120 * 1024 * 1024),
    )(A_x.reshape(S, D), A_mem0.reshape(MEM, D), A_Wq, A_Wk, A_Wv, A_Wo.reshape(H * E, D),
      B_x.reshape(S, D), B_wqkv, B_wo)
    return out.reshape(1, S, 2 * D)


def pallas_concat_heads__memory_aug_recurrent_mem_tr__sliding_local_dilated__prompt_kernel(
    A_x: jax.Array,
    A_mem0: jax.Array,
    A_Wq: jax.Array,
    A_Wk: jax.Array,
    A_Wv: jax.Array,
    A_Wo: jax.Array,
    A_seg_len,
    B_x: jax.Array,
    B_wqkv: jax.Array,
    B_wo: jax.Array,
):
    if isinstance(A_seg_len, int):
        assert A_seg_len == SEG
    return _run(A_x, A_mem0, A_Wq, A_Wk, A_Wv, A_Wo, B_x, B_wqkv, B_wo)
```

```python
import functools

import jax
import jax.numpy as jnp
from jax import lax
import jax.experimental.pallas as pl
import jax.experimental.pallas.tpu as pltpu

BF = jnp.bfloat16
F32 = jnp.float32
U32 = jnp.uint32

S = 2048
D = 1024
H = 32
E = 128
MEM = 8
SEG = 32
L = MEM + SEG
NSEG = S // SEG
XR = 24
PRE = S - NSEG * XR
NS = 17
PAIR = 2 * L
OLROWS = NSEG * 32 + PRE
WIN = 8
DIL = 2
HIST = 16
NCH = 12
NEG = -1000000000.0
LOG2E = 1.4426950408889634
MB = 128
CFG = dict(wpad=0, ntw=4, twp=80, sst=False, lag=1, skip=(), vticks=60, q0=64, q1=128, mdead=(0, 2, 4, 6), sspan=2, exp2=False, G=1, d1=1, d2=4, o21=True, NB=4, bqk=(1, 4, 7, 10), bpv=(5, 8, 11, 14), qspan=36, vspan=36, tstep=1, early=2, bdead=(2, 5, 8, 11), U=2, nobc=True, battn=(2, 5, 8, 11), SPLIT=24, W0P=4)
U = CFG['U']
NB = 4
NG = L // 8
SPLIT = CFG['SPLIT']
NX = 4 * U
W0P = CFG['W0P']

SEM_N = (3, W0P, NCH, 12, 8, 8, 2, 2)
SEM_BASE = tuple(sum(SEM_N[:i]) for i in range(len(SEM_N)))


def _rcp(d):
    r = pl.reciprocal(d, approx=True)
    return r * (2.0 - d * r)


def _dot(a, b):
    return jnp.dot(a, b, preferred_element_type=F32)


def _lo_hi(a, b):
    lo = (a & U32(0xFFFF)) | (b << 16)
    hi = (a >> 16) | (b & U32(0xFFFF0000))
    return lo, hi


def _kernel(xa, mem0, wq, wk, wv, wo, xb, wqkv, wob, out,
            xar, xbb, memb, wa0, wa1, woa, wb, wobp,
            r0, r1, r2, r3, acc, fill, qb, kb, vb, pb, ob, zero,
            sem, sem_out):
    class _Sems:
        def __init__(self, base):
            self.base = base
            self.at = self

        def __getitem__(self, i):
            return sem.at[self.base + i]

    sem_x, sem_w0, sem_w, sem_b, sem_wob, sem_woa, sem_hx, sem_xb = [_Sems(b) for b in SEM_BASE]
    rings = (r0, r1, r2, r3)
    was = (wa0, wa1)
    wsrc = (wq, wk, wv)

    def xar_copy(q):
        n = NSEG * XR // 2
        return pltpu.make_async_copy(
            xa.at[pl.ds(PRE + q * n, n), :], xar.at[pl.ds(q * n, n), :], sem_hx.at[q])

    def xb_copy(q):
        n = S // 2
        return pltpu.make_async_copy(
            xb.at[pl.ds(q * n, n), :], xbb.at[pl.ds(q * n, n), :], sem_xb.at[q])

    mem_copy = pltpu.make_async_copy(mem0, memb, sem_x.at[0])

    def phase1(xpre, wst, woast, bst, wobst, tw, tb, tob):
        def w_copy(c):
            t = c // 4 if isinstance(c, int) else 0
            g = c % 4 if isinstance(c, int) else 0
            return pltpu.make_async_copy(
                wsrc[t].at[:, pl.ds(g * 8, 8), :], wst.at[c, pl.ds(0, D)], sem_w.at[c])

        def w0_copy(q):
            n = D // W0P
            return pltpu.make_async_copy(
                wq.at[pl.ds(q * n, n), pl.ds(0, 8), :], wst.at[0, pl.ds(q * n, n)], sem_w0.at[q])

        def x_copy(q):
            lo, n = ((0, MB), (MB, PRE - MB))[q]
            return pltpu.make_async_copy(
                xa.at[pl.ds(lo, n), :], xpre.at[pl.ds(lo, n), :], sem_x.at[1 + q])

        def b_copy(b):
            bs = b if isinstance(b, int) else 0
            return pltpu.make_async_copy(
                wqkv.at[pl.ds((bs % 4) * 256, 256), pl.ds((bs // 4) * D, D)],
                bst.at[b, pl.ds(0, 256)], sem_b.at[b])

        def wob_copy(j):
            js = j if isinstance(j, int) else 0
            return pltpu.make_async_copy(
                wob.at[:, pl.ds(js * 128, 128)], wobst.at[j, pl.ds(0, D)], sem_wob.at[j])

        def woa_copy(j):
            js = j if isinstance(j, int) else 0
            return pltpu.make_async_copy(
                wo.at[pl.ds(js * 512, 512), :], woast.at[j, pl.ds(0, 512)], sem_woa.at[j])

        def b_blocks(j):
            i, par = j // 2, j % 2
            return (3 * i, 3 * i + 1) if par == 0 else (3 * i + 2,)

        for q in range(W0P):
            w0_copy(q).start()
        x_copy(0).start()
        x_copy(1).start()
        for c in range(1, 6):
            w_copy(c).start()
        for j in range(8):
            woa_copy(j).start()
            wob_copy(j).start()
            for b in b_blocks(j):
                b_copy(b).start()
            if j + 6 < NCH:
                w_copy(j + 6).start()
        mem_copy.start()
        for q in range(2):
            xb_copy(q).start()
            xar_copy(q).start()

        ri = lax.broadcasted_iota(jnp.int32, (PAIR, PAIR), 0)
        ci = lax.broadcasted_iota(jnp.int32, (PAIR, PAIR), 1)
        rb = (ri >> 3) & 1
        cb = (ci >> 3) & 1
        rl = ((ri >> 4) << 3) | (ri & 7)
        cl = ((ci >> 4) << 3) | (ci & 7)
        allowed = (rl < MEM) | (rl >= cl)
        fill[...] = jnp.where(rb == cb, jnp.where(allowed, 0.0, NEG / E ** -0.5 if CFG['exp2'] else NEG), -jnp.inf).astype(F32)
        kb[...] = jnp.zeros(kb.shape, F32)
        vb[...] = jnp.zeros(vb.shape, F32)
        pb[...] = jnp.zeros(pb.shape, F32)
        zero[...] = jnp.zeros(zero.shape, U32)

        def relayout1(c, blk, gate=None):
            v = wst[c, blk * 16:(blk + 1) * 16]
            v = pltpu.bitcast(v.reshape(128, 128), U32)
            t = tw.at[blk % tw.shape[0]]
            for dp in range(8):
                x = v[8 * dp:8 * dp + 8]
                x = x if gate is None else x | gate()
                if CFG['sst']:
                    t[pl.ds(dp, 8, stride=9), :] = x
                else:
                    t[9 * dp:9 * dp + 8, :] = x

        def relayout2(c, par, blk, gate=None):
            base = (c // 2) * 8
            t = tw.at[blk % tw.shape[0]]
            for j in range(4):
                if CFG['sst']:
                    a, b = t[9 * j:9 * j + 8, :], t[9 * (4 + j):9 * (4 + j) + 8, :]
                else:
                    a, b = t[pl.ds(j, 8, stride=9), :], t[pl.ds(4 + j, 8, stride=9), :]
                if gate is not None and CFG['lag']:
                    g = gate()
                    a, b = a | g, b | g
                lo, hi = _lo_hi(a, b)
                was[par][base + 2 * j, blk * 8:blk * 8 + 8, :] = lo
                was[par][base + 2 * j + 1, blk * 8:blk * 8 + 8, :] = hi

        def relayout(c, par, blocks):
            for blk in blocks:
                relayout1(c, blk)
                relayout2(c, par, blk)

        def pre_matmul(c, par, hh, mb):
            base = (c // 2) * 8
            t = c // 4
            g = c % 4
            r32 = _dot(xpre[mb * MB:(mb + 1) * MB, :], pltpu.bitcast(was[par][base + hh, 0:D // 2], BF))
            r = r32.astype(BF)
            ring = rings[hh // 2]
            off = pl.multiple_of(g * 16, 16) + (hh % 2) * 8
            for k in range(MB // 8):
                gx = mb * MB // 8 + k
                ring[t, (gx // 4) * NG + 1 + gx % 4, pl.ds(off, 8), :] = r[8 * k:8 * k + 8]
            return r32

        def gated(x, gate):
            return jnp.concatenate([x[i:i + 8] | gate() for i in range(0, x.shape[0], 8)], axis=0)

        def b_prep1(b, k, cc, gate):
            x32 = gated(pltpu.bitcast(bst[b, 0:256, cc * 128:(cc + 1) * 128], U32), gate).T
            for hl in range(4):
                h = 4 * cc + hl
                tb[k, 33 * h:33 * h + 32, :] = x32[32 * hl:32 * hl + 32]

        def b_prep2(b, k, cc, gate):
            y = jnp.concatenate(
                [tb[k, pl.ds(4 * cc + dl + 33 * 8 * g, 8, stride=33), :] for dl in range(4) for g in range(4)],
                axis=0)
            z = gated(y, gate).T
            row = pl.multiple_of((b % 4) * 128, 128)
            wb[(b // 4) * 8 + cc, pl.ds(row, 128), :] = z

        def wob_prep(j, g, gate):
            v = gated(pltpu.bitcast(wobst[j, g * 512:(g + 1) * 512, :], U32), gate)
            for hp in range(8):
                tob[g, 33 * hp:33 * hp + 32, :] = v[32 * hp:32 * hp + 32]
            for dp in range(16):
                lo, hi = _lo_hi(tob[g, pl.ds(dp, 8, stride=33), :], tob[g, pl.ds(16 + dp, 8, stride=33), :])
                wobp[j, (2 * dp) * 16 + 8 * g:(2 * dp) * 16 + 8 * g + 8, :] = lo
                wobp[j, (2 * dp + 1) * 16 + 8 * g:(2 * dp + 1) * 16 + 8 * g + 8, :] = hi

        def woa_prep(j, q, gate):
            row = pl.multiple_of(j * 256, 256)
            woa[q, pl.ds(row, 256), :] = gated(pltpu.bitcast(woast[j, 0:512, q * 128:(q + 1) * 128], U32), gate)

        nu = 8 * PRE // MB
        nblk = D // 16

        def run_units(c, par, units, jobs):
            ticks = []
            for hh, mb in units:
                r32 = pre_matmul(c, par, hh, mb)
                ticks += [r32[i:i + 8] for i in range(0, MB, 8 * CFG['tstep'])]
            if not jobs:
                return
            ticks = ticks[:len(ticks) * (len(units) - CFG['early']) // len(units)]
            total = sum(n for n, _ in jobs)
            z = zero[...]
            cache = {}
            cnt = [0]

            def gate():
                k = cnt[0] * len(ticks) // total
                cnt[0] += 1
                if k not in cache:
                    cache[k] = pltpu.bitcast(ticks[k], U32) & z
                return cache[k]

            for _, fn in jobs:
                fn(gate=gate)

        def relayout_jobs(cn, par, grp):
            jobs = []
            lag = CFG['lag']
            for blk in range(nblk + lag):
                if blk < nblk:
                    jobs.append((8, functools.partial(relayout1, cn, blk)))
                if blk >= lag:
                    jobs.append((4 if lag else 0, functools.partial(relayout2, cn, par, blk - lag)))
            return jobs

        def interleave(*lists):
            items = []
            for l in lists:
                items += [((i + 0.5) / len(l), k, x) for k, (i, x) in enumerate(enumerate(l))]
            items.sort(key=lambda z: z[0])
            return [x for _, _, x in items]

        units_hm = [(hh, mb) for hh in range(8) for mb in range(PRE // MB)]
        units_mh = [(hh, mb) for mb in range(PRE // MB) for hh in range(8)]

        for q in range(W0P):
            w0_copy(q).wait()
            relayout(0, 0, range(q * nblk // W0P, (q + 1) * nblk // W0P))
        x_copy(0).wait()

        def loop_x(i, carry):
            c = 2 * i
            run_units(c, 0, units_mh[0:8], [])

            @pl.when(i == 0)
            def _():
                x_copy(1).wait()

            run_units(c, 0, units_mh[8:22], [])
            w_copy(c + 1).wait()
            run_units(c, 0, units_mh[22:32], relayout_jobs(c + 1, 1, 4))
            w_copy(c + 2).wait()
            run_units(c + 1, 1, units_hm, relayout_jobs(c + 2, 0, 2))
            return carry

        def loop_y(i, carry):
            for par in range(2):
                c = 2 * i + par
                j = c - 4
                i3 = 3 * (i - 2)
                blocks = (i3, i3 + 1) if par == 0 else (i3 + 2,)
                @pl.when(c + 1 < NCH)
                def _():
                    w_copy(c + 1).wait()

                woa_copy(j).wait()
                wob_copy(j).wait()
                for b in blocks:
                    b_copy(b).wait()

                cn = jnp.where(c + 1 < NCH, c + 1, NCH - 2)
                bjobs = []
                for k, b in enumerate(blocks):
                    bjobs += [(16, functools.partial(b_prep1, b, k, cc)) for cc in range(8)]
                for k, b in enumerate(blocks):
                    bjobs += [(16, functools.partial(b_prep2, b, k, cc)) for cc in range(8)]
                jl = [relayout_jobs(cn, 1 - par, 2),
                      [(32, functools.partial(woa_prep, j, q)) for q in range(8)],
                      [(32, functools.partial(wob_prep, j, g)) for g in range(2)],
                      bjobs]
                jobs = interleave(*[l for k, l in enumerate(jl) if k not in CFG['skip']])
                run_units(c, par, units_hm, jobs)
            return carry

        lax.fori_loop(0, 2, loop_x, 0)
        lax.fori_loop(2, NCH // 2, loop_y, 0)

    vm = pltpu.VMEM
    pl.run_scoped(
        phase1,
        vm((PRE, D), BF),
        vm((NCH, D, 8, E), BF),
        vm((8, 512, D), BF),
        vm((12, 256, D), BF),
        vm((8, D, 128), BF),
        vm((CFG['ntw'], CFG['twp'], 128), U32),
        vm((2, 33 * H, 128), U32),
        vm((2, 33 * 8, 128), U32),
    )
    mem_copy.wait()
    xb_copy(0).wait()
    xar_copy(0).wait()

    def wa_ref(t, h):
        g = h // 8
        return pltpu.bitcast(was[g % 2][(2 * t + g // 2) * 8 + h % 8, 0:D // 2], BF)

    a_scale = E ** -0.5
    b_scale = (D // H) ** -0.5

    def phase23(ola, olb, outa, outb):
        def ol_ref(h):
            return (ola, h) if h < SPLIT else (olb, h - SPLIT)

        def b_out(s):
            o = ob[...]
            tk = []
            row = pl.multiple_of(s * SEG, SEG)
            for j in range(8):
                r = _dot(o, pltpu.bitcast(wobp[j], BF))
                tk.extend(r[8 * i:8 * i + 8] for i in range(4))
                outb[pl.ds(row, SEG), j * 128:(j + 1) * 128] = r.astype(BF)
            return tk

        def outb_copy(s, n):
            row = pl.multiple_of(s * SEG, SEG)
            return pltpu.make_async_copy(
                outb.at[pl.ds(row, n * SEG), :], out.at[pl.ds(row, n * SEG), pl.ds(D, D)], sem_out.at[1])

        def outa_copy(row, n):
            return pltpu.make_async_copy(
                outa.at[pl.ds(row, n), :], out.at[pl.ds(row, n), pl.ds(0, D)], sem_out.at[0])

        def make_gate(tk, n):
            cnt = [0]
            cache = {}

            def gate(x):
                if not tk:
                    return x
                k = cnt[0] * len(tk) // n
                cnt[0] += 1
                if k not in cache:
                    cache[k] = pltpu.bitcast(tk[k], U32) & zero[...]
                return pltpu.bitcast(pltpu.bitcast(x, U32) | cache[k], F32)
            return gate

        def b_qk(s, i, gate):
            q = [qb[cc, 8 * i:8 * i + 8, :] for cc in range(8)]
            pos = s * SEG + 8 * i + lax.broadcasted_iota(jnp.int32, (8, 128), 0)
            logits = []
            for w in range(WIN):
                lo = HIST + 8 * i - DIL * w
                t = None
                for cc in range(8):
                    x = gate(kb[cc, lo:lo + 8, :]) * q[cc]
                    t = x if t is None else t + x
                t = t + pltpu.roll(t, 64, 1)
                t = t + pltpu.roll(t, 32, 1)
                if w > 0:
                    t = jnp.where(pos >= DIL * w, t, NEG)
                logits.append(t)
            m = functools.reduce(jnp.maximum, logits)
            return logits, m

        def b_sm(i, logits, m, gate):
            ex = [jnp.exp(gate(t) - m) for t in logits]
            r = _rcp(functools.reduce(lambda a, b: a + b, ex))
            for w in range(WIN):
                pb[w, 8 * i:8 * i + 8, :] = gate(ex[w]) * r

        def b_pv(gate):
            for i in range(4):
                p = [pb[w, 8 * i:8 * i + 8, :] for w in range(WIN)]
                for cc in range(8):
                    t = None
                    for w in range(WIN):
                        lo = HIST + 8 * i - DIL * w
                        x = gate(vb[cc, lo:lo + 8, :]) * p[w]
                        t = x if t is None else t + x
                    ob[8 * i:8 * i + 8, cc * 128:(cc + 1) * 128] = t.astype(BF)

        def step(s):
            xrows = xbb[pl.ds(pl.multiple_of(s * SEG, SEG), SEG), :]
            bt = []
            for cc in range(8):
                kb[cc, 0:HIST, :] = kb[cc, SEG:SEG + HIST, :]
            for cc in range(8):
                r = _dot(xrows, pltpu.bitcast(wb[cc], BF))
                qb[cc] = r * b_scale
                bt.extend(r[8 * i:8 * i + 8] for i in range(4))
                r = _dot(xrows, pltpu.bitcast(wb[8 + cc], BF))
                kb[cc, HIST:HIST + SEG, :] = r
                bt.extend(r[8 * i:8 * i + 8] for i in range(4))
            b_pv(make_gate(bt[:CFG['vticks']], 256))
            for cc in range(8):
                vb[cc, 0:HIST, :] = vb[cc, SEG:SEG + HIST, :]
            for cc in range(8):
                r = _dot(xrows, pltpu.bitcast(wb[16 + cc], BF))
                vb[cc, HIST:HIST + SEG, :] = r
                bt.extend(r[8 * i:8 * i + 8] for i in range(4))
            bt.extend(b_out(jnp.maximum(s - 1, 0)))
            gate = make_gate(bt[CFG['q0']:CFG['q1']], 256)
            lm = [b_qk(s, i, gate) for i in range(4)]

            lhs = jnp.concatenate([memb[...], xar[pl.ds(pl.multiple_of(s * XR, 8), XR), :]], axis=0)
            slot = (s % NS) * NG
            offs = [slot]
            for i in range(3):
                g = PRE // 8 + 3 * s + i
                offs.append(((g // 4) % NS) * NG + 1 + g % 4)
            oofs = [pl.multiple_of(s * 32, 32)]
            for i in range(4):
                g = 4 * s + i
                oofs.append(pl.multiple_of(
                    jnp.where(g < 3 * NSEG, (g // 3) * 32 + MEM + 8 * (g % 3),
                              NSEG * 32 + (g - 3 * NSEG) * 8), 8))

            def proj(h):
                p = h // 2
                ring = rings[p % NB]
                ro = (p // NB) * 16 + (h % 2) * 8
                for t in range(3):
                    r32 = _dot(lhs, wa_ref(t, h))
                    for i in range(4):
                        if CFG['mdead'][i] == 3 * h + t:
                            d0 = pltpu.bitcast(lm[i][1], U32) & zero[...]
                            a0 = pltpu.bitcast(pltpu.bitcast(r32[0:8], U32) | d0, F32)
                            r32 = jnp.concatenate([a0, r32[8:]], axis=0)
                    ticks.extend(r32[8 * i:8 * i + 8] for i in range(4))
                    for i in range(4):
                        if CFG['mdead'][i] + CFG['sspan'] == 3 * h + t:
                            b_sm(i, lm[i][0], lm[i][1], make_gate(ticks[-4 * CFG['sspan']:], 16))
                    r = r32.astype(BF)
                    for i in range(4):
                        ring[t, offs[i], ro:ro + 8, :] = r[8 * i:8 * i + 8]

            probs = {}
            ticks = []
            bticks = {}

            def pair(t, p):
                ro = (p // NB) * 16
                return rings[p % NB][t, pl.ds(slot, NG), ro:ro + 16, :].reshape(PAIR, E)

            def att1(p, dead=None):
                q = pair(0, p)
                k = pair(1, p)
                sc = lax.dot_general(q, k, (((1,), (1,)), ((), ())), preferred_element_type=F32)
                if not CFG['exp2']:
                    sc = sc * a_scale
                fl = fill[...]
                if dead is not None:
                    d0 = (pltpu.bitcast(dead, U32) & zero[...])[:, :PAIR]
                    f0 = pltpu.bitcast(pltpu.bitcast(fl[0:8], U32) | d0, F32)
                    fl = jnp.concatenate([f0, fl[8:]], axis=0)
                sc = jnp.where(fl == 0.0, sc, fl)
                if CFG['exp2']:
                    e = jnp.exp2((sc - jnp.max(sc, axis=1, keepdims=True)) * (a_scale * LOG2E))
                else:
                    e = jnp.exp(sc - jnp.max(sc, axis=1, keepdims=True))
                probs[p] = (e * _rcp(jnp.sum(e, axis=1, keepdims=True))).astype(BF)

            def att2(p):
                o = _dot(probs.pop(p), pair(2, p)).astype(BF)
                for i in range(NG):
                    for hh in range(2):
                        ol, hi = ol_ref(2 * p + hh)
                        ol[pl.ds(oofs[i], 8), hi * E:(hi + 1) * E] = o[16 * i + 8 * hh:16 * i + 8 * hh + 8]

            def do(ev):
                kind, p = ev
                if kind == 1:
                    att1(p)
                else:
                    att2(p)

            events = {}
            G = CFG['G']
            for p in range(H // 2):
                if G == 1:
                    h1, h2 = 2 * p + 2, 2 * p + 5
                    if h1 >= H: h1 = H + (h1 - H)
                    if h2 >= H: h2 = H + (h2 - H + 1)
                else:
                    g0 = (p // G) * G
                    h1 = 2 * (g0 + G) - 1 + CFG['d1']
                    h2 = h1 + CFG['d2']
                events.setdefault(h1, []).append((1, p))
                events.setdefault(h2, []).append((2, p))
            for h in events:
                events[h].sort(key=lambda e: (-e[0], e[1]) if CFG['o21'] else e)
            for h in range(H):
                proj(h)
                for ev in events.get(h, []):
                    do(ev)
            l1 = ola[pl.ds(oofs[0], 32), :]
            for j in range(8):
                r = _dot(l1, pltpu.bitcast(woa[j, :SPLIT * 64, :], BF))
                acc[j] = r
                ticks.extend(r[8 * i:8 * i + 8] for i in range(4))
                for ev in events.get(H + j, []):
                    do(ev)
            assert max(events) < H + 8
            assert all(p >= SPLIT // 2 for h in events if h >= H for k, p in events[h] if k == 2)
            l2 = olb[pl.ds(oofs[0], 32), :]
            orow = pl.multiple_of(s * XR, 8)
            for j in range(8):
                res = (acc[j] + _dot(l2, pltpu.bitcast(woa[j, SPLIT * 64:, :], BF))).astype(BF)
                memb[:, j * 128:(j + 1) * 128] = res[0:MEM]
                outa[pl.ds(orow, XR), j * 128:(j + 1) * 128] = res[MEM:]

        def steps(i, carry):
            s0 = i * U

            @pl.when(i == NSEG // U // 2)
            def _():
                xb_copy(1).wait()
                xar_copy(1).wait()

            @pl.when(i >= 1)
            def _():
                outa_copy(pl.multiple_of((s0 - U) * XR, 8), U * XR).start()

            @pl.when(i >= 2)
            def _():
                outb_copy(s0 - 2 * U, U).start()

            for u in range(U):
                step(s0 + u)
            return carry

        lax.fori_loop(0, NSEG // U, steps, 0)

        outa_copy((NSEG - U) * XR, U * XR).start()
        outb_copy(NSEG - 2 * U, U).start()
        b_pv(make_gate([], 1))
        b_out(NSEG - 1)
        outb_copy(NSEG - U, U).start()

        def post(i, carry):
            lrow = pl.multiple_of(NSEG * 32 + i * 128, 128)
            lhs = jnp.concatenate([ola[pl.ds(lrow, 128), :], olb[pl.ds(lrow, 128), :]], axis=1)
            row = pl.multiple_of(NSEG * XR + i * 128, 128)
            for j in range(8):
                outa[pl.ds(row, 128), j * 128:(j + 1) * 128] = _dot(lhs, pltpu.bitcast(woa[j], BF)).astype(BF)
            outa_copy(row, 128).start()
            return carry

        lax.fori_loop(0, PRE // 128, post, 0)

        pltpu.make_async_copy(outb, out.at[:, pl.ds(D, D)], sem_out.at[1]).wait()
        pltpu.make_async_copy(outa, out.at[:, pl.ds(0, D)], sem_out.at[0]).wait()

    pl.run_scoped(
        phase23,
        vm((OLROWS, SPLIT * E), BF),
        vm((OLROWS, (H - SPLIT) * E), BF),
        vm((S, D), BF),
        vm((S, D), BF),
    )


@jax.jit
def _run(A_x, A_mem0, A_Wq, A_Wk, A_Wv, A_Wo, B_x, B_wqkv, B_wo):
    assert A_x.shape == (1, S, D) and A_mem0.shape == (1, MEM, D)
    assert A_Wq.shape == (D, H, E) and A_Wo.shape == (H, E, D)
    assert B_x.shape == (1, S, D) and B_wqkv.shape == (D, 3 * D) and B_wo.shape == (D, D)
    vm = pltpu.VMEM
    dma = pltpu.SemaphoreType.DMA
    scratch = [
        vm((NSEG * XR, D), BF),
        vm((S, D), BF),
        vm((MEM, D), BF),
        vm((48, D // 2 + CFG['wpad'], E), U32),
        vm((48, D // 2 + CFG['wpad'], E), U32),
        vm((8, H * E // 2, 128), U32),
        vm((24, D // 2, 128), U32),
        vm((8, D // 2, 128), U32),
    ] + [vm((3, NS * NG, 64, E), BF)] * NB + [
        vm((8, 32, 128), F32),
        vm((PAIR, PAIR), F32),
        vm((8, SEG, 128), F32),
        vm((8, HIST + SEG, 128), F32),
        vm((8, HIST + SEG, 128), F32),
        vm((WIN, SEG, 128), F32),
        vm((SEG, D), BF),
        vm((8, 128), U32),
        dma((sum(SEM_N),)), dma((2,)),
    ]
    out = pl.pallas_call(
        _kernel,
        out_shape=jax.ShapeDtypeStruct((S, 2 * D), BF),
        in_specs=[pl.BlockSpec(memory_space=pl.ANY)] * 9,
        out_specs=pl.BlockSpec(memory_space=pl.ANY),
        scratch_shapes=scratch,
        compiler_params=pltpu.CompilerParams(vmem_limit_bytes=120 * 1024 * 1024,
                                             disable_bounds_checks=CFG['nobc']),
    )(A_x.reshape(S, D), A_mem0.reshape(MEM, D), A_Wq, A_Wk, A_Wv, A_Wo.reshape(H * E, D),
      B_x.reshape(S, D), B_wqkv, B_wo)
    return out.reshape(1, S, 2 * D)


def pallas_concat_heads__memory_aug_recurrent_mem_tr__sliding_local_dilated__prompt_kernel(
    A_x, A_mem0, A_Wq, A_Wk, A_Wv, A_Wo, A_seg_len, B_x, B_wqkv, B_wo):
    if isinstance(A_seg_len, int):
        assert A_seg_len == SEG
    return _run(A_x, A_mem0, A_Wq, A_Wk, A_Wv, A_Wo, B_x, B_wqkv, B_wo)
```

```python
import functools

import jax
import jax.numpy as jnp
from jax import lax
import jax.experimental.pallas as pl
import jax.experimental.pallas.tpu as pltpu

BF = jnp.bfloat16
F32 = jnp.float32
U32 = jnp.uint32

S = 2048
D = 1024
H = 32
E = 128
MEM = 8
SEG = 32
L = MEM + SEG
NSEG = S // SEG
XR = 24
PRE = S - NSEG * XR
NS = 17
PAIR = 2 * L
OLROWS = 80
BM = 2 * SEG
WIN = 8
DIL = 2
HIST = 16
NCH = 12
NEG = -1000000000.0
LOG2E = 1.4426950408889634
CFG = dict(nv=4, ng=4, qn=2, m0=4, mstep=2, ks=3, pvj=4, pv0=0, e1=0, e2=2, e3=2, nq=2, sideall=True, MB=128, KO=8, nosc=True, itscope=False, k1=22, k2=6, pcol=4, PM=128, nox=False, wpad=0, ntw=4, twp=80, sst=False, lag=1, skip=(), vticks=60, q0=64, q1=128, mdead=(0, 2, 4, 6), sspan=2, exp2=False, d1=3, d2=9, order=((0, 0), (0, 1), (0, 2), (1, 0), (1, 1), (1, 2)), bqk=(1, 4, 7, 10), bpv=(5, 8, 11, 14), qspan=36, vspan=36, tstep=1, early=2, bdead=(2, 5, 8, 11), U=4, nobc=True, battn=(2, 5, 8, 11), SPLIT=24, W0P=4)
U = CFG['U']
MB = CFG['MB']
NB = 4
NG = L // 8
SPLIT = CFG['SPLIT']
KO = CFG['KO']
W0P = CFG['W0P']

SEM_N = (3, W0P, NCH, 4, 4, 4, 1, 1)
SEM_BASE = tuple(sum(SEM_N[:i]) for i in range(len(SEM_N)))


def _rcp(d):
    r = pl.reciprocal(d, approx=True)
    return r * (2.0 - d * r)


def _dot(a, b):
    return jnp.dot(a, b, preferred_element_type=F32)


def _divmod(x, d):
    m = 65536 // d + 1
    assert all((v * m) >> 16 == v // d for v in range(1024))
    q = lax.shift_right_logical(x * m, 16)
    return q, x - q * d


def _lo_hi(a, b):
    lo = (a & U32(0xFFFF)) | (b << 16)
    hi = (a >> 16) | (b & U32(0xFFFF0000))
    return lo, hi


def _kernel(xa, mem0, wq, wk, wv, wo, xb, wqkv, wob, out,
            xar, xbb, memb, wa0, wa1, woa, wb, wobp,
            r0, r1, r2, r3, acc, fill, qb, kb, vb, pb, ob, zero,
            sem, sem_out):
    class _Sems:
        def __init__(self, base):
            self.base = base
            self.at = self

        def __getitem__(self, i):
            return sem.at[self.base + i]

    sem_x, sem_w0, sem_w, sem_b, sem_wob, sem_woa, sem_hx, sem_xb = [_Sems(b) for b in SEM_BASE]
    rings = (r0, r1, r2, r3)
    was = (wa0, wa1)
    wsrc = (wq, wk, wv)

    xar_copy = pltpu.make_async_copy(xa.at[pl.ds(PRE, NSEG * XR), :], xar, sem_hx.at[0])
    xb_copy = pltpu.make_async_copy(xb, xbb, sem_xb.at[0])
    mem_copy = pltpu.make_async_copy(mem0, memb, sem_x.at[0])

    def phase1(xpre, wst, woast, bst, wobst, tw, tb, tob):
        def st(i):
            return i if isinstance(i, int) else 0

        def w_copy(c):
            return pltpu.make_async_copy(
                wsrc[st(c) // 4].at[:, pl.ds((st(c) % 4) * 8, 8), :], wst.at[c], sem_w.at[c])

        def w0_copy(q):
            n = D // W0P
            return pltpu.make_async_copy(
                wq.at[pl.ds(q * n, n), pl.ds(0, 8), :], wst.at[0, pl.ds(q * n, n)], sem_w0.at[q])

        def x_copy(q):
            lo, n = ((0, MB), (MB, PRE - MB))[q]
            return pltpu.make_async_copy(
                xa.at[pl.ds(lo, n), :], xpre.at[pl.ds(lo, n), :], sem_x.at[1 + q])

        def b_copy(j):
            return pltpu.make_async_copy(wqkv.at[pl.ds(st(j) * 256, 256), :], bst.at[j], sem_b.at[j])

        def wob_copy(j):
            return pltpu.make_async_copy(wob.at[:, pl.ds(st(j) * 256, 256)], wobst.at[j], sem_wob.at[j])

        def woa_copy(j):
            return pltpu.make_async_copy(
                wo.at[pl.ds(st(j) * 2, 2)], woast.at[pl.ds(j * 2, 2)], sem_woa.at[j])

        for q in range(W0P):
            w0_copy(q).start()
        x_copy(0).start()
        x_copy(1).start()
        for c in range(1, 5):
            w_copy(c).start()
        for j in range(4):
            woa_copy(j).start()
            wob_copy(j).start()
            b_copy(j).start()
            w_copy(2 * j + 5).start()
            if 2 * j + 6 < NCH:
                w_copy(2 * j + 6).start()
        mem_copy.start()
        xb_copy.start()
        xar_copy.start()

        def zero_fill(i, carry):
            r = pl.multiple_of(i * 16, 16)
            woast[8, pl.ds(2 * r, 32), :] = jnp.zeros((32, D), BF)
            bst[4, pl.ds(r, 16), :] = jnp.zeros((16, 3 * D), BF)
            wobst[4, pl.ds(4 * r, 64), :] = jnp.zeros((64, 256), BF)
            return carry

        lax.fori_loop(0, 16, zero_fill, 0)

        ri = lax.broadcasted_iota(jnp.int32, (PAIR, PAIR), 0)
        ci = lax.broadcasted_iota(jnp.int32, (PAIR, PAIR), 1)
        rb = (ri >> 3) & 1
        cb = (ci >> 3) & 1
        rl = ((ri >> 4) << 3) | (ri & 7)
        cl = ((ci >> 4) << 3) | (ci & 7)
        allowed = (rl < MEM) | (rl >= cl)
        fill[...] = jnp.where(rb == cb, jnp.where(allowed, 0.0, NEG / E ** -0.5 if CFG['exp2'] else NEG), -jnp.inf).astype(F32)
        kb[...] = jnp.zeros(kb.shape, F32)
        vb[...] = jnp.zeros(vb.shape, F32)
        zero[...] = jnp.zeros(zero.shape, U32)

        def relayout1(c, blk, slot, gate=None):
            v = wst[c, pl.ds(blk * 16, 16)]
            v = pltpu.bitcast(v.reshape(128, 128), U32)
            for dp in range(8):
                x = v[8 * dp:8 * dp + 8]
                tw[slot, 9 * dp:9 * dp + 8, :] = x if gate is None else x | gate()

        def relayout2(dst, base, blk, slot, gate=None):
            row = blk * 8 if isinstance(blk, int) else pl.multiple_of(blk * 8, 8)
            for j in range(4):
                a, b = tw[slot, pl.ds(j, 8, stride=9), :], tw[slot, pl.ds(4 + j, 8, stride=9), :]
                if gate is not None:
                    g = gate()
                    a, b = a | g, b | g
                lo, hi = _lo_hi(a, b)
                dst[base + 2 * j, pl.ds(row, 8), :] = lo
                dst[base + 2 * j + 1, pl.ds(row, 8), :] = hi

        def pre_matmul(c, src, base, hh, mb):
            t = c >> 2
            g = c & 3
            row = mb * MB if isinstance(mb, int) else pl.multiple_of(mb * MB, MB)
            r32 = _dot(xpre[pl.ds(row, MB), :], pltpu.bitcast(src[base + hh], BF))
            r = r32.astype(BF)
            ring = rings[hh // 2]
            off = (g * 16 if isinstance(g, int) else pl.multiple_of(g * 16, 16)) + (hh % 2) * 8
            for k in range(MB // 8):
                ring[t, mb * (MB // SEG * NG) + (k // 4) * NG + 1 + k % 4, pl.ds(off, 8), :] = r[8 * k:8 * k + 8]
            return [r32[i:i + 8] for i in range(0, MB, 8 * CFG['tstep'])]

        def quarters(c, src, base, mbs):
            ticks = []
            for mb in mbs:
                for hh in range(8):
                    ticks += pre_matmul(c, src, base, hh, mb)
            return ticks

        def gated(x, gate):
            return jnp.concatenate([x[i:i + 8] | gate() for i in range(0, x.shape[0], 8)], axis=0)

        def b_prep1(js, p, cc, gate):
            col = p * D + cc * 128
            x32 = gated(pltpu.bitcast(bst[js, :, col:col + 128], U32), gate).T
            for hl in range(4):
                h = 4 * cc + hl
                tb[p, 33 * h:33 * h + 32, :] = x32[32 * hl:32 * hl + 32]

        def b_prep2(jd, p, cc, gate):
            y = jnp.concatenate(
                [tb[p, pl.ds(4 * cc + dl + 33 * 8 * g, 8, stride=33), :] for dl in range(4) for g in range(4)],
                axis=0)
            wb[p * 8 + cc, pl.ds(pl.multiple_of(jd * 128, 128), 128), :] = gated(y, gate).T

        def wob_prep(js, jd, e, g, gate):
            v = wobst[js, g * 512:(g + 1) * 512, e * 128:(e + 1) * 128]
            v = gated(pltpu.bitcast(v, U32), gate)
            for hp in range(8):
                tob[g, 33 * hp:33 * hp + 32, :] = v[32 * hp:32 * hp + 32]
            for dp in range(16):
                lo, hi = _lo_hi(tob[g, pl.ds(dp, 8, stride=33), :], tob[g, pl.ds(16 + dp, 8, stride=33), :])
                wobp[2 * jd + e, (2 * dp) * 16 + 8 * g:(2 * dp) * 16 + 8 * g + 8, :] = lo
                wobp[2 * jd + e, (2 * dp + 1) * 16 + 8 * g:(2 * dp + 1) * 16 + 8 * g + 8, :] = hi

        def woa_prep(us, ud, q, gate):
            row = pl.multiple_of(ud * 256, 256)
            woa[q, pl.ds(row, 256), :] = gated(pltpu.bitcast(woast[us, :, q * 128:(q + 1) * 128], U32), gate)

        nblk = D // 16
        ntw = tw.shape[0]

        def run_jobs(ticks, jobs):
            total = sum(n for n, _ in jobs)
            z = zero[...]
            cache = {}
            cnt = [0]

            def gate():
                k = cnt[0] * len(ticks) // total
                cnt[0] += 1
                if k not in cache:
                    cache[k] = pltpu.bitcast(ticks[k], U32) & z
                return cache[k]

            for _, fn in jobs:
                fn(gate=gate)

        def relayout_jobs(c, dst, base):
            jobs = []
            for blk in range(nblk + 1):
                if blk < nblk:
                    jobs.append((8, functools.partial(relayout1, c, blk, blk % ntw)))
                if blk >= 1:
                    jobs.append((4, functools.partial(relayout2, dst, base, blk - 1, (blk - 1) % ntw)))
            return jobs

        def interleave(*lists):
            items = []
            for l in lists:
                items += [((i + 0.5) / len(l), x) for i, x in enumerate(l)]
            items.sort(key=lambda z: z[0])
            return [x for _, x in items]

        def trim(ticks, units):
            return ticks[:len(ticks) - units * (MB // 8 // CFG['tstep'])]

        def first_chunk(q, carry):
            w0_copy(q).wait()
            n = nblk // W0P
            for k in range(n):
                relayout1(0, q * n + k, k % ntw)
                relayout2(wa0, 0, q * n + k, k % ntw)
            return carry

        lax.fori_loop(0, W0P, first_chunk, 0)
        x_copy(0).wait()

        def pair_of_chunks(i, carry):
            c = 2 * i
            w_copy(c + 1).wait()
            ticks = quarters(c, wa0, i * 8, [3])
            run_jobs(trim(ticks, CFG['e1']), relayout_jobs(c + 1, wa1, i * 8))
            quarters(c + 1, wa1, i * 8, range(CFG['nq']))
            w_copy(c + 2).wait()

            @pl.when(i >= 1)
            def _():
                woa_copy(i - 1).wait()
                wob_copy(i - 1).wait()
                b_copy(i - 1).wait()

            ticks = quarters(c + 1, wa1, i * 8, range(CFG['nq'], 4))
            run_jobs(trim(ticks, CFG['e2']), relayout_jobs(c + 2, wa0, i * 8 + 8))
            ticks2 = quarters(c + 2, wa0, i * 8 + 8, range(3))
            js = jnp.where(i >= 1, i - 1, 4)
            jd = jnp.maximum(i - 1, 0)
            us = [jnp.where(i >= 1, 2 * i - 2 + e, 8) for e in range(2)]
            jobs = interleave(
                [(32, functools.partial(woa_prep, us[e], 2 * jd + e, q)) for e in range(2) for q in range(8)],
                [(32, functools.partial(wob_prep, js, jd, e, g)) for e in range(2) for g in range(2)],
                [(16, functools.partial(f, j_, p, cc))
                 for p in range(3) for f, j_ in ((b_prep1, js), (b_prep2, jd)) for cc in range(8)])
            run_jobs(trim((ticks if CFG['sideall'] else []) + ticks2, CFG['e3']), jobs)
            return carry

        def outer(k, carry):
            def quarter(mb, carry2):
                @pl.when((k == 0) & (mb == 1))
                def _():
                    x_copy(1).wait()

                quarters(k * (NCH - 1), wa0, k * 48, [mb])
                return carry2

            lax.fori_loop(0, 3 + k, quarter, 0)

            @pl.when(k == 0)
            def _():
                lax.fori_loop(0, NCH // 2 - 1, pair_of_chunks, 0)
                w_copy(NCH - 1).wait()
                ticks = quarters(NCH - 2, wa0, 40, [3])
                run_jobs(trim(ticks, CFG['e1']), relayout_jobs(NCH - 1, wa0, 48))

            return carry

        lax.fori_loop(0, 2, outer, 0)

    vm = pltpu.VMEM
    pl.run_scoped(
        phase1,
        vm((PRE, D), BF),
        vm((NCH, D, 8, E), BF),
        vm((9, 512, D), BF),
        vm((5, 256, 3 * D), BF),
        vm((5, D, 256), BF),
        vm((CFG['ntw'], CFG['twp'], 128), U32),
        vm((3, 33 * H + 40, 128), U32),
        vm((2, 33 * 8 + 32, 128), U32),
    )
    mem_copy.wait()
    xb_copy.wait()
    xar_copy.wait()

    def wa_ref(t, h):
        c = 4 * t + h // 8
        ref, base = (wa0, 48) if c == NCH - 1 else (was[c % 2], (c // 2) * 8)
        return pltpu.bitcast(ref[base + h % 8], BF)

    a_scale = E ** -0.5
    b_scale = (D // H) ** -0.5

    def phase23(ola, olb, outa, outb):
        def ol_ref(h):
            return (ola, h) if h < SPLIT else (olb, h - SPLIT)

        def out_copy(buf, row, c0, nc, half):
            return pltpu.make_async_copy(
                buf.at[pl.ds(row, BM), pl.ds(c0, nc)], out.at[pl.ds(row, BM), pl.ds(half * D + c0, nc)],
                sem_out.at[half])

        def b_out(row):
            o = ob[...]
            for j in range(8):
                outb[pl.ds(row, BM), j * 128:(j + 1) * 128] = _dot(o, pltpu.bitcast(wobp[j], BF)).astype(BF)
                if (j + 1) % CFG['pcol'] == 0:
                    out_copy(outb, row, (j + 1 - CFG['pcol']) * 128, CFG['pcol'] * 128, 1).start()

        def make_gate(tk, n):
            cnt = [0]
            cache = {}

            def gate(x):
                if not tk:
                    return x
                k = cnt[0] * len(tk) // n
                cnt[0] += 1
                if k not in cache:
                    cache[k] = pltpu.bitcast(tk[k], U32) & zero[...]
                return pltpu.bitcast(pltpu.bitcast(x, U32) | cache[k], F32)
            return gate

        def b_qk(row, i, gate):
            q = [qb[cc, 8 * i:8 * i + 8, :] for cc in range(8)]
            pos = row + 8 * i + lax.broadcasted_iota(jnp.int32, (8, 128), 0)
            logits = []
            for w in range(WIN):
                lo = HIST + 8 * i - DIL * w
                t = None
                for cc in range(8):
                    x = gate(kb[cc, lo:lo + 8, :]) * q[cc]
                    t = x if t is None else t + x
                t = t + pltpu.roll(t, 64, 1)
                t = t + pltpu.roll(t, 32, 1)
                if 8 * i < DIL * w:
                    t = jnp.where(pos >= DIL * w, t, NEG)
                logits.append(t)
            m = functools.reduce(jnp.maximum, logits)
            return logits, m

        def b_sm(i, logits, m, gate):
            ex = [jnp.exp(gate(t) - m) for t in logits]
            r = _rcp(functools.reduce(lambda a, b: a + b, ex))
            for w in range(WIN):
                pb[w, 8 * i:8 * i + 8, :] = gate(ex[w]) * r

        def b_pv(gate):
            for i in range(BM // 8):
                p = [pb[w, 8 * i:8 * i + 8, :] for w in range(WIN)]
                for cc in range(8):
                    t = None
                    for w in range(WIN):
                        lo = HIST + 8 * i - DIL * w
                        x = gate(vb[cc, lo:lo + 8, :]) * p[w]
                        t = x if t is None else t + x
                    ob[8 * i:8 * i + 8, cc * 128:(cc + 1) * 128] = t.astype(BF)

        def step(s, u):
            brow = pl.multiple_of((s - u % 2) * SEG, BM)
            xrows = xbb[pl.ds(brow, BM), :]
            nv = CFG['nv']
            if u % 2 == 0:
                for cc in range(8):
                    kb[cc, 0:HIST, :] = kb[cc, BM:BM + HIST, :]
                    vb[cc, 0:HIST, :] = vb[cc, BM:BM + HIST, :]
                for cc in range(8):
                    qb[cc] = _dot(xrows, pltpu.bitcast(wb[cc], BF)) * b_scale
                    kb[cc, HIST:HIST + BM, :] = _dot(xrows, pltpu.bitcast(wb[8 + cc], BF))
            ticks = []
            for cc in (range(nv) if u % 2 == 0 else range(nv, 8)):
                r = _dot(xrows, pltpu.bitcast(wb[16 + cc], BF))
                vb[cc, HIST:HIST + BM, :] = r
                ticks.extend(r[8 * i:8 * i + 8] for i in range(BM // 8))
            groups = range(CFG['ng']) if u % 2 == 0 else range(CFG['ng'], BM // 8)
            lm = {}

            lhs = jnp.concatenate([memb[...], xar[pl.ds(pl.multiple_of(s * XR, 8), XR), :]], axis=0)
            slot = _divmod(s, NS)[1] * NG
            offs = [slot]
            for i in range(3):
                g = PRE // 8 + 3 * s + i
                offs.append(_divmod(g >> 2, NS)[1] * NG + 1 + (g & 3))
            oofs = (0, 8, 16, 24, 40) if u % 2 == 0 else (32, 48, 56, 64, 72)
            nrow = 32 if u % 2 == 0 else 48

            def proj(h, t, n):
                p = h // 2
                ring = rings[p % NB]
                ro = (p // NB) * 16 + (h % 2) * 8
                r32 = _dot(lhs, wa_ref(t, h))
                for k, i in enumerate(groups):
                    if CFG['m0'] + CFG['mstep'] * k == n:
                        d0 = pltpu.bitcast(lm[i][1], U32) & zero[...]
                        a0 = pltpu.bitcast(pltpu.bitcast(r32[0:8], U32) | d0, F32)
                        r32 = jnp.concatenate([a0, r32[8:]], axis=0)
                ticks.extend(r32[8 * i:8 * i + 8] for i in range(4))
                if n == CFG['qn']:
                    gate = make_gate(list(ticks), 64 * len(groups))
                    for i in groups:
                        lm[i] = b_qk(brow, i, gate)
                for k, i in enumerate(groups):
                    if CFG['m0'] + CFG['mstep'] * k + CFG['sspan'] == n:
                        b_sm(i, lm[i][0], lm[i][1], make_gate(ticks[-4 * CFG['sspan']:], 16))
                r = r32.astype(BF)
                for i in range(4):
                    ring[t, offs[i], ro:ro + 8, :] = r[8 * i:8 * i + 8]

            probs = {}

            def pair(t, p):
                ro = (p // NB) * 16
                return rings[p % NB][t, pl.ds(slot, NG), ro:ro + 16, :].reshape(PAIR, E)

            def att1(p, dead=None):
                q = pair(0, p)
                k = pair(1, p)
                sc = lax.dot_general(q, k, (((1,), (1,)), ((), ())), preferred_element_type=F32)
                if not CFG['exp2']:
                    sc = sc * a_scale
                fl = fill[...]
                if dead is not None:
                    d0 = (pltpu.bitcast(dead, U32) & zero[...])[:, :PAIR]
                    f0 = pltpu.bitcast(pltpu.bitcast(fl[0:8], U32) | d0, F32)
                    fl = jnp.concatenate([f0, fl[8:]], axis=0)
                sc = jnp.where(fl == 0.0, sc, fl)
                if CFG['exp2']:
                    e = jnp.exp2((sc - jnp.max(sc, axis=1, keepdims=True)) * (a_scale * LOG2E))
                else:
                    e = jnp.exp(sc - jnp.max(sc, axis=1, keepdims=True))
                probs[p] = (e * _rcp(jnp.sum(e, axis=1, keepdims=True))).astype(BF)

            def att2(p):
                o = _dot(probs.pop(p), pair(2, p)).astype(BF)
                for i in range(NG):
                    for hh in range(2):
                        ol, hi = ol_ref(2 * p + hh)
                        ol[oofs[i]:oofs[i] + 8, hi * E:(hi + 1) * E] = o[16 * i + 8 * hh:16 * i + 8 * hh + 8]

            def do(ev):
                kind, p = ev
                if kind == 1:
                    att1(p)
                else:
                    att2(p)

            events = {}
            for p in range(H // 2):
                n1 = 6 * p + 5 + CFG['d1']
                n2 = n1 + CFG['d2']
                events.setdefault(n1, []).append((1, p))
                events.setdefault(n2, []).append((2, p))
            order = CFG['order']
            n = 0
            for p in range(H // 2):
                for hh, t in order:
                    proj(2 * p + hh, t, n)
                    for ev in events.get(n, []):
                        do(ev)
                    n += 1
            oticks = []
            ks = CFG['ks'] if u % 2 == 1 else 1
            kw = SPLIT * 128 // ks
            l1 = ola[oofs[0]:oofs[0] + nrow, :]
            for j in range(8):
                r = None
                for k in range(ks):
                    x = _dot(l1[:, k * kw:(k + 1) * kw], pltpu.bitcast(woa[j, k * kw // 2:(k + 1) * kw // 2, :], BF))
                    r = x if r is None else r + x
                    oticks.extend(r[8 * i:8 * i + 8] for i in range(nrow // 8))
                acc[j, 0:nrow, :] = r
                for n in range(3 * H + 3 * j, 3 * H + 3 * j + 3):
                    for ev in events.get(n, []):
                        do(ev)
            assert max(events) < 3 * H + 24
            assert all(p >= SPLIT // 2 for n in events if n >= 3 * H for k, p in events[n] if k == 2)
            l2 = olb[oofs[0]:oofs[0] + nrow, :]
            orow = pl.multiple_of(s * SEG - (u % 2) * 8, 8)
            for j in range(8):
                r = acc[j, 0:nrow, :] + _dot(l2, pltpu.bitcast(woa[j, SPLIT * 64:, :], BF))
                if j < CFG['pvj']:
                    oticks.extend(r[8 * i:8 * i + 8] for i in range(nrow // 8))
                res = r.astype(BF)
                memb[:, j * 128:(j + 1) * 128] = res[0:MEM]
                outa[pl.ds(orow, nrow - MEM), j * 128:(j + 1) * 128] = res[MEM:]
            if u % 2 == 1:
                out_copy(outa, brow, 0, D, 0).start()
                b_pv(make_gate(oticks[CFG['pv0']:], 8 * BM))
                b_out(brow)

        def steps(i, carry):
            for u in range(U):
                step(i * U + u, u)
            return carry

        lax.fori_loop(0, NSEG // U, steps, 0)

        pltpu.make_async_copy(outb, out.at[:, pl.ds(D, D)], sem_out.at[1]).wait()
        pltpu.make_async_copy(outa, out.at[:, pl.ds(0, D)], sem_out.at[0]).wait()

    pl.run_scoped(
        phase23,
        vm((OLROWS, SPLIT * E), BF),
        vm((OLROWS, (H - SPLIT) * E), BF),
        vm((S, D), BF),
        vm((S, D), BF),
    )


@jax.jit
def _run(A_x, A_mem0, A_Wq, A_Wk, A_Wv, A_Wo, B_x, B_wqkv, B_wo):
    assert A_x.shape == (1, S, D) and A_mem0.shape == (1, MEM, D)
    assert A_Wq.shape == (D, H, E) and A_Wo.shape == (H, E, D)
    assert B_x.shape == (1, S, D) and B_wqkv.shape == (D, 3 * D) and B_wo.shape == (D, D)
    vm = pltpu.VMEM
    dma = pltpu.SemaphoreType.DMA
    scratch = [
        vm((NSEG * XR, D), BF),
        vm((S, D), BF),
        vm((MEM, D), BF),
        vm((56, D // 2, E), U32),
        vm((40, D // 2, E), U32),
        vm((8, H * E // 2, 128), U32),
        vm((24, D // 2, 128), U32),
        vm((8, D // 2, 128), U32),
    ] + [vm((3, NS * NG, 64, E), BF)] * NB + [
        vm((8, 48, 128), F32),
        vm((PAIR, PAIR), F32),
        vm((8, BM, 128), F32),
        vm((8, HIST + BM, 128), F32),
        vm((8, HIST + BM, 128), F32),
        vm((WIN, BM, 128), F32),
        vm((BM, D), BF),
        vm((8, 128), U32),
        dma((sum(SEM_N),)), dma((2,)),
    ]
    out = pl.pallas_call(
        _kernel,
        out_shape=jax.ShapeDtypeStruct((S, 2 * D), BF),
        in_specs=[pl.BlockSpec(memory_space=pl.ANY)] * 9,
        out_specs=pl.BlockSpec(memory_space=pl.ANY),
        scratch_shapes=scratch,
        compiler_params=pltpu.CompilerParams(vmem_limit_bytes=120 * 1024 * 1024,
                                             disable_bounds_checks=CFG['nobc'],
                                             disable_semaphore_checks=CFG['nosc']),
    )(A_x.reshape(S, D), A_mem0.reshape(MEM, D), A_Wq, A_Wk, A_Wv, A_Wo.reshape(8, 512, D),
      B_x.reshape(S, D), B_wqkv, B_wo)
    return out.reshape(1, S, 2 * D)


def pallas_concat_heads__memory_aug_recurrent_mem_tr__sliding_local_dilated__prompt_kernel(
    A_x, A_mem0, A_Wq, A_Wk, A_Wv, A_Wo, A_seg_len, B_x, B_wqkv, B_wo):
    if isinstance(A_seg_len, int):
        assert A_seg_len == SEG
    return _run(A_x, A_mem0, A_Wq, A_Wk, A_Wv, A_Wo, B_x, B_wqkv, B_wo)
```

```python
import functools

import jax
import jax.numpy as jnp
from jax import lax
import jax.experimental.pallas as pl
import jax.experimental.pallas.tpu as pltpu

BF = jnp.bfloat16
F32 = jnp.float32
U32 = jnp.uint32

S = 2048
D = 1024
H = 32
E = 128
MEM = 8
SEG = 32
L = MEM + SEG
NSEG = S // SEG
XR = 24
PRE = S - NSEG * XR
NS = 17
PAIR = 2 * L
OLROWS = 80
BM = 2 * SEG
WIN = 8
DIL = 2
HIST = 16
NCH = 12
NEG = -1000000000.0
LOG2E = 1.4426950408889634
CFG = dict(f0=0, f1=100, ka=20, e0=4, e0b=0, w1a=640, only2=False, nv=4, ng=4, qn=2, m0=5, mstep=2, ks=3, pvj=4, pv0=0, e1=2, e2=2, e3=2, nq=2, sideall=True, MB=128, KO=8, nosc=True, itscope=False, k1=16, k2=6, pcol=4, PM=128, nox=False, wpad=0, ntw=4, twp=80, sst=False, lag=1, skip=(), vticks=60, q0=64, q1=128, mdead=(0, 2, 4, 6), sspan=2, exp2=True, d1=3, d2=9, order=((0, 0), (0, 1), (0, 2), (1, 0), (1, 1), (1, 2)), bqk=(1, 4, 7, 10), bpv=(5, 8, 11, 14), qspan=36, vspan=36, tstep=1, early=2, bdead=(2, 5, 8, 11), U=4, nobc=True, battn=(2, 5, 8, 11), SPLIT=24, W0P=4)
U = CFG['U']
MB = CFG['MB']
NB = 4
NG = L // 8
SPLIT = CFG['SPLIT']
KO = CFG['KO']
W0P = CFG['W0P']

KP = D // W0P
W1A = CFG['w1a']
SEM_N = (1 + W0P, W0P, NCH, 6, 8, 8, 1, 1)
OA0 = NCH - 1 - 8
OB0 = NCH - 1 - 6
SEM_BASE = tuple(sum(SEM_N[:i]) for i in range(len(SEM_N)))


def _rcp(d):
    r = pl.reciprocal(d, approx=True)
    return r * (2.0 - d * r)


def _dot(a, b):
    return jnp.dot(a, b, preferred_element_type=F32)


def _divmod(x, d):
    m = 65536 // d + 1
    assert all((v * m) >> 16 == v // d for v in range(1024))
    q = lax.shift_right_logical(x * m, 16)
    return q, x - q * d


def _lo_hi(a, b):
    lo = (a & U32(0xFFFF)) | (b << 16)
    hi = (a >> 16) | (b & U32(0xFFFF0000))
    return lo, hi


def _kernel(xa, mem0, wq, wk, wv, wo, xb, wqkv, wob, out,
            xar, xbb, memb, wa, woa, wb, wobp,
            r0, r1, r2, r3, acc, fill, qb, kb, vb, pb, ob, zero,
            sem, sem_out):
    class _Sems:
        def __init__(self, base):
            self.base = base
            self.at = self

        def __getitem__(self, i):
            return sem.at[self.base + i]

    sem_x, sem_w0, sem_w, sem_b, sem_wob, sem_woa, sem_hx, sem_xb = [_Sems(b) for b in SEM_BASE]
    rings = (r0, r1, r2, r3)
    wsrc = (wq, wk, wv)

    xar_copy = pltpu.make_async_copy(xa.at[pl.ds(PRE, NSEG * XR), :], xar, sem_hx.at[0])
    xb_copy = pltpu.make_async_copy(xb, xbb, sem_xb.at[0])
    mem_copy = pltpu.make_async_copy(mem0, memb, sem_x.at[0])

    def phase1(xpre, wst, woast, bst, wobst, tw, tb, tob, pacc):
        def st(i):
            return i if isinstance(i, int) else 0

        def w_copy(c):
            return pltpu.make_async_copy(
                wsrc[st(c) // 4].at[:, pl.ds((st(c) % 4) * 8, 8), :], wst.at[c], sem_w.at[c])

        def w0_copy(q):
            lo = q * KP if isinstance(q, int) else pl.multiple_of(q * KP, KP)
            return pltpu.make_async_copy(
                wq.at[pl.ds(st(q) * KP, KP), pl.ds(0, 8), :], wst.at[0, pl.ds(lo, KP)], sem_w0.at[q])

        def w1_copy(q):
            lo, n = ((0, W1A), (W1A, D - W1A))[q]
            return pltpu.make_async_copy(
                wq.at[pl.ds(lo, n), pl.ds(8, 8), :], wst.at[1, pl.ds(lo, n)], sem_w.at[q])

        def x_copy(q):
            return pltpu.make_async_copy(
                xa.at[pl.ds(0, PRE), pl.ds(st(q) * KP, KP)], xpre.at[q], sem_x.at[1 + q])

        def b_copy(j):
            return pltpu.make_async_copy(
                wqkv.at[pl.ds((st(j) % 2) * 512, 512), pl.ds((st(j) // 2) * D, D)], bst.at[j], sem_b.at[j])

        def wob_copy(j):
            return pltpu.make_async_copy(wob.at[:, pl.ds(st(j) * 128, 128)], wobst.at[j], sem_wob.at[j])

        def woa_copy(j):
            return pltpu.make_async_copy(wo.at[st(j)], woast.at[j], sem_woa.at[j])

        for q in range(W0P):
            w0_copy(q).start()
            x_copy(q).start()
        w1_copy(0).start()
        w1_copy(1).start()
        for c in range(1, NCH - 1):
            w_copy(c + 1).start()
            if c >= OA0:
                woa_copy(c - OA0).start()
                wob_copy(c - OA0).start()
            if c >= OB0:
                b_copy(c - OB0).start()
        mem_copy.start()
        xb_copy.start()
        xar_copy.start()

        def zero_fill(i, carry):
            r = pl.multiple_of(i * 32, 32)
            woast[8, pl.ds(r, 32), :] = jnp.zeros((32, D), BF)
            bst[6, pl.ds(r, 32), :] = jnp.zeros((32, D), BF)
            wobst[8, pl.ds(2 * r, 64), :] = jnp.zeros((64, 128), BF)
            return carry

        lax.fori_loop(0, 16, zero_fill, 0)

        ri = lax.broadcasted_iota(jnp.int32, (PAIR, PAIR), 0)
        ci = lax.broadcasted_iota(jnp.int32, (PAIR, PAIR), 1)
        rb = (ri >> 3) & 1
        cb = (ci >> 3) & 1
        rl = ((ri >> 4) << 3) | (ri & 7)
        cl = ((ci >> 4) << 3) | (ci & 7)
        allowed = (rl < MEM) | (rl >= cl)
        fill[...] = jnp.where(rb == cb, jnp.where(allowed, 0.0, NEG / E ** -0.5 if CFG['exp2'] else NEG), -jnp.inf).astype(F32)
        kb[...] = jnp.zeros(kb.shape, F32)
        vb[...] = jnp.zeros(vb.shape, F32)
        zero[...] = jnp.zeros(zero.shape, U32)
        for u in range(CFG['ka'], 32):
            pacc[u % 8, (u // 8) * MB:(u // 8 + 1) * MB, :] = jnp.zeros((MB, E), F32)

        def relayout1(c, blk, slot, r0=0, gate=None):
            v = wst[c, pl.ds(2 * r0 + blk * 16, 16)]
            v = pltpu.bitcast(v.reshape(128, 128), U32)
            for dp in range(8):
                x = v[8 * dp:8 * dp + 8]
                tw[slot, 9 * dp:9 * dp + 8, :] = x if gate is None else x | gate()

        def relayout2(base, blk, slot, r0=0, gate=None):
            row = r0 + blk * 8
            for j in range(4):
                a, b = tw[slot, pl.ds(j, 8, stride=9), :], tw[slot, pl.ds(4 + j, 8, stride=9), :]
                if gate is not None:
                    g = gate()
                    a, b = a | g, b | g
                lo, hi = _lo_hi(a, b)
                wa[base + 2 * j, pl.ds(row, 8), :] = lo
                wa[base + 2 * j + 1, pl.ds(row, 8), :] = hi

        def ring_store(c, hh, mb, r32):
            t = c >> 2
            g = c & 3
            r = r32.astype(BF)
            ring = rings[hh // 2]
            off = (g * 16 if isinstance(g, int) else pl.multiple_of(g * 16, 16)) + (hh % 2) * 8
            for k in range(MB // 8):
                ring[t, mb * (MB // SEG * NG) + (k // 4) * NG + 1 + k % 4, pl.ds(off, 8), :] = r[8 * k:8 * k + 8]
            return [r32[i:i + 8] for i in range(0, MB, 8 * CFG['tstep'])]

        def pre_matmul(c, base, hh, mb):
            lhs = jnp.concatenate([xpre[q, mb * MB:(mb + 1) * MB, :] for q in range(W0P)], axis=1)
            r32 = _dot(lhs, pltpu.bitcast(wa[base + hh], BF))
            return ring_store(c, hh, mb, r32)

        def run_pieces(q, wrow, u0, u1, first=False):
            ticks = []
            for u in range(u0, u1):
                hh, mb = u % 8, u // 8
                rows = slice(mb * MB, (mb + 1) * MB)
                r32 = _dot(xpre[q, rows, :], pltpu.bitcast(wa[hh, pl.ds(wrow, KP // 2), :], BF))
                if not first:
                    r32 = r32 + pacc[hh, rows, :]
                pacc[hh, rows, :] = r32
                ticks += [r32[i:i + 8] for i in range(0, MB, 8 * CFG['tstep'])]
            return ticks

        def finish_chunk0(u, gate):
            hh, mb = u % 8, u // 8
            r = pltpu.bitcast(pacc[hh, mb * MB:(mb + 1) * MB, :], U32)
            ring_store(0, hh, mb, pltpu.bitcast(gated(r, gate), F32))

        def run_units(c, base, u0, u1):
            ticks = []
            for u in range(u0, u1):
                ticks += pre_matmul(c, base, u % 8, u // 8)
            return ticks

        def gated(x, gate):
            return jnp.concatenate([x[i:i + 8] | gate() for i in range(0, x.shape[0], 8)], axis=0)

        def b_prep1(js, e, cc, gate):
            x32 = pltpu.bitcast(bst[js, e * 256:(e + 1) * 256, cc * 128:(cc + 1) * 128], U32)
            x32 = gated(x32, gate).T
            for hl in range(4):
                h = 4 * cc + hl
                tb[e, 33 * h:33 * h + 32, :] = x32[32 * hl:32 * hl + 32]

        def b_prep2(jd, e, cc, gate):
            y = jnp.concatenate(
                [tb[e, pl.ds(4 * cc + dl + 33 * 8 * g, 8, stride=33), :] for dl in range(4) for g in range(4)],
                axis=0)
            row = pl.multiple_of((jd & 1) * 256, 256) + e * 128
            wb[(jd >> 1) * 8 + cc, pl.ds(row, 128), :] = gated(y, gate).T

        def wob_prep1(js, g, gate):
            v = gated(pltpu.bitcast(wobst[js, g * 512:(g + 1) * 512, :], U32), gate)
            for hp in range(8):
                tob[g, 33 * hp:33 * hp + 32, :] = v[32 * hp:32 * hp + 32]

        def wob_prep2(jd, g, gate):
            for dp in range(16):
                z = gate()
                lo, hi = _lo_hi(tob[g, pl.ds(dp, 8, stride=33), :] | z, tob[g, pl.ds(16 + dp, 8, stride=33), :] | z)
                wobp[jd, (2 * dp) * 16 + 8 * g:(2 * dp) * 16 + 8 * g + 8, :] = lo
                wobp[jd, (2 * dp + 1) * 16 + 8 * g:(2 * dp + 1) * 16 + 8 * g + 8, :] = hi

        def woa_prep(js, jd, q, gate):
            row = pl.multiple_of(jd * 256, 256)
            woa[q, pl.ds(row, 256), :] = gated(pltpu.bitcast(woast[js, :, q * 128:(q + 1) * 128], U32), gate)

        nblk = D // 16
        ntw = tw.shape[0]

        def run_jobs(ticks, jobs, free=0):
            total = sum(n for n, _ in jobs)
            z = zero[...]
            cache = {}
            cnt = [0]

            def gate():
                k = (cnt[0] - free) * len(ticks) // (total - free)
                cnt[0] += 1
                if k < 0:
                    return z
                if k not in cache:
                    cache[k] = pltpu.bitcast(ticks[k], U32) & z
                return cache[k]

            for _, fn in jobs:
                fn(gate=gate)

        def relayout_jobs(c, base, b0=0, b1=nblk, r0=0):
            jobs = []
            for blk in range(b0, b1 + 1):
                if blk < b1:
                    jobs.append((8, functools.partial(relayout1, c, blk, blk % ntw, r0)))
                if blk > b0:
                    jobs.append((4, functools.partial(relayout2, base, blk - 1, (blk - 1) % ntw, r0)))
            return jobs

        def interleave(*lists):
            items = []
            for l in lists:
                items += [((i + 0.5) / len(l), x) for i, x in enumerate(l)]
            items.sort(key=lambda z: z[0])
            return [x for _, x in items]

        def trim(ticks, units):
            return ticks[:len(ticks) - units * (MB // 8 // CFG['tstep'])]

        def relayout(c, base, b0, b1):
            for blk in range(b0, b1):
                relayout1(c, blk, blk % ntw)
                relayout2(base, blk, blk % ntw)

        nb = KP // 16
        KA = CFG['ka']
        w0_copy(0).wait()
        relayout(0, 0, 0, nb)
        x_copy(0).wait()
        def piece(q, carry):
            w0_copy(q + 1).wait()
            x_copy(q + 1).wait()
            wrow = pl.multiple_of(q * (KP // 2), KP // 2)
            ticks = run_pieces(q, wrow, KA, 32)
            run_jobs(trim(ticks, CFG['e0']), relayout_jobs(0, 0, nb, 2 * nb, wrow), CFG['f0'])
            run_pieces(q + 1, wrow + KP // 2, 0, KA)
            return carry

        run_pieces(0, 0, 0, KA, first=True)
        lax.fori_loop(0, W0P - 1, piece, 0)
        w1_copy(0).wait()
        ticks = run_pieces(W0P - 1, (W0P - 1) * KP // 2, KA, 32)
        run_jobs(trim(ticks, CFG['e0b']), relayout_jobs(1, 8, 0, W1A // 16), CFG['f1'])
        w1_copy(1).wait()

        K1 = CFG['k1']

        def chunk(c, carry):
            w_copy(c + 1).wait()

            @pl.when(c >= OA0)
            def _():
                woa_copy(c - OA0).wait()
                wob_copy(c - OA0).wait()

            @pl.when(c >= OB0)
            def _():
                b_copy(c - OB0).wait()

            c8 = c * 8
            ticks = run_units(c, c8, K1, 32)
            run_jobs(trim(ticks, CFG['e1']), relayout_jobs(c + 1, c8 + 8))
            ticks = run_units(c + 1, c8 + 8, 0, K1)
            ja = jnp.maximum(c - OA0, 0)
            jb = jnp.maximum(c - OB0, 0)
            sa = jnp.where(c >= OA0, ja, 8)
            sb = jnp.where(c >= OB0, jb, 6)
            jobs = interleave(
                [(32, functools.partial(woa_prep, sa, ja, q)) for q in range(8)],
                [(32, functools.partial(wob_prep1, sa, g)) for g in range(2)]
                + [(16, functools.partial(wob_prep2, ja, g)) for g in range(2)],
                [(16, functools.partial(f, j_, e, cc))
                 for e in range(2) for f, j_ in ((b_prep1, sb), (b_prep2, jb)) for cc in range(8)])
            run_jobs(trim(ticks, CFG['e3']), jobs)
            return carry

        relayout(1, 8, W1A // 16, nblk)
        ticks = run_units(1, 8, 0, K1)
        run_jobs(trim(ticks, 2), [(16, functools.partial(finish_chunk0, u)) for u in range(32)])
        lax.fori_loop(1, NCH - 1, chunk, 0)
        run_units(NCH - 1, (NCH - 1) * 8, K1, 32)

    vm = pltpu.VMEM
    (pl.run_scoped if not CFG['only2'] else (lambda *a: None))(
        phase1,
        vm((W0P, PRE, KP), BF),
        vm((NCH, D, 8, E), BF),
        vm((9, 512, D), BF),
        vm((7, 512, D), BF),
        vm((9, D, 128), BF),
        vm((CFG['ntw'], CFG['twp'], 128), U32),
        vm((2, 33 * H + 40, 128), U32),
        vm((2, 33 * 8 + 32, 128), U32),
        vm((8, PRE, E), F32),
    )
    mem_copy.wait()
    xb_copy.wait()
    xar_copy.wait()

    def wa_ref(t, h):
        return pltpu.bitcast(wa[t * H + h], BF)

    a_scale = E ** -0.5
    b_scale = (D // H) ** -0.5

    def phase23(ola, olb, outa, outb):
        def ol_ref(h):
            return (ola, h) if h < SPLIT else (olb, h - SPLIT)

        def out_copy(buf, row, c0, nc, half):
            return pltpu.make_async_copy(
                buf.at[pl.ds(row, BM), pl.ds(c0, nc)], out.at[pl.ds(row, BM), pl.ds(half * D + c0, nc)],
                sem_out.at[half])

        def b_out(row):
            o = ob[...]
            for j in range(8):
                outb[pl.ds(row, BM), j * 128:(j + 1) * 128] = _dot(o, pltpu.bitcast(wobp[j], BF)).astype(BF)
                if (j + 1) % CFG['pcol'] == 0:
                    out_copy(outb, row, (j + 1 - CFG['pcol']) * 128, CFG['pcol'] * 128, 1).start()

        def make_gate(tk, n):
            cnt = [0]
            cache = {}

            def gate(x):
                if not tk:
                    return x
                k = cnt[0] * len(tk) // n
                cnt[0] += 1
                if k not in cache:
                    cache[k] = pltpu.bitcast(tk[k], U32) & zero[...]
                return pltpu.bitcast(pltpu.bitcast(x, U32) | cache[k], F32)
            return gate

        def b_qk(row, i, gate):
            q = [qb[cc, 8 * i:8 * i + 8, :] for cc in range(8)]
            pos = row + 8 * i + lax.broadcasted_iota(jnp.int32, (8, 128), 0)
            logits = []
            for w in range(WIN):
                lo = HIST + 8 * i - DIL * w
                t = None
                for cc in range(8):
                    x = gate(kb[cc, lo:lo + 8, :]) * q[cc]
                    t = x if t is None else t + x
                t = t + pltpu.roll(t, 64, 1)
                t = t + pltpu.roll(t, 32, 1)
                if 8 * i < DIL * w:
                    t = jnp.where(pos >= DIL * w, t, NEG)
                logits.append(t)
            m = functools.reduce(jnp.maximum, logits)
            return logits, m

        def b_sm(i, logits, m, gate):
            ex = [jnp.exp(gate(t) - m) for t in logits]
            r = _rcp(functools.reduce(lambda a, b: a + b, ex))
            for w in range(WIN):
                pb[w, 8 * i:8 * i + 8, :] = gate(ex[w]) * r

        def b_pv(gate):
            for i in range(BM // 8):
                p = [pb[w, 8 * i:8 * i + 8, :] for w in range(WIN)]
                for cc in range(8):
                    t = None
                    for w in range(WIN):
                        lo = HIST + 8 * i - DIL * w
                        x = gate(vb[cc, lo:lo + 8, :]) * p[w]
                        t = x if t is None else t + x
                    ob[8 * i:8 * i + 8, cc * 128:(cc + 1) * 128] = t.astype(BF)

        def step(s, u):
            brow = pl.multiple_of((s - u % 2) * SEG, BM)
            xrows = xbb[pl.ds(brow, BM), :]
            nv = CFG['nv']
            if u % 2 == 0:
                for cc in range(8):
                    kb[cc, 0:HIST, :] = kb[cc, BM:BM + HIST, :]
                    vb[cc, 0:HIST, :] = vb[cc, BM:BM + HIST, :]
                for cc in range(8):
                    qb[cc] = _dot(xrows, pltpu.bitcast(wb[cc], BF)) * b_scale
                    kb[cc, HIST:HIST + BM, :] = _dot(xrows, pltpu.bitcast(wb[8 + cc], BF))
            ticks = []
            for cc in (range(nv) if u % 2 == 0 else range(nv, 8)):
                r = _dot(xrows, pltpu.bitcast(wb[16 + cc], BF))
                vb[cc, HIST:HIST + BM, :] = r
                ticks.extend(r[8 * i:8 * i + 8] for i in range(BM // 8))
            groups = range(CFG['ng']) if u % 2 == 0 else range(CFG['ng'], BM // 8)
            lm = {}

            lhs = jnp.concatenate([memb[...], xar[pl.ds(pl.multiple_of(s * XR, 8), XR), :]], axis=0)
            slot = _divmod(s, NS)[1] * NG
            offs = [slot]
            for i in range(3):
                g = PRE // 8 + 3 * s + i
                offs.append(_divmod(g >> 2, NS)[1] * NG + 1 + (g & 3))
            oofs = (0, 8, 16, 24, 40) if u % 2 == 0 else (32, 48, 56, 64, 72)
            nrow = 32 if u % 2 == 0 else 48

            def proj(h, t, n):
                p = h // 2
                ring = rings[p % NB]
                ro = (p // NB) * 16 + (h % 2) * 8
                r32 = _dot(lhs, wa_ref(t, h))
                for k, i in enumerate(groups):
                    if CFG['m0'] + CFG['mstep'] * k == n:
                        d0 = pltpu.bitcast(lm[i][1], U32) & zero[...]
                        a0 = pltpu.bitcast(pltpu.bitcast(r32[0:8], U32) | d0, F32)
                        r32 = jnp.concatenate([a0, r32[8:]], axis=0)
                ticks.extend(r32[8 * i:8 * i + 8] for i in range(4))
                if n == CFG['qn']:
                    gate = make_gate(list(ticks), 64 * len(groups))
                    for i in groups:
                        lm[i] = b_qk(brow, i, gate)
                for k, i in enumerate(groups):
                    if CFG['m0'] + CFG['mstep'] * k + CFG['sspan'] == n:
                        b_sm(i, lm[i][0], lm[i][1], make_gate(ticks[-4 * CFG['sspan']:], 16))
                r = r32.astype(BF)
                for i in range(4):
                    ring[t, offs[i], ro:ro + 8, :] = r[8 * i:8 * i + 8]

            probs = {}

            def pair(t, p):
                ro = (p // NB) * 16
                return rings[p % NB][t, pl.ds(slot, NG), ro:ro + 16, :].reshape(PAIR, E)

            def att1(p, dead=None):
                q = pair(0, p)
                k = pair(1, p)
                sc = lax.dot_general(q, k, (((1,), (1,)), ((), ())), preferred_element_type=F32)
                if not CFG['exp2']:
                    sc = sc * a_scale
                fl = fill[...]
                if dead is not None:
                    d0 = (pltpu.bitcast(dead, U32) & zero[...])[:, :PAIR]
                    f0 = pltpu.bitcast(pltpu.bitcast(fl[0:8], U32) | d0, F32)
                    fl = jnp.concatenate([f0, fl[8:]], axis=0)
                sc = jnp.where(fl == 0.0, sc, fl)
                if CFG['exp2']:
                    e = jnp.exp2((sc - jnp.max(sc, axis=1, keepdims=True)) * (a_scale * LOG2E))
                else:
                    e = jnp.exp(sc - jnp.max(sc, axis=1, keepdims=True))
                probs[p] = (e * _rcp(jnp.sum(e, axis=1, keepdims=True))).astype(BF)

            def att2(p):
                o = _dot(probs.pop(p), pair(2, p)).astype(BF)
                for i in range(NG):
                    for hh in range(2):
                        ol, hi = ol_ref(2 * p + hh)
                        ol[oofs[i]:oofs[i] + 8, hi * E:(hi + 1) * E] = o[16 * i + 8 * hh:16 * i + 8 * hh + 8]

            def do(ev):
                kind, p = ev
                if kind == 1:
                    att1(p)
                else:
                    att2(p)

            events = {}
            for p in range(H // 2):
                n1 = 6 * p + 5 + CFG['d1']
                n2 = n1 + CFG['d2']
                events.setdefault(n1, []).append((1, p))
                events.setdefault(n2, []).append((2, p))
            order = CFG['order']
            n = 0
            for p in range(H // 2):
                for hh, t in order:
                    proj(2 * p + hh, t, n)
                    for ev in events.get(n, []):
                        do(ev)
                    n += 1
            oticks = []
            ks = CFG['ks'] if u % 2 == 1 else 1
            kw = SPLIT * 128 // ks
            l1 = ola[oofs[0]:oofs[0] + nrow, :]
            for j in range(8):
                r = None
                for k in range(ks):
                    x = _dot(l1[:, k * kw:(k + 1) * kw], pltpu.bitcast(woa[j, k * kw // 2:(k + 1) * kw // 2, :], BF))
                    r = x if r is None else r + x
                    oticks.extend(r[8 * i:8 * i + 8] for i in range(nrow // 8))
                acc[j, 0:nrow, :] = r
                for n in range(3 * H + 3 * j, 3 * H + 3 * j + 3):
                    for ev in events.get(n, []):
                        do(ev)
            assert max(events) < 3 * H + 24
            assert all(p >= SPLIT // 2 for n in events if n >= 3 * H for k, p in events[n] if k == 2)
            l2 = olb[oofs[0]:oofs[0] + nrow, :]
            orow = pl.multiple_of(s * SEG - (u % 2) * 8, 8)
            for j in range(8):
                r = acc[j, 0:nrow, :] + _dot(l2, pltpu.bitcast(woa[j, SPLIT * 64:, :], BF))
                if j < CFG['pvj']:
                    oticks.extend(r[8 * i:8 * i + 8] for i in range(nrow // 8))
                res = r.astype(BF)
                memb[:, j * 128:(j + 1) * 128] = res[0:MEM]
                outa[pl.ds(orow, nrow - MEM), j * 128:(j + 1) * 128] = res[MEM:]
            if u % 2 == 1:
                out_copy(outa, brow, 0, D, 0).start()
                b_pv(make_gate(oticks[CFG['pv0']:], 8 * BM))
                b_out(brow)

        def steps(i, carry):
            for u in range(U):
                step(i * U + u, u)
            return carry

        lax.fori_loop(0, NSEG // U, steps, 0)

        pltpu.make_async_copy(outb, out.at[:, pl.ds(D, D)], sem_out.at[1]).wait()
        pltpu.make_async_copy(outa, out.at[:, pl.ds(0, D)], sem_out.at[0]).wait()

    pl.run_scoped(
        phase23,
        vm((OLROWS, SPLIT * E), BF),
        vm((OLROWS, (H - SPLIT) * E), BF),
        vm((S, D), BF),
        vm((S, D), BF),
    )


@jax.jit
def _run(A_x, A_mem0, A_Wq, A_Wk, A_Wv, A_Wo, B_x, B_wqkv, B_wo):
    assert A_x.shape == (1, S, D) and A_mem0.shape == (1, MEM, D)
    assert A_Wq.shape == (D, H, E) and A_Wo.shape == (H, E, D)
    assert B_x.shape == (1, S, D) and B_wqkv.shape == (D, 3 * D) and B_wo.shape == (D, D)
    vm = pltpu.VMEM
    dma = pltpu.SemaphoreType.DMA
    scratch = [
        vm((NSEG * XR, D), BF),
        vm((S, D), BF),
        vm((MEM, D), BF),
        vm((3 * H, D // 2, E), U32),
        vm((8, H * E // 2, 128), U32),
        vm((24, D // 2, 128), U32),
        vm((8, D // 2, 128), U32),
    ] + [vm((3, NS * NG, 64, E), BF)] * NB + [
        vm((8, 48, 128), F32),
        vm((PAIR, PAIR), F32),
        vm((8, BM, 128), F32),
        vm((8, HIST + BM, 128), F32),
        vm((8, HIST + BM, 128), F32),
        vm((WIN, BM, 128), F32),
        vm((BM, D), BF),
        vm((8, 128), U32),
        dma((sum(SEM_N),)), dma((2,)),
    ]
    out = pl.pallas_call(
        _kernel,
        out_shape=jax.ShapeDtypeStruct((S, 2 * D), BF),
        in_specs=[pl.BlockSpec(memory_space=pl.ANY)] * 9,
        out_specs=pl.BlockSpec(memory_space=pl.ANY),
        scratch_shapes=scratch,
        compiler_params=pltpu.CompilerParams(vmem_limit_bytes=120 * 1024 * 1024,
                                             disable_bounds_checks=CFG['nobc'],
                                             disable_semaphore_checks=CFG['nosc']),
    )(A_x.reshape(S, D), A_mem0.reshape(MEM, D), A_Wq, A_Wk, A_Wv, A_Wo.reshape(8, 512, D),
      B_x.reshape(S, D), B_wqkv, B_wo)
    return out.reshape(1, S, 2 * D)


def pallas_concat_heads__memory_aug_recurrent_mem_tr__sliding_local_dilated__prompt_kernel(
    A_x, A_mem0, A_Wq, A_Wk, A_Wv, A_Wo, A_seg_len, B_x, B_wqkv, B_wo):
    if isinstance(A_seg_len, int):
        assert A_seg_len == SEG
    return _run(A_x, A_mem0, A_Wq, A_Wk, A_Wv, A_Wo, B_x, B_wqkv, B_wo)
```

```python
import functools

import jax
import jax.numpy as jnp
from jax import lax
import jax.experimental.pallas as pl
import jax.experimental.pallas.tpu as pltpu

BF = jnp.bfloat16
F32 = jnp.float32
U32 = jnp.uint32

S = 2048
D = 1024
H = 32
E = 128
MEM = 8
SEG = 32
L = MEM + SEG
NG = L // 8
NSEG = S // SEG
WIN = 8
DIL = 2
NEG = -1000000000.0
LOG2E = 1.4426950408889634

XR = 24
PRE = S - NSEG * XR
NS = 17
NB = 4
PAIR = 2 * L
SPLIT = 24
U = 4
BM = 2 * SEG
HIST = 16

NCH = 12
MB = 128
NKP = 4
KP = D // NKP
KA = 20
K1 = 16
W1A = 640
OA0 = NCH - 1 - 8
OB0 = NCH - 1 - 6
NTW = 4

SEM_MEM, SEM_X, SEM_W0, SEM_W, SEM_B, SEM_WOB, SEM_WOA, SEM_XA, SEM_XB, NSEM = (
    0, 1, 5, 9, 21, 27, 35, 43, 44, 45)


def _rcp(d):
    r = pl.reciprocal(d, approx=True)
    return r * (2.0 - d * r)


def _dot(a, b):
    return jnp.dot(a, b, preferred_element_type=F32)


def _unpack(w):
    return pltpu.bitcast(w, BF)


def _mod(x, d):
    m = 65536 // d + 1
    assert all((v * m) >> 16 == v // d for v in range(1024))
    return x - lax.shift_right_logical(x * m, 16) * d


def _lo_hi(a, b):
    lo = (a & U32(0xFFFF)) | (b << 16)
    hi = (a >> 16) | (b & U32(0xFFFF0000))
    return lo, hi


def _vregs(x):
    return [x[i:i + 8] for i in range(0, x.shape[0], 8)]


def _kernel(xa, mem0, wq, wk, wv, wo, xb, wqkv, wob, out,
            xar, xbb, memb, wa, woa, wb, wobp,
            r0, r1, r2, r3, acc, fill, qb, kb, vb, pb, ob, zero,
            sem, sem_out):
    rings = (r0, r1, r2, r3)
    wsrc = (wq, wk, wv)
    a_scale = E ** -0.5
    b_scale = (D // H) ** -0.5

    xar_copy = pltpu.make_async_copy(xa.at[pl.ds(PRE, NSEG * XR), :], xar, sem.at[SEM_XA])
    xb_copy = pltpu.make_async_copy(xb, xbb, sem.at[SEM_XB])
    mem_copy = pltpu.make_async_copy(mem0, memb, sem.at[SEM_MEM])

    def phase1(xpre, wst, woast, bst, wobst, tw, tb, tob, pacc):
        def st(i):
            return i if isinstance(i, int) else 0

        def w_copy(c):
            return pltpu.make_async_copy(
                wsrc[st(c) // 4].at[:, pl.ds((st(c) % 4) * 8, 8), :], wst.at[c], sem.at[SEM_W + c])

        def w0_copy(q):
            lo = q * KP if isinstance(q, int) else pl.multiple_of(q * KP, KP)
            return pltpu.make_async_copy(
                wq.at[pl.ds(st(q) * KP, KP), pl.ds(0, 8), :], wst.at[0, pl.ds(lo, KP)], sem.at[SEM_W0 + q])

        def w1_copy(q):
            lo, n = ((0, W1A), (W1A, D - W1A))[q]
            return pltpu.make_async_copy(
                wq.at[pl.ds(lo, n), pl.ds(8, 8), :], wst.at[1, pl.ds(lo, n)], sem.at[SEM_W + q])

        def x_copy(q):
            return pltpu.make_async_copy(
                xa.at[pl.ds(0, PRE), pl.ds(st(q) * KP, KP)], xpre.at[q], sem.at[SEM_X + q])

        def b_copy(j):
            return pltpu.make_async_copy(
                wqkv.at[pl.ds((st(j) % 2) * 512, 512), pl.ds((st(j) // 2) * D, D)], bst.at[j],
                sem.at[SEM_B + j])

        def wob_copy(j):
            return pltpu.make_async_copy(
                wob.at[:, pl.ds(st(j) * 128, 128)], wobst.at[j], sem.at[SEM_WOB + j])

        def woa_copy(j):
            return pltpu.make_async_copy(wo.at[st(j)], woast.at[j], sem.at[SEM_WOA + j])

        for q in range(NKP):
            w0_copy(q).start()
            x_copy(q).start()
        w1_copy(0).start()
        w1_copy(1).start()
        for c in range(1, NCH - 1):
            w_copy(c + 1).start()
            if c >= OA0:
                woa_copy(c - OA0).start()
                wob_copy(c - OA0).start()
            if c >= OB0:
                b_copy(c - OB0).start()
        mem_copy.start()
        xb_copy.start()
        xar_copy.start()

        def zero_fill(i, carry):
            r = pl.multiple_of(i * 32, 32)
            woast[8, pl.ds(r, 32), :] = jnp.zeros((32, D), BF)
            bst[6, pl.ds(r, 32), :] = jnp.zeros((32, D), BF)
            wobst[8, pl.ds(2 * r, 64), :] = jnp.zeros((64, 128), BF)
            return carry

        lax.fori_loop(0, 16, zero_fill, 0)

        ri = lax.broadcasted_iota(jnp.int32, (PAIR, PAIR), 0)
        ci = lax.broadcasted_iota(jnp.int32, (PAIR, PAIR), 1)
        rb = (ri >> 3) & 1
        cb = (ci >> 3) & 1
        rl = ((ri >> 4) << 3) | (ri & 7)
        cl = ((ci >> 4) << 3) | (ci & 7)
        allowed = (rl < MEM) | (rl >= cl)
        fill[...] = jnp.where(rb == cb, jnp.where(allowed, 0.0, NEG / a_scale), -jnp.inf).astype(F32)
        kb[...] = jnp.zeros(kb.shape, F32)
        vb[...] = jnp.zeros(vb.shape, F32)
        zero[...] = jnp.zeros(zero.shape, U32)
        for u in range(KA, 32):
            pacc[u % 8, (u // 8) * MB:(u // 8 + 1) * MB, :] = jnp.zeros((MB, E), F32)

        def gated(x, gate):
            return jnp.concatenate([v | gate() for v in _vregs(x)], axis=0)

        def relayout1(c, blk, row0=0, gate=None):
            v = wst[c, pl.ds(2 * row0 + blk * 16, 16)]
            v = pltpu.bitcast(v.reshape(128, 128), U32)
            for dp in range(8):
                x = v[8 * dp:8 * dp + 8]
                tw[blk % NTW, 9 * dp:9 * dp + 8, :] = x if gate is None else x | gate()

        def relayout2(base, blk, row0=0, gate=None):
            row = row0 + blk * 8
            for j in range(4):
                a = tw[blk % NTW, pl.ds(j, 8, stride=9), :]
                b = tw[blk % NTW, pl.ds(4 + j, 8, stride=9), :]
                if gate is not None:
                    g = gate()
                    a, b = a | g, b | g
                lo, hi = _lo_hi(a, b)
                wa[base + 2 * j, pl.ds(row, 8), :] = lo
                wa[base + 2 * j + 1, pl.ds(row, 8), :] = hi

        def relayout(c, base, b0, b1):
            for blk in range(b0, b1):
                relayout1(c, blk)
                relayout2(base, blk)

        def relayout_jobs(c, base, b0=0, b1=D // 16, row0=0):
            jobs = []
            for blk in range(b0, b1 + 1):
                if blk < b1:
                    jobs.append((8, functools.partial(relayout1, c, blk, row0)))
                if blk > b0:
                    jobs.append((4, functools.partial(relayout2, base, blk - 1, row0)))
            return jobs

        def b_prep1(src, e, cc, gate):
            x = pltpu.bitcast(bst[src, e * 256:(e + 1) * 256, cc * 128:(cc + 1) * 128], U32)
            x = gated(x, gate).T
            for hl in range(4):
                h = 4 * cc + hl
                tb[e, 33 * h:33 * h + 32, :] = x[32 * hl:32 * hl + 32]

        def b_prep2(j, e, cc, gate):
            y = jnp.concatenate(
                [tb[e, pl.ds(4 * cc + dl + 33 * 8 * g, 8, stride=33), :] for dl in range(4) for g in range(4)],
                axis=0)
            row = pl.multiple_of((j & 1) * 256, 256) + e * 128
            wb[(j >> 1) * 8 + cc, pl.ds(row, 128), :] = gated(y, gate).T

        def wob_prep1(src, g, gate):
            v = pltpu.bitcast(wobst[src, g * 512:(g + 1) * 512, :], U32)
            v = gated(v, gate)
            for hp in range(8):
                tob[g, 33 * hp:33 * hp + 32, :] = v[32 * hp:32 * hp + 32]

        def wob_prep2(j, g, gate):
            for dp in range(16):
                z = gate()
                lo, hi = _lo_hi(tob[g, pl.ds(dp, 8, stride=33), :] | z,
                                tob[g, pl.ds(16 + dp, 8, stride=33), :] | z)
                wobp[j, (2 * dp) * 16 + 8 * g:(2 * dp) * 16 + 8 * g + 8, :] = lo
                wobp[j, (2 * dp + 1) * 16 + 8 * g:(2 * dp + 1) * 16 + 8 * g + 8, :] = hi

        def woa_prep(src, j, q, gate):
            v = pltpu.bitcast(woast[src, :, q * 128:(q + 1) * 128], U32)
            woa[q, pl.ds(pl.multiple_of(j * 256, 256), 256), :] = gated(v, gate)

        def ring_store(c, hh, mb, r32):
            t = c >> 2
            g = c & 3
            r = r32.astype(BF)
            ring = rings[hh // 2]
            off = (g * 16 if isinstance(g, int) else pl.multiple_of(g * 16, 16)) + (hh % 2) * 8
            for k in range(MB // 8):
                plane = mb * (MB // SEG * NG) + (k // 4) * NG + 1 + k % 4
                ring[t, plane, pl.ds(off, 8), :] = r[8 * k:8 * k + 8]

        def run_units(c, base, u0, u1):
            ticks = []
            for u in range(u0, u1):
                hh, mb = u % 8, u // 8
                lhs = jnp.concatenate([xpre[q, mb * MB:(mb + 1) * MB, :] for q in range(NKP)], axis=1)
                r32 = _dot(lhs, _unpack(wa[base + hh]))
                ring_store(c, hh, mb, r32)
                ticks += _vregs(r32)
            return ticks

        def run_pieces(q, wrow, u0, u1, first=False):
            ticks = []
            for u in range(u0, u1):
                hh, mb = u % 8, u // 8
                rows = slice(mb * MB, (mb + 1) * MB)
                r32 = _dot(xpre[q, rows, :], _unpack(wa[hh, pl.ds(wrow, KP // 2), :]))
                if not first:
                    r32 = r32 + pacc[hh, rows, :]
                pacc[hh, rows, :] = r32
                ticks += _vregs(r32)
            return ticks

        def finish_chunk0(u, gate):
            hh, mb = u % 8, u // 8
            r = pltpu.bitcast(pacc[hh, mb * MB:(mb + 1) * MB, :], U32)
            ring_store(0, hh, mb, pltpu.bitcast(gated(r, gate), F32))

        def run_jobs(ticks, spare, jobs, free=0):
            ticks = ticks[:len(ticks) - spare * (MB // 8)]
            total = sum(n for n, _ in jobs)
            z = zero[...]
            cache = {}
            cnt = [0]

            def gate():
                k = (cnt[0] - free) * len(ticks) // (total - free)
                cnt[0] += 1
                if k < 0:
                    return z
                if k not in cache:
                    cache[k] = pltpu.bitcast(ticks[k], U32) & z
                return cache[k]

            for _, fn in jobs:
                fn(gate=gate)

        def interleave(*lists):
            items = []
            for l in lists:
                items += [((i + 0.5) / len(l), x) for i, x in enumerate(l)]
            items.sort(key=lambda z: z[0])
            return [x for _, x in items]

        nb = KP // 16

        def piece(q, carry):
            w0_copy(q + 1).wait()
            x_copy(q + 1).wait()
            wrow = pl.multiple_of(q * (KP // 2), KP // 2)
            ticks = run_pieces(q, wrow, KA, 32)
            run_jobs(ticks, 4, relayout_jobs(0, 0, nb, 2 * nb, wrow))
            run_pieces(q + 1, wrow + KP // 2, 0, KA)
            return carry

        def chunk(c, carry):
            w_copy(c + 1).wait()

            @pl.when(c >= OA0)
            def _():
                woa_copy(c - OA0).wait()
                wob_copy(c - OA0).wait()

            @pl.when(c >= OB0)
            def _():
                b_copy(c - OB0).wait()

            c8 = c * 8
            ticks = run_units(c, c8, K1, 32)
            run_jobs(ticks, 2, relayout_jobs(c + 1, c8 + 8))
            ticks = run_units(c + 1, c8 + 8, 0, K1)
            ja = jnp.maximum(c - OA0, 0)
            jb = jnp.maximum(c - OB0, 0)
            sa = jnp.where(c >= OA0, ja, 8)
            sb = jnp.where(c >= OB0, jb, 6)
            jobs = interleave(
                [(32, functools.partial(woa_prep, sa, ja, q)) for q in range(8)],
                [(32, functools.partial(wob_prep1, sa, g)) for g in range(2)]
                + [(16, functools.partial(wob_prep2, ja, g)) for g in range(2)],
                [(16, functools.partial(f, j, e, cc))
                 for e in range(2) for f, j in ((b_prep1, sb), (b_prep2, jb)) for cc in range(8)])
            run_jobs(ticks, 2, jobs)
            return carry

        w0_copy(0).wait()
        relayout(0, 0, 0, nb)
        x_copy(0).wait()
        run_pieces(0, 0, 0, KA, first=True)
        lax.fori_loop(0, NKP - 1, piece, 0)
        w1_copy(0).wait()
        ticks = run_pieces(NKP - 1, (NKP - 1) * KP // 2, KA, 32)
        run_jobs(ticks, 0, relayout_jobs(1, 8, 0, W1A // 16), free=100)
        w1_copy(1).wait()
        relayout(1, 8, W1A // 16, D // 16)
        ticks = run_units(1, 8, 0, K1)
        run_jobs(ticks, 2, [(16, functools.partial(finish_chunk0, u)) for u in range(32)])
        lax.fori_loop(1, NCH - 1, chunk, 0)
        run_units(NCH - 1, (NCH - 1) * 8, K1, 32)

    vm = pltpu.VMEM
    pl.run_scoped(
        phase1,
        vm((NKP, PRE, KP), BF),
        vm((NCH, D, 8, E), BF),
        vm((9, 512, D), BF),
        vm((7, 512, D), BF),
        vm((9, D, 128), BF),
        vm((NTW, 80, 128), U32),
        vm((2, 33 * H + 40, 128), U32),
        vm((2, 33 * 8 + 32, 128), U32),
        vm((8, PRE, E), F32),
    )
    mem_copy.wait()
    xb_copy.wait()
    xar_copy.wait()

    def phase2(ola, olb, outa, outb):
        def out_copy(buf, row, c0, nc, half):
            return pltpu.make_async_copy(
                buf.at[pl.ds(row, BM), pl.ds(c0, nc)], out.at[pl.ds(row, BM), pl.ds(half * D + c0, nc)],
                sem_out.at[half])

        def tie(x, y):
            return pltpu.bitcast(pltpu.bitcast(x, U32) | y, F32)

        def nil(y):
            return pltpu.bitcast(y, U32) & zero[...]

        def make_gate(ticks, n):
            cnt = [0]
            cache = {}

            def gate(x):
                k = cnt[0] * len(ticks) // n
                cnt[0] += 1
                if k not in cache:
                    cache[k] = nil(ticks[k])
                return tie(x, cache[k])
            return gate

        def b_logits(row, i, gate):
            q = [qb[cc, 8 * i:8 * i + 8, :] for cc in range(8)]
            pos = row + 8 * i + lax.broadcasted_iota(jnp.int32, (8, 128), 0)
            logits = []
            for w in range(WIN):
                lo = HIST + 8 * i - DIL * w
                t = None
                for cc in range(8):
                    x = gate(kb[cc, lo:lo + 8, :]) * q[cc]
                    t = x if t is None else t + x
                t = t + pltpu.roll(t, 64, 1)
                t = t + pltpu.roll(t, 32, 1)
                if 8 * i < DIL * w:
                    t = jnp.where(pos >= DIL * w, t, NEG)
                logits.append(t)
            return logits, functools.reduce(jnp.maximum, logits)

        def b_softmax(i, logits, m, gate):
            ex = [jnp.exp(gate(t) - m) for t in logits]
            r = _rcp(functools.reduce(lambda a, b: a + b, ex))
            for w in range(WIN):
                pb[w, 8 * i:8 * i + 8, :] = gate(ex[w]) * r

        def b_values(gate):
            for i in range(BM // 8):
                p = [pb[w, 8 * i:8 * i + 8, :] for w in range(WIN)]
                for cc in range(8):
                    t = None
                    for w in range(WIN):
                        lo = HIST + 8 * i - DIL * w
                        x = gate(vb[cc, lo:lo + 8, :]) * p[w]
                        t = x if t is None else t + x
                    ob[8 * i:8 * i + 8, cc * 128:(cc + 1) * 128] = t.astype(BF)

        def b_out(row):
            o = ob[...]
            for j in range(8):
                outb[pl.ds(row, BM), j * 128:(j + 1) * 128] = _dot(o, _unpack(wobp[j])).astype(BF)
                if j % 4 == 3:
                    out_copy(outb, row, (j - 3) * 128, 512, 1).start()

        def step(s, odd):
            brow = pl.multiple_of((s - odd) * SEG, BM)
            xrows = xbb[pl.ds(brow, BM), :]
            if not odd:
                for cc in range(8):
                    kb[cc, 0:HIST, :] = kb[cc, BM:BM + HIST, :]
                    vb[cc, 0:HIST, :] = vb[cc, BM:BM + HIST, :]
                for cc in range(8):
                    qb[cc] = _dot(xrows, _unpack(wb[cc])) * b_scale
                    kb[cc, HIST:HIST + BM, :] = _dot(xrows, _unpack(wb[8 + cc]))
            ticks = []
            for cc in range(4 * odd, 4 * odd + 4):
                r = _dot(xrows, _unpack(wb[16 + cc]))
                vb[cc, HIST:HIST + BM, :] = r
                ticks.extend(_vregs(r))
            groups = range(4 * odd, 4 * odd + 4)
            lm = {}

            lhs = jnp.concatenate([memb[...], xar[pl.ds(pl.multiple_of(s * XR, 8), XR), :]], axis=0)
            slot = _mod(s, NS) * NG
            planes = [slot]
            for i in range(3):
                g = PRE // 8 + 3 * s + i
                planes.append(_mod(g >> 2, NS) * NG + 1 + (g & 3))
            orows = (32, 48, 56, 64, 72) if odd else (0, 8, 16, 24, 40)
            nrow = 48 if odd else 32

            def proj(h, t):
                n = 3 * h + t
                p = h // 2
                r32 = _dot(lhs, _unpack(wa[t * H + h]))
                for k, i in enumerate(groups):
                    if n == 5 + 2 * k:
                        r32 = jnp.concatenate([tie(r32[0:8], nil(lm[i][1])), r32[8:]], axis=0)
                ticks.extend(_vregs(r32))
                if n == 2:
                    gate = make_gate(list(ticks), 64 * len(groups))
                    for i in groups:
                        lm[i] = b_logits(brow, i, gate)
                for k, i in enumerate(groups):
                    if n == 7 + 2 * k:
                        b_softmax(i, lm[i][0], lm[i][1], make_gate(ticks[-8:], 16))
                r = r32.astype(BF)
                ro = (p // NB) * 16 + (h % 2) * 8
                for i in range(4):
                    rings[p % NB][t, planes[i], ro:ro + 8, :] = r[8 * i:8 * i + 8]

            probs = {}

            def pair(t, p):
                ro = (p // NB) * 16
                return rings[p % NB][t, pl.ds(slot, NG), ro:ro + 16, :].reshape(PAIR, E)

            def scores(p):
                sc = lax.dot_general(pair(0, p), pair(1, p), (((1,), (1,)), ((), ())),
                                     preferred_element_type=F32)
                fl = fill[...]
                sc = jnp.where(fl == 0.0, sc, fl)
                e = jnp.exp2((sc - jnp.max(sc, axis=1, keepdims=True)) * (a_scale * LOG2E))
                probs[p] = (e * _rcp(jnp.sum(e, axis=1, keepdims=True))).astype(BF)

            def values(p):
                o = _dot(probs.pop(p), pair(2, p)).astype(BF)
                for i in range(NG):
                    for hh in range(2):
                        h = 2 * p + hh
                        ol, hi = (ola, h) if h < SPLIT else (olb, h - SPLIT)
                        ol[orows[i]:orows[i] + 8, hi * E:(hi + 1) * E] = o[16 * i + 8 * hh:16 * i + 8 * hh + 8]

            after = {}
            for p in range(H // 2):
                after[2 * p + 2] = functools.partial(scores, p)
                after[2 * p + 5] = functools.partial(values, p)
            assert 2 * (SPLIT // 2 - 1) + 5 < H

            for h in range(H):
                for t in range(3):
                    proj(h, t)
                if h in after:
                    after[h]()

            oticks = []
            ks = 3 if odd else 1
            kw = SPLIT * E // ks
            l1 = ola[orows[0]:orows[0] + nrow, :]
            for j in range(8):
                r = None
                for k in range(ks):
                    x = _dot(l1[:, k * kw:(k + 1) * kw], _unpack(woa[j, k * kw // 2:(k + 1) * kw // 2, :]))
                    r = x if r is None else r + x
                    oticks.extend(_vregs(r))
                acc[j, 0:nrow, :] = r
                if H + j in after:
                    after[H + j]()
            l2 = olb[orows[0]:orows[0] + nrow, :]
            arow = pl.multiple_of(s * SEG - odd * 8, 8)
            for j in range(8):
                r = acc[j, 0:nrow, :] + _dot(l2, _unpack(woa[j, SPLIT * E // 2:, :]))
                if j < 4:
                    oticks.extend(_vregs(r))
                res = r.astype(BF)
                memb[:, j * 128:(j + 1) * 128] = res[0:MEM]
                outa[pl.ds(arow, nrow - MEM), j * 128:(j + 1) * 128] = res[MEM:]
            if odd:
                out_copy(outa, brow, 0, D, 0).start()
                b_values(make_gate(oticks, 8 * BM))
                b_out(brow)

        def steps(i, carry):
            for u in range(U):
                step(i * U + u, u % 2)
            return carry

        lax.fori_loop(0, NSEG // U, steps, 0)

        pltpu.make_async_copy(outb, out.at[:, pl.ds(D, D)], sem_out.at[1]).wait()
        pltpu.make_async_copy(outa, out.at[:, pl.ds(0, D)], sem_out.at[0]).wait()

    pl.run_scoped(
        phase2,
        vm((PAIR, SPLIT * E), BF),
        vm((PAIR, (H - SPLIT) * E), BF),
        vm((S, D), BF),
        vm((S, D), BF),
    )


@jax.jit
def _run(A_x, A_mem0, A_Wq, A_Wk, A_Wv, A_Wo, B_x, B_wqkv, B_wo):
    assert A_x.shape == (1, S, D) and A_mem0.shape == (1, MEM, D)
    assert A_Wq.shape == (D, H, E) and A_Wo.shape == (H, E, D)
    assert B_x.shape == (1, S, D) and B_wqkv.shape == (D, 3 * D) and B_wo.shape == (D, D)
    vm = pltpu.VMEM
    dma = pltpu.SemaphoreType.DMA
    scratch = [
        vm((NSEG * XR, D), BF),
        vm((S, D), BF),
        vm((MEM, D), BF),
        vm((3 * H, D // 2, E), U32),
        vm((8, H * E // 2, 128), U32),
        vm((24, D // 2, 128), U32),
        vm((8, D // 2, 128), U32),
    ] + [vm((3, NS * NG, 64, E), BF)] * NB + [
        vm((8, 48, 128), F32),
        vm((PAIR, PAIR), F32),
        vm((8, BM, 128), F32),
        vm((8, HIST + BM, 128), F32),
        vm((8, HIST + BM, 128), F32),
        vm((WIN, BM, 128), F32),
        vm((BM, D), BF),
        vm((8, 128), U32),
        dma((NSEM,)), dma((2,)),
    ]
    out = pl.pallas_call(
        _kernel,
        out_shape=jax.ShapeDtypeStruct((S, 2 * D), BF),
        in_specs=[pl.BlockSpec(memory_space=pl.ANY)] * 9,
        out_specs=pl.BlockSpec(memory_space=pl.ANY),
        scratch_shapes=scratch,
        compiler_params=pltpu.CompilerParams(vmem_limit_bytes=120 * 1024 * 1024,
                                             disable_bounds_checks=True,
                                             disable_semaphore_checks=True),
    )(A_x.reshape(S, D), A_mem0.reshape(MEM, D), A_Wq, A_Wk, A_Wv, A_Wo.reshape(8, 512, D),
      B_x.reshape(S, D), B_wqkv, B_wo)
    return out.reshape(1, S, 2 * D)


def pallas_concat_heads__memory_aug_recurrent_mem_tr__sliding_local_dilated__prompt_kernel(
    A_x: jax.Array,
    A_mem0: jax.Array,
    A_Wq: jax.Array,
    A_Wk: jax.Array,
    A_Wv: jax.Array,
    A_Wo: jax.Array,
    A_seg_len,
    B_x: jax.Array,
    B_wqkv: jax.Array,
    B_wo: jax.Array,
):
    if isinstance(A_seg_len, int):
        assert A_seg_len == SEG
    return _run(A_x, A_mem0, A_Wq, A_Wk, A_Wv, A_Wo, B_x, B_wqkv, B_wo)
```

```python
import functools

import jax
import jax.numpy as jnp
from jax import lax
import jax.experimental.pallas as pl
import jax.experimental.pallas.tpu as pltpu

BF = jnp.bfloat16
F32 = jnp.float32
U32 = jnp.uint32

S = 2048
D = 1024
H = 32
E = 128
MEM = 8
SEG = 32
L = MEM + SEG
NG = L // 8
NSEG = S // SEG
WIN = 8
DIL = 2
NEG = -1000000000.0
LOG2E = 1.4426950408889634

XR = 24
PRE = S - NSEG * XR
NS = 17
NB = 4
PAIR = 2 * L
SPLIT = 24
U = 4
BM = 2 * SEG
HIST = 16

NCH = 12
MB = 128
NKP = 4
KP = D // NKP
KA = 20
K1 = 16
W1A = 640
OA0 = NCH - 1 - 8
OB0 = NCH - 1 - 6
NTW = 4

SEM_MEM, SEM_X, SEM_W0, SEM_W, SEM_B, SEM_WOB, SEM_WOA, SEM_XA, SEM_XB, NSEM = (
    0, 1, 5, 9, 21, 27, 35, 43, 44, 45)


def _rcp(d):
    r = pl.reciprocal(d, approx=True)
    return r * (2.0 - d * r)


def _dot(a, b):
    return jnp.dot(a, b, preferred_element_type=F32)


def _unpack(w):
    return pltpu.bitcast(w, BF)


def _mod(x, d):
    m = 65536 // d + 1
    assert all((v * m) >> 16 == v // d for v in range(1024))
    return x - lax.shift_right_logical(x * m, 16) * d


def _lo_hi(a, b):
    lo = (a & U32(0xFFFF)) | (b << 16)
    hi = (a >> 16) | (b & U32(0xFFFF0000))
    return lo, hi


def _vregs(x):
    return [x[i:i + 8] for i in range(0, x.shape[0], 8)]


def _kernel(xa, mem0, wq, wk, wv, wo, xb, wqkv, wob, out,
            xar, xbb, memb, wa, woa, wb, wobp,
            r0, r1, r2, r3, acc, fill, qb, kb, vb, pb, ob, zero,
            sem, sem_out):
    rings = (r0, r1, r2, r3)
    wsrc = (wq, wk, wv)
    a_scale = E ** -0.5
    b_scale = (D // H) ** -0.5

    xar_copy = pltpu.make_async_copy(xa.at[pl.ds(PRE, NSEG * XR), :], xar, sem.at[SEM_XA])
    xb_copy = pltpu.make_async_copy(xb, xbb, sem.at[SEM_XB])
    mem_copy = pltpu.make_async_copy(mem0, memb, sem.at[SEM_MEM])

    def phase1(xpre, wst, woast, bst, wobst, tw, tb, tob, pacc):
        def st(i):
            return i if isinstance(i, int) else 0

        def w_copy(c):
            return pltpu.make_async_copy(
                wsrc[st(c) // 4].at[:, pl.ds((st(c) % 4) * 8, 8), :], wst.at[c], sem.at[SEM_W + c])

        def w0_copy(q):
            lo = q * KP if isinstance(q, int) else pl.multiple_of(q * KP, KP)
            return pltpu.make_async_copy(
                wq.at[pl.ds(st(q) * KP, KP), pl.ds(0, 8), :], wst.at[0, pl.ds(lo, KP)], sem.at[SEM_W0 + q])

        def w1_copy(q):
            lo, n = ((0, W1A), (W1A, D - W1A))[q]
            return pltpu.make_async_copy(
                wq.at[pl.ds(lo, n), pl.ds(8, 8), :], wst.at[1, pl.ds(lo, n)], sem.at[SEM_W + q])

        def x_copy(q):
            return pltpu.make_async_copy(
                xa.at[pl.ds(0, PRE), pl.ds(st(q) * KP, KP)], xpre.at[q], sem.at[SEM_X + q])

        def b_copy(j):
            return pltpu.make_async_copy(
                wqkv.at[pl.ds((st(j) % 2) * 512, 512), pl.ds((st(j) // 2) * D, D)], bst.at[j],
                sem.at[SEM_B + j])

        def wob_copy(j):
            return pltpu.make_async_copy(
                wob.at[:, pl.ds(st(j) * 128, 128)], wobst.at[j], sem.at[SEM_WOB + j])

        def woa_copy(j):
            return pltpu.make_async_copy(wo.at[st(j)], woast.at[j], sem.at[SEM_WOA + j])

        for q in range(NKP):
            w0_copy(q).start()
            x_copy(q).start()
        w1_copy(0).start()
        w1_copy(1).start()
        for c in range(1, NCH - 1):
            w_copy(c + 1).start()
            if c >= OA0:
                woa_copy(c - OA0).start()
                wob_copy(c - OA0).start()
            if c >= OB0:
                b_copy(c - OB0).start()
        mem_copy.start()
        xb_copy.start()
        xar_copy.start()

        def zero_fill(i, carry):
            r = pl.multiple_of(i * 32, 32)
            woast[8, pl.ds(r, 32), :] = jnp.zeros((32, D), BF)
            bst[6, pl.ds(r, 32), :] = jnp.zeros((32, D), BF)
            wobst[8, pl.ds(2 * r, 64), :] = jnp.zeros((64, 128), BF)
            for u in range(KA, 32):
                pacc[u % 8, pl.ds((u // 8) * MB + pl.multiple_of(i * 8, 8), 8), :] = jnp.zeros((8, E), F32)
            return carry

        lax.fori_loop(0, 16, zero_fill, 0)

        ri = lax.broadcasted_iota(jnp.int32, (PAIR, PAIR), 0)
        ci = lax.broadcasted_iota(jnp.int32, (PAIR, PAIR), 1)
        rb = (ri >> 3) & 1
        cb = (ci >> 3) & 1
        rl = ((ri >> 4) << 3) | (ri & 7)
        cl = ((ci >> 4) << 3) | (ci & 7)
        allowed = (rl < MEM) | (rl >= cl)
        fill[...] = jnp.where(rb == cb, jnp.where(allowed, 0.0, NEG / a_scale), -jnp.inf).astype(F32)
        kb[:, BM:BM + HIST, :] = jnp.zeros((8, HIST, 128), F32)
        vb[:, BM:BM + HIST, :] = jnp.zeros((8, HIST, 128), F32)
        zero[...] = jnp.zeros(zero.shape, U32)

        def gated(x, gate):
            return jnp.concatenate([v | gate() for v in _vregs(x)], axis=0)

        def relayout1(c, blk, row0=0, gate=None):
            v = wst[c, pl.ds(2 * row0 + blk * 16, 16)]
            v = pltpu.bitcast(v.reshape(128, 128), U32)
            for dp in range(8):
                x = v[8 * dp:8 * dp + 8]
                tw[blk % NTW, 9 * dp:9 * dp + 8, :] = x if gate is None else x | gate()

        def relayout2(base, blk, row0=0, gate=None):
            row = row0 + blk * 8
            for j in range(4):
                a = tw[blk % NTW, pl.ds(j, 8, stride=9), :]
                b = tw[blk % NTW, pl.ds(4 + j, 8, stride=9), :]
                if gate is not None:
                    g = gate()
                    a, b = a | g, b | g
                lo, hi = _lo_hi(a, b)
                wa[base + 2 * j, pl.ds(row, 8), :] = lo
                wa[base + 2 * j + 1, pl.ds(row, 8), :] = hi

        def relayout(c, base, b0, b1):
            for blk in range(b0, b1):
                relayout1(c, blk)
                relayout2(base, blk)

        def relayout_jobs(c, base, b0=0, b1=D // 16, row0=0):
            jobs = []
            for blk in range(b0, b1 + 1):
                if blk < b1:
                    jobs.append((8, functools.partial(relayout1, c, blk, row0)))
                if blk > b0:
                    jobs.append((4, functools.partial(relayout2, base, blk - 1, row0)))
            return jobs

        def b_prep1(src, e, cc, gate):
            x = pltpu.bitcast(bst[src, e * 256:(e + 1) * 256, cc * 128:(cc + 1) * 128], U32)
            x = gated(x, gate).T
            for hl in range(4):
                h = 4 * cc + hl
                tb[e, 33 * h:33 * h + 32, :] = x[32 * hl:32 * hl + 32]

        def b_prep2(j, e, cc, gate):
            y = jnp.concatenate(
                [tb[e, pl.ds(4 * cc + dl + 33 * 8 * g, 8, stride=33), :] for dl in range(4) for g in range(4)],
                axis=0)
            row = pl.multiple_of((j & 1) * 256, 256) + e * 128
            wb[(j >> 1) * 8 + cc, pl.ds(row, 128), :] = gated(y, gate).T

        def wob_prep1(src, g, gate):
            v = pltpu.bitcast(wobst[src, g * 512:(g + 1) * 512, :], U32)
            v = gated(v, gate)
            for hp in range(8):
                tob[g, 33 * hp:33 * hp + 32, :] = v[32 * hp:32 * hp + 32]

        def wob_prep2(j, g, gate):
            for dp in range(16):
                z = gate()
                lo, hi = _lo_hi(tob[g, pl.ds(dp, 8, stride=33), :] | z,
                                tob[g, pl.ds(16 + dp, 8, stride=33), :] | z)
                wobp[j, (2 * dp) * 16 + 8 * g:(2 * dp) * 16 + 8 * g + 8, :] = lo
                wobp[j, (2 * dp + 1) * 16 + 8 * g:(2 * dp + 1) * 16 + 8 * g + 8, :] = hi

        def woa_prep(src, j, q, gate):
            v = pltpu.bitcast(woast[src, :, q * 128:(q + 1) * 128], U32)
            woa[q, pl.ds(pl.multiple_of(j * 256, 256), 256), :] = gated(v, gate)

        def ring_store(c, hh, mb, r32):
            t = c >> 2
            g = c & 3
            r = r32.astype(BF)
            ring = rings[hh // 2]
            off = (g * 16 if isinstance(g, int) else pl.multiple_of(g * 16, 16)) + (hh % 2) * 8
            for k in range(MB // 8):
                plane = mb * (MB // SEG * NG) + (k // 4) * NG + 1 + k % 4
                ring[t, plane, pl.ds(off, 8), :] = r[8 * k:8 * k + 8]

        def run_units(c, base, u0, u1):
            ticks = []
            for u in range(u0, u1):
                hh, mb = u % 8, u // 8
                lhs = jnp.concatenate([xpre[q, mb * MB:(mb + 1) * MB, :] for q in range(NKP)], axis=1)
                r32 = _dot(lhs, _unpack(wa[base + hh]))
                ring_store(c, hh, mb, r32)
                ticks += _vregs(r32)
            return ticks

        def run_pieces(q, wrow, u0, u1, first=False):
            ticks = []
            for u in range(u0, u1):
                hh, mb = u % 8, u // 8
                rows = slice(mb * MB, (mb + 1) * MB)
                r32 = _dot(xpre[q, rows, :], _unpack(wa[hh, pl.ds(wrow, KP // 2), :]))
                if not first:
                    r32 = r32 + pacc[hh, rows, :]
                pacc[hh, rows, :] = r32
                ticks += _vregs(r32)
            return ticks

        def finish_chunk0(u, gate):
            hh, mb = u % 8, u // 8
            r = pltpu.bitcast(pacc[hh, mb * MB:(mb + 1) * MB, :], U32)
            ring_store(0, hh, mb, pltpu.bitcast(gated(r, gate), F32))

        def run_jobs(ticks, spare, jobs, free=0):
            ticks = ticks[:len(ticks) - spare * (MB // 8)]
            total = sum(n for n, _ in jobs)
            z = zero[...]
            cache = {}
            cnt = [0]

            def gate():
                k = (cnt[0] - free) * len(ticks) // (total - free)
                cnt[0] += 1
                if k < 0:
                    return z
                if k not in cache:
                    cache[k] = pltpu.bitcast(ticks[k], U32) & z
                return cache[k]

            for _, fn in jobs:
                fn(gate=gate)

        def interleave(*lists):
            items = []
            for l in lists:
                items += [((i + 0.5) / len(l), x) for i, x in enumerate(l)]
            items.sort(key=lambda z: z[0])
            return [x for _, x in items]

        nb = KP // 16

        def piece(q, carry):
            w0_copy(q + 1).wait()
            x_copy(q + 1).wait()
            wrow = pl.multiple_of(q * (KP // 2), KP // 2)
            ticks = run_pieces(q, wrow, KA, 32)
            run_jobs(ticks, 4, relayout_jobs(0, 0, nb, 2 * nb, wrow))
            run_pieces(q + 1, wrow + KP // 2, 0, KA)
            return carry

        def chunk(c, carry):
            w_copy(c + 1).wait()

            @pl.when(c >= OA0)
            def _():
                woa_copy(c - OA0).wait()
                wob_copy(c - OA0).wait()

            @pl.when(c >= OB0)
            def _():
                b_copy(c - OB0).wait()

            c8 = c * 8
            ticks = run_units(c, c8, K1, 32)
            run_jobs(ticks, 2, relayout_jobs(c + 1, c8 + 8))
            ticks = run_units(c + 1, c8 + 8, 0, K1)
            ja = jnp.maximum(c - OA0, 0)
            jb = jnp.maximum(c - OB0, 0)
            sa = jnp.where(c >= OA0, ja, 8)
            sb = jnp.where(c >= OB0, jb, 6)
            jobs = interleave(
                [(32, functools.partial(woa_prep, sa, ja, q)) for q in range(8)],
                [(32, functools.partial(wob_prep1, sa, g)) for g in range(2)]
                + [(16, functools.partial(wob_prep2, ja, g)) for g in range(2)],
                [(16, functools.partial(f, j, e, cc))
                 for e in range(2) for f, j in ((b_prep1, sb), (b_prep2, jb)) for cc in range(8)])
            run_jobs(ticks, 2, jobs)
            return carry

        w0_copy(0).wait()
        relayout(0, 0, 0, nb)
        x_copy(0).wait()
        run_pieces(0, 0, 0, KA, first=True)
        lax.fori_loop(0, NKP - 1, piece, 0)
        w1_copy(0).wait()
        ticks = run_pieces(NKP - 1, (NKP - 1) * KP // 2, KA, 32)
        run_jobs(ticks, 0, relayout_jobs(1, 8, 0, W1A // 16), free=100)
        w1_copy(1).wait()
        relayout(1, 8, W1A // 16, D // 16)
        ticks = run_units(1, 8, 0, K1)
        run_jobs(ticks, 2, [(16, functools.partial(finish_chunk0, u)) for u in range(32)])
        lax.fori_loop(1, NCH - 1, chunk, 0)
        run_units(NCH - 1, (NCH - 1) * 8, K1, 32)

    vm = pltpu.VMEM
    pl.run_scoped(
        phase1,
        vm((NKP, PRE, KP), BF),
        vm((NCH, D, 8, E), BF),
        vm((9, 512, D), BF),
        vm((7, 512, D), BF),
        vm((9, D, 128), BF),
        vm((NTW, 80, 128), U32),
        vm((2, 33 * H + 40, 128), U32),
        vm((2, 33 * 8 + 32, 128), U32),
        vm((8, PRE, E), F32),
    )
    mem_copy.wait()
    xb_copy.wait()
    xar_copy.wait()

    def phase2(ola, olb, outa, outb):
        def out_copy(buf, row, c0, nc, half):
            return pltpu.make_async_copy(
                buf.at[pl.ds(row, BM), pl.ds(c0, nc)], out.at[pl.ds(row, BM), pl.ds(half * D + c0, nc)],
                sem_out.at[half])

        def tie(x, y):
            return pltpu.bitcast(pltpu.bitcast(x, U32) | y, F32)

        def nil(y):
            return pltpu.bitcast(y, U32) & zero[...]

        def make_gate(ticks, n):
            cnt = [0]
            cache = {}

            def gate(x):
                k = cnt[0] * len(ticks) // n
                cnt[0] += 1
                if k not in cache:
                    cache[k] = nil(ticks[k])
                return tie(x, cache[k])
            return gate

        def b_logits(row, i, gate):
            q = [qb[cc, 8 * i:8 * i + 8, :] for cc in range(8)]
            pos = row + 8 * i + lax.broadcasted_iota(jnp.int32, (8, 128), 0)
            logits = []
            for w in range(WIN):
                lo = HIST + 8 * i - DIL * w
                t = None
                for cc in range(8):
                    x = gate(kb[cc, lo:lo + 8, :]) * q[cc]
                    t = x if t is None else t + x
                t = t + pltpu.roll(t, 64, 1)
                t = t + pltpu.roll(t, 32, 1)
                if 8 * i < DIL * w:
                    t = jnp.where(pos >= DIL * w, t, NEG)
                logits.append(t)
            return logits, functools.reduce(jnp.maximum, logits)

        def b_softmax(i, logits, m, gate):
            ex = [jnp.exp(gate(t) - m) for t in logits]
            r = _rcp(functools.reduce(lambda a, b: a + b, ex))
            for w in range(WIN):
                pb[w, 8 * i:8 * i + 8, :] = gate(ex[w]) * r

        def b_values(gate):
            for i in range(BM // 8):
                p = [pb[w, 8 * i:8 * i + 8, :] for w in range(WIN)]
                for cc in range(8):
                    t = None
                    for w in range(WIN):
                        lo = HIST + 8 * i - DIL * w
                        x = gate(vb[cc, lo:lo + 8, :]) * p[w]
                        t = x if t is None else t + x
                    ob[8 * i:8 * i + 8, cc * 128:(cc + 1) * 128] = t.astype(BF)

        def b_out(row):
            o = ob[...]
            for j in range(8):
                outb[pl.ds(row, BM), j * 128:(j + 1) * 128] = _dot(o, _unpack(wobp[j])).astype(BF)
                if j % 2 == 1:
                    out_copy(outb, row, (j - 1) * 128, 256, 1).start()

        def step(s, odd):
            brow = pl.multiple_of((s - odd) * SEG, BM)
            xrows = xbb[pl.ds(brow, BM), :]
            if not odd:
                for cc in range(8):
                    kb[cc, 0:HIST, :] = kb[cc, BM:BM + HIST, :]
                    vb[cc, 0:HIST, :] = vb[cc, BM:BM + HIST, :]
                for cc in range(8):
                    qb[cc] = _dot(xrows, _unpack(wb[cc])) * b_scale
                    kb[cc, HIST:HIST + BM, :] = _dot(xrows, _unpack(wb[8 + cc]))
            ticks = []
            for cc in range(4 * odd, 4 * odd + 4):
                r = _dot(xrows, _unpack(wb[16 + cc]))
                vb[cc, HIST:HIST + BM, :] = r
                ticks.extend(_vregs(r))
            groups = range(4 * odd, 4 * odd + 4)
            lm = {}

            lhs = jnp.concatenate([memb[...], xar[pl.ds(pl.multiple_of(s * XR, 8), XR), :]], axis=0)
            slot = _mod(s, NS) * NG
            planes = [slot]
            for i in range(3):
                g = PRE // 8 + 3 * s + i
                planes.append(_mod(g >> 2, NS) * NG + 1 + (g & 3))
            orows = (32, 48, 56, 64, 72) if odd else (0, 8, 16, 24, 40)
            nrow = 48 if odd else 32

            def proj(h, t):
                n = 3 * h + t
                p = h // 2
                r32 = _dot(lhs, _unpack(wa[t * H + h]))
                for k, i in enumerate(groups):
                    if n == 5 + 2 * k:
                        r32 = jnp.concatenate([tie(r32[0:8], nil(lm[i][1])), r32[8:]], axis=0)
                ticks.extend(_vregs(r32))
                if n == 2:
                    gate = make_gate(list(ticks), 64 * len(groups))
                    for i in groups:
                        lm[i] = b_logits(brow, i, gate)
                for k, i in enumerate(groups):
                    if n == 7 + 2 * k:
                        b_softmax(i, lm[i][0], lm[i][1], make_gate(ticks[-8:], 16))
                r = r32.astype(BF)
                ro = (p // NB) * 16 + (h % 2) * 8
                for i in range(4):
                    rings[p % NB][t, planes[i], ro:ro + 8, :] = r[8 * i:8 * i + 8]

            probs = {}

            def pair(t, p):
                ro = (p // NB) * 16
                return rings[p % NB][t, pl.ds(slot, NG), ro:ro + 16, :].reshape(PAIR, E)

            def scores(p):
                sc = lax.dot_general(pair(0, p), pair(1, p), (((1,), (1,)), ((), ())),
                                     preferred_element_type=F32)
                fl = fill[...]
                sc = jnp.where(fl == 0.0, sc, fl)
                e = jnp.exp2((sc - jnp.max(sc, axis=1, keepdims=True)) * (a_scale * LOG2E))
                probs[p] = (e * _rcp(jnp.sum(e, axis=1, keepdims=True))).astype(BF)

            def values(p):
                o = _dot(probs.pop(p), pair(2, p)).astype(BF)
                for i in range(NG):
                    for hh in range(2):
                        h = 2 * p + hh
                        ol, hi = (ola, h) if h < SPLIT else (olb, h - SPLIT)
                        ol[orows[i]:orows[i] + 8, hi * E:(hi + 1) * E] = o[16 * i + 8 * hh:16 * i + 8 * hh + 8]

            after = {}
            for p in range(H // 2):
                after[2 * p + 2] = functools.partial(scores, p)
                after[2 * p + 5] = functools.partial(values, p)
            assert 2 * (SPLIT // 2 - 1) + 5 < H

            for h in range(H):
                for t in range(3):
                    proj(h, t)
                if h in after:
                    after[h]()

            oticks = []
            ks = 3 if odd else 1
            kw = SPLIT * E // ks
            l1 = ola[orows[0]:orows[0] + nrow, :]
            for j in range(8):
                r = None
                for k in range(ks):
                    x = _dot(l1[:, k * kw:(k + 1) * kw], _unpack(woa[j, k * kw // 2:(k + 1) * kw // 2, :]))
                    r = x if r is None else r + x
                    oticks.extend(_vregs(r))
                acc[j, 0:nrow, :] = r
                if H + j in after:
                    after[H + j]()
            l2 = olb[orows[0]:orows[0] + nrow, :]
            arow = pl.multiple_of(s * SEG - odd * 8, 8)
            for j in range(8):
                r = acc[j, 0:nrow, :] + _dot(l2, _unpack(woa[j, SPLIT * E // 2:, :]))
                if j < 4:
                    oticks.extend(_vregs(r))
                res = r.astype(BF)
                memb[:, j * 128:(j + 1) * 128] = res[0:MEM]
                outa[pl.ds(arow, nrow - MEM), j * 128:(j + 1) * 128] = res[MEM:]
            if odd:
                out_copy(outa, brow, 0, D, 0).start()
                b_values(make_gate(oticks, 8 * BM))
                b_out(brow)

        def steps(i, carry):
            for u in range(U):
                step(i * U + u, u % 2)
            return carry

        lax.fori_loop(0, NSEG // U, steps, 0)

        pltpu.make_async_copy(outb, out.at[:, pl.ds(D, D)], sem_out.at[1]).wait()
        pltpu.make_async_copy(outa, out.at[:, pl.ds(0, D)], sem_out.at[0]).wait()

    pl.run_scoped(
        phase2,
        vm((PAIR, SPLIT * E), BF),
        vm((PAIR, (H - SPLIT) * E), BF),
        vm((S, D), BF),
        vm((S, D), BF),
    )


@jax.jit
def _run(A_x, A_mem0, A_Wq, A_Wk, A_Wv, A_Wo, B_x, B_wqkv, B_wo):
    assert A_x.shape == (1, S, D) and A_mem0.shape == (1, MEM, D)
    assert A_Wq.shape == (D, H, E) and A_Wo.shape == (H, E, D)
    assert B_x.shape == (1, S, D) and B_wqkv.shape == (D, 3 * D) and B_wo.shape == (D, D)
    vm = pltpu.VMEM
    dma = pltpu.SemaphoreType.DMA
    scratch = [
        vm((NSEG * XR, D), BF),
        vm((S, D), BF),
        vm((MEM, D), BF),
        vm((3 * H, D // 2, E), U32),
        vm((8, H * E // 2, 128), U32),
        vm((24, D // 2, 128), U32),
        vm((8, D // 2, 128), U32),
    ] + [vm((3, NS * NG, 64, E), BF)] * NB + [
        vm((8, 48, 128), F32),
        vm((PAIR, PAIR), F32),
        vm((8, BM, 128), F32),
        vm((8, HIST + BM, 128), F32),
        vm((8, HIST + BM, 128), F32),
        vm((WIN, BM, 128), F32),
        vm((BM, D), BF),
        vm((8, 128), U32),
        dma((NSEM,)), dma((2,)),
    ]
    out = pl.pallas_call(
        _kernel,
        out_shape=jax.ShapeDtypeStruct((S, 2 * D), BF),
        in_specs=[pl.BlockSpec(memory_space=pl.ANY)] * 9,
        out_specs=pl.BlockSpec(memory_space=pl.ANY),
        scratch_shapes=scratch,
        compiler_params=pltpu.CompilerParams(vmem_limit_bytes=120 * 1024 * 1024,
                                             disable_bounds_checks=True,
                                             disable_semaphore_checks=True),
    )(A_x.reshape(S, D), A_mem0.reshape(MEM, D), A_Wq, A_Wk, A_Wv, A_Wo.reshape(8, 512, D),
      B_x.reshape(S, D), B_wqkv, B_wo)
    return out.reshape(1, S, 2 * D)


def pallas_concat_heads__memory_aug_recurrent_mem_tr__sliding_local_dilated__prompt_kernel(
    A_x: jax.Array,
    A_mem0: jax.Array,
    A_Wq: jax.Array,
    A_Wk: jax.Array,
    A_Wv: jax.Array,
    A_Wo: jax.Array,
    A_seg_len,
    B_x: jax.Array,
    B_wqkv: jax.Array,
    B_wo: jax.Array,
):
    if isinstance(A_seg_len, int):
        assert A_seg_len == SEG
    return _run(A_x, A_mem0, A_Wq, A_Wk, A_Wv, A_Wo, B_x, B_wqkv, B_wo)
```

```python
import functools

import jax
import jax.numpy as jnp
from jax import lax
import jax.experimental.pallas as pl
import jax.experimental.pallas.tpu as pltpu

BF = jnp.bfloat16
F32 = jnp.float32
U32 = jnp.uint32

S = 2048
D = 1024
H = 32
E = 128
MEM = 8
SEG = 32
L = MEM + SEG
NG = L // 8
NSEG = S // SEG
WIN = 8
DIL = 2
NEG = -1000000000.0
LOG2E = 1.4426950408889634

XR = 24
PRE = S - NSEG * XR
NS = 17
NB = 4
PAIR = 2 * L
SPLIT = 24
U = 4
BM = 2 * SEG
HIST = 16

NCH = 12
MB = 128
NKP = 4
KP = D // NKP
KA = 20
K1 = 16
W1A = 640
OA0 = NCH - 1 - 8
OB0 = NCH - 1 - 6
NTW = 4

SEM_MEM, SEM_X, SEM_W0, SEM_W, SEM_B, SEM_WOB, SEM_WOA, SEM_XA, SEM_XB, NSEM = (
    0, 1, 5, 9, 21, 27, 35, 43, 44, 45)


def _rcp(d):
    r = pl.reciprocal(d, approx=True)
    return r * (2.0 - d * r)


def _dot(a, b):
    return jnp.dot(a, b, preferred_element_type=F32)


def _unpack(w):
    return pltpu.bitcast(w, BF)


def _mod(x, d):
    m = 65536 // d + 1
    assert all((v * m) >> 16 == v // d for v in range(1024))
    return x - lax.shift_right_logical(x * m, 16) * d


def _lo_hi(a, b):
    lo = (a & U32(0xFFFF)) | (b << 16)
    hi = (a >> 16) | (b & U32(0xFFFF0000))
    return lo, hi


def _vregs(x):
    return [x[i:i + 8] for i in range(0, x.shape[0], 8)]


def _kernel(xa, mem0, wq, wk, wv, wo, xb, wqkv, wob, out,
            xar, xbb, memb, wa, woa, wb, wobp,
            r0, r1, r2, r3, acc, fill, qb, kb, vb, pb, ob, zero,
            sem, sem_out):
    rings = (r0, r1, r2, r3)
    wsrc = (wq, wk, wv)
    a_scale = E ** -0.5
    b_scale = (D // H) ** -0.5

    xar_copy = pltpu.make_async_copy(xa.at[pl.ds(PRE, NSEG * XR), :], xar, sem.at[SEM_XA])
    xb_copy = pltpu.make_async_copy(xb, xbb, sem.at[SEM_XB])
    mem_copy = pltpu.make_async_copy(mem0, memb, sem.at[SEM_MEM])

    def phase1(xpre, wst, woast, bst, wobst, tw, tb, tob, pacc):
        def st(i):
            return i if isinstance(i, int) else 0

        def w_copy(c):
            return pltpu.make_async_copy(
                wsrc[st(c) // 4].at[:, pl.ds((st(c) % 4) * 8, 8), :], wst.at[c], sem.at[SEM_W + c])

        def w0_copy(q):
            lo = q * KP if isinstance(q, int) else pl.multiple_of(q * KP, KP)
            return pltpu.make_async_copy(
                wq.at[pl.ds(st(q) * KP, KP), pl.ds(0, 8), :], wst.at[0, pl.ds(lo, KP)], sem.at[SEM_W0 + q])

        def w1_copy(q):
            lo, n = ((0, W1A), (W1A, D - W1A))[q]
            return pltpu.make_async_copy(
                wq.at[pl.ds(lo, n), pl.ds(8, 8), :], wst.at[1, pl.ds(lo, n)], sem.at[SEM_W + q])

        def x_copy(q):
            return pltpu.make_async_copy(
                xa.at[pl.ds(0, PRE), pl.ds(st(q) * KP, KP)], xpre.at[q], sem.at[SEM_X + q])

        def b_copy(j):
            return pltpu.make_async_copy(
                wqkv.at[pl.ds((st(j) % 2) * 512, 512), pl.ds((st(j) // 2) * D, D)], bst.at[j],
                sem.at[SEM_B + j])

        def wob_copy(j):
            return pltpu.make_async_copy(
                wob.at[:, pl.ds(st(j) * 128, 128)], wobst.at[j], sem.at[SEM_WOB + j])

        def woa_copy(j):
            return pltpu.make_async_copy(wo.at[st(j)], woast.at[j], sem.at[SEM_WOA + j])

        for q in range(NKP):
            w0_copy(q).start()
            x_copy(q).start()
        w1_copy(0).start()
        w1_copy(1).start()
        for c in range(1, NCH - 1):
            w_copy(c + 1).start()
            if c >= OA0:
                woa_copy(c - OA0).start()
                wob_copy(c - OA0).start()
            if c >= OB0:
                b_copy(c - OB0).start()
        mem_copy.start()
        xb_copy.start()
        xar_copy.start()

        def zero_fill(i, carry):
            r = pl.multiple_of(i * 32, 32)
            woast[8, pl.ds(r, 32), :] = jnp.zeros((32, D), BF)
            bst[6, pl.ds(r, 32), :] = jnp.zeros((32, D), BF)
            wobst[8, pl.ds(2 * r, 64), :] = jnp.zeros((64, 128), BF)
            for u in range(KA, 32):
                pacc[u % 8, pl.ds((u // 8) * MB + pl.multiple_of(i * 8, 8), 8), :] = jnp.zeros((8, E), F32)
            return carry

        lax.fori_loop(0, 16, zero_fill, 0)

        ri = lax.broadcasted_iota(jnp.int32, (PAIR, PAIR), 0)
        ci = lax.broadcasted_iota(jnp.int32, (PAIR, PAIR), 1)
        rb = (ri >> 3) & 1
        cb = (ci >> 3) & 1
        rl = ((ri >> 4) << 3) | (ri & 7)
        cl = ((ci >> 4) << 3) | (ci & 7)
        allowed = (rl < MEM) | (rl >= cl)
        fill[...] = jnp.where(rb == cb, jnp.where(allowed, 0.0, NEG / a_scale), -jnp.inf).astype(F32)
        kb[:, BM:BM + HIST, :] = jnp.zeros((8, HIST, 128), F32)
        vb[:, BM:BM + HIST, :] = jnp.zeros((8, HIST, 128), F32)
        zero[...] = jnp.zeros(zero.shape, U32)

        def gated(x, gate):
            return jnp.concatenate([v | gate() for v in _vregs(x)], axis=0)

        def relayout1(c, blk, row0=0, gate=None):
            v = wst[c, pl.ds(2 * row0 + blk * 16, 16)]
            v = pltpu.bitcast(v.reshape(128, 128), U32)
            for dp in range(8):
                x = v[8 * dp:8 * dp + 8]
                tw[blk % NTW, 9 * dp:9 * dp + 8, :] = x if gate is None else x | gate()

        def relayout2(base, blk, row0=0, gate=None):
            row = row0 + blk * 8
            for j in range(4):
                a = tw[blk % NTW, pl.ds(j, 8, stride=9), :]
                b = tw[blk % NTW, pl.ds(4 + j, 8, stride=9), :]
                if gate is not None:
                    g = gate()
                    a, b = a | g, b | g
                lo, hi = _lo_hi(a, b)
                wa[base + 2 * j, pl.ds(row, 8), :] = lo
                wa[base + 2 * j + 1, pl.ds(row, 8), :] = hi

        def relayout(c, base, b0, b1):
            for blk in range(b0, b1):
                relayout1(c, blk)
                relayout2(base, blk)

        def relayout_jobs(c, base, b0=0, b1=D // 16, row0=0):
            jobs = []
            for blk in range(b0, b1 + 1):
                if blk < b1:
                    jobs.append((8, functools.partial(relayout1, c, blk, row0)))
                if blk > b0:
                    jobs.append((4, functools.partial(relayout2, base, blk - 1, row0)))
            return jobs

        def b_prep1(src, e, cc, gate):
            x = pltpu.bitcast(bst[src, e * 256:(e + 1) * 256, cc * 128:(cc + 1) * 128], U32)
            x = gated(x, gate).T
            for hl in range(4):
                h = 4 * cc + hl
                tb[e, 33 * h:33 * h + 32, :] = x[32 * hl:32 * hl + 32]

        def b_prep2(j, e, cc, gate):
            y = jnp.concatenate(
                [tb[e, pl.ds(4 * cc + dl + 33 * 8 * g, 8, stride=33), :] for dl in range(4) for g in range(4)],
                axis=0)
            row = pl.multiple_of((j & 1) * 256, 256) + e * 128
            wb[(j >> 1) * 8 + cc, pl.ds(row, 128), :] = gated(y, gate).T

        def wob_prep1(src, g, gate):
            v = pltpu.bitcast(wobst[src, g * 512:(g + 1) * 512, :], U32)
            v = gated(v, gate)
            for hp in range(8):
                tob[g, 33 * hp:33 * hp + 32, :] = v[32 * hp:32 * hp + 32]

        def wob_prep2(j, g, gate):
            for dp in range(16):
                z = gate()
                lo, hi = _lo_hi(tob[g, pl.ds(dp, 8, stride=33), :] | z,
                                tob[g, pl.ds(16 + dp, 8, stride=33), :] | z)
                wobp[j, (2 * dp) * 16 + 8 * g:(2 * dp) * 16 + 8 * g + 8, :] = lo
                wobp[j, (2 * dp + 1) * 16 + 8 * g:(2 * dp + 1) * 16 + 8 * g + 8, :] = hi

        def woa_prep(src, j, q, gate):
            v = pltpu.bitcast(woast[src, :, q * 128:(q + 1) * 128], U32)
            woa[q, pl.ds(pl.multiple_of(j * 256, 256), 256), :] = gated(v, gate)

        def ring_store(c, hh, mb, r32):
            t = c >> 2
            g = c & 3
            r = r32.astype(BF)
            ring = rings[hh // 2]
            off = (g * 16 if isinstance(g, int) else pl.multiple_of(g * 16, 16)) + (hh % 2) * 8
            for k in range(MB // 8):
                plane = mb * (MB // SEG * NG) + (k // 4) * NG + 1 + k % 4
                ring[t, plane, pl.ds(off, 8), :] = r[8 * k:8 * k + 8]

        def run_units(c, base, u0, u1):
            ticks = []
            for u in range(u0, u1):
                hh, mb = u % 8, u // 8
                lhs = jnp.concatenate([xpre[q, mb * MB:(mb + 1) * MB, :] for q in range(NKP)], axis=1)
                r32 = _dot(lhs, _unpack(wa[base + hh]))
                ring_store(c, hh, mb, r32)
                ticks += _vregs(r32)
            return ticks

        def run_pieces(q, wrow, u0, u1, first=False):
            ticks = []
            for u in range(u0, u1):
                hh, mb = u % 8, u // 8
                rows = slice(mb * MB, (mb + 1) * MB)
                r32 = _dot(xpre[q, rows, :], _unpack(wa[hh, pl.ds(wrow, KP // 2), :]))
                if not first:
                    r32 = r32 + pacc[hh, rows, :]
                pacc[hh, rows, :] = r32
                ticks += _vregs(r32)
            return ticks

        def finish_chunk0(u, gate):
            hh, mb = u % 8, u // 8
            r = pltpu.bitcast(pacc[hh, mb * MB:(mb + 1) * MB, :], U32)
            ring_store(0, hh, mb, pltpu.bitcast(gated(r, gate), F32))

        def run_jobs(ticks, spare, jobs, free=0):
            ticks = ticks[:len(ticks) - spare * (MB // 8)]
            total = sum(n for n, _ in jobs)
            z = zero[...]
            cache = {}
            cnt = [0]

            def gate():
                k = (cnt[0] - free) * len(ticks) // (total - free)
                cnt[0] += 1
                if k < 0:
                    return z
                if k not in cache:
                    cache[k] = pltpu.bitcast(ticks[k], U32) & z
                return cache[k]

            for _, fn in jobs:
                fn(gate=gate)

        def interleave(*lists):
            items = []
            for l in lists:
                items += [((i + 0.5) / len(l), x) for i, x in enumerate(l)]
            items.sort(key=lambda z: z[0])
            return [x for _, x in items]

        nb = KP // 16

        def piece(q, carry):
            w0_copy(q + 1).wait()
            x_copy(q + 1).wait()
            wrow = pl.multiple_of(q * (KP // 2), KP // 2)
            ticks = run_pieces(q, wrow, KA, 32)
            run_jobs(ticks, 4, relayout_jobs(0, 0, nb, 2 * nb, wrow))
            run_pieces(q + 1, wrow + KP // 2, 0, KA)
            return carry

        def chunk(c, carry):
            w_copy(c + 1).wait()

            @pl.when(c >= OA0)
            def _():
                woa_copy(c - OA0).wait()
                wob_copy(c - OA0).wait()

            @pl.when(c >= OB0)
            def _():
                b_copy(c - OB0).wait()

            c8 = c * 8
            ticks = run_units(c, c8, K1, 32)
            run_jobs(ticks, 2, relayout_jobs(c + 1, c8 + 8))
            ticks = run_units(c + 1, c8 + 8, 0, K1)
            ja = jnp.maximum(c - OA0, 0)
            jb = jnp.maximum(c - OB0, 0)
            sa = jnp.where(c >= OA0, ja, 8)
            sb = jnp.where(c >= OB0, jb, 6)
            jobs = interleave(
                [(32, functools.partial(woa_prep, sa, ja, q)) for q in range(8)],
                [(32, functools.partial(wob_prep1, sa, g)) for g in range(2)]
                + [(16, functools.partial(wob_prep2, ja, g)) for g in range(2)],
                [(16, functools.partial(f, j, e, cc))
                 for e in range(2) for f, j in ((b_prep1, sb), (b_prep2, jb)) for cc in range(8)])
            run_jobs(ticks, 2, jobs)
            return carry

        w0_copy(0).wait()
        relayout(0, 0, 0, nb)
        x_copy(0).wait()
        run_pieces(0, 0, 0, KA, first=True)
        lax.fori_loop(0, NKP - 1, piece, 0)
        w1_copy(0).wait()
        ticks = run_pieces(NKP - 1, (NKP - 1) * KP // 2, KA, 32)
        run_jobs(ticks, 0, relayout_jobs(1, 8, 0, W1A // 16), free=100)
        w1_copy(1).wait()
        relayout(1, 8, W1A // 16, D // 16)
        ticks = run_units(1, 8, 0, K1)
        run_jobs(ticks, 2, [(16, functools.partial(finish_chunk0, u)) for u in range(32)])
        lax.fori_loop(1, NCH - 1, chunk, 0)
        run_units(NCH - 1, (NCH - 1) * 8, K1, 32)

    vm = pltpu.VMEM
    pl.run_scoped(
        phase1,
        vm((NKP, PRE, KP), BF),
        vm((NCH, D, 8, E), BF),
        vm((9, 512, D), BF),
        vm((7, 512, D), BF),
        vm((9, D, 128), BF),
        vm((NTW, 80, 128), U32),
        vm((2, 33 * H + 40, 128), U32),
        vm((2, 33 * 8 + 32, 128), U32),
        vm((8, PRE, E), F32),
    )
    mem_copy.wait()
    xb_copy.wait()
    xar_copy.wait()

    def phase2(ola, olb, outa, outb):
        def out_copy(buf, row, c0, nc, half):
            return pltpu.make_async_copy(
                buf.at[pl.ds(row, BM), pl.ds(c0, nc)], out.at[pl.ds(row, BM), pl.ds(half * D + c0, nc)],
                sem_out.at[half])

        def tie(x, y):
            return pltpu.bitcast(pltpu.bitcast(x, U32) | y, F32)

        def nil(y):
            return pltpu.bitcast(y, U32) & zero[...]

        def tie_lhs(x, ys):
            if not ys:
                return x
            t = pltpu.bitcast(x[0:16, 0:128], U32)
            for y in ys:
                t = t | nil(y)
            top = jnp.concatenate([pltpu.bitcast(t, BF), x[0:16, 128:]], axis=1)
            return jnp.concatenate([top, x[16:]], axis=0)

        def make_gate(ticks, n):
            cnt = [0]
            cache = {}

            def gate(x):
                k = cnt[0] * len(ticks) // n
                cnt[0] += 1
                if k not in cache:
                    cache[k] = nil(ticks[k])
                return tie(x, cache[k])
            return gate

        def b_logits(row, i, gate):
            q = [qb[cc, 8 * i:8 * i + 8, :] for cc in range(8)]
            pos = row + 8 * i + lax.broadcasted_iota(jnp.int32, (8, 128), 0)
            logits = []
            for w in range(WIN):
                lo = HIST + 8 * i - DIL * w
                t = None
                for cc in range(8):
                    x = gate(kb[cc, lo:lo + 8, :]) * q[cc]
                    t = x if t is None else t + x
                t = t + pltpu.roll(t, 64, 1)
                t = t + pltpu.roll(t, 32, 1)
                if 8 * i < DIL * w:
                    t = jnp.where(pos >= DIL * w, t, NEG)
                logits.append(t)
            return logits, functools.reduce(jnp.maximum, logits)

        def b_softmax(i, logits, m, gate):
            ex = [jnp.exp(gate(t) - m) for t in logits]
            r = _rcp(functools.reduce(lambda a, b: a + b, ex))
            for w in range(WIN):
                pb[w, 8 * i:8 * i + 8, :] = gate(ex[w]) * r

        def b_values(i, gate):
            p = [pb[w, 8 * i:8 * i + 8, :] for w in range(WIN)]
            for cc in range(8):
                t = None
                for w in range(WIN):
                    lo = HIST + 8 * i - DIL * w
                    x = gate(vb[cc, lo:lo + 8, :]) * p[w]
                    t = x if t is None else t + x
                ob[8 * i:8 * i + 8, cc * 128:(cc + 1) * 128] = t.astype(BF)

        def b_out(row):
            o = ob[...]
            for j in range(8):
                outb[pl.ds(row, BM), j * 128:(j + 1) * 128] = _dot(o, _unpack(wobp[j])).astype(BF)
                if j % 2 == 1:
                    out_copy(outb, row, (j - 1) * 128, 256, 1).start()

        def o_store(h, row, o):
            ol, hi = (ola, h) if h < SPLIT else (olb, h - SPLIT)
            ol[row:row + 8, hi * E:(hi + 1) * E] = o

        def b_project(s, brow):
            slot = _mod(s - 1, NS) * NG

            def grp(t, h, i):
                p = h // 2
                ro = (p // NB) * 16 + (h % 2) * 8
                return rings[p % NB][t, slot + i, ro:ro + 8, :].astype(F32)

            def v_scores(h, gate):
                sub = lax.broadcasted_iota(jnp.int32, (8, 1), 0)
                q = grp(0, h, 1) * (a_scale * LOG2E)
                sc = []
                for kg in range(2):
                    k = gate(grp(1, h, kg))
                    for j in range(8):
                        x = jnp.sum(jnp.broadcast_to(k[j:j + 1, :], (8, E)) * q, axis=1, keepdims=True)
                        if kg == 1 and j > 0:
                            x = jnp.where(sub >= j, x, NEG * LOG2E)
                        sc.append(jnp.broadcast_to(x, (8, E)))
                return sc, functools.reduce(jnp.maximum, sc)

            def v_values(h, sc, m, gate):
                den = None
                o = None
                for kg in range(2):
                    v = grp(2, h, kg)
                    mg = gate(m)
                    for j in range(8):
                        e = jnp.exp2(sc[8 * kg + j] - mg)
                        den = e if den is None else den + e
                        x = e * jnp.broadcast_to(v[j:j + 1, :], (8, E))
                        o = x if o is None else o + x
                o_store(h, 40, (o * _rcp(den)).astype(BF))

            xrows = xbb[pl.ds(brow, BM), :]
            for cc in range(8):
                kb[cc, 0:HIST, :] = kb[cc, BM:BM + HIST, :]
                vb[cc, 0:HIST, :] = vb[cc, BM:BM + HIST, :]
            sm = {}
            dead = {}
            nq = 21

            def heads(n):
                return range(n * H // nq, (n + 1) * H // nq) if 0 <= n < nq else []

            for n in range(24):
                part, cc = (n % 2, n // 2) if n < 16 else (2, n - 16)
                r = _dot(tie_lhs(xrows, dead.get(n)), _unpack(wb[8 * part + cc]))
                if part == 0:
                    qb[cc] = r * b_scale
                elif part == 1:
                    kb[cc, HIST:HIST + BM, :] = r
                else:
                    vb[cc, HIST:HIST + BM, :] = r
                gate = make_gate(_vregs(r), 2 * len(heads(n)))
                for h in heads(n):
                    sm[h] = v_scores(h, gate)
                    dead.setdefault(n + 5, []).append(sm[h][1])
                gate = make_gate(_vregs(r), 2 * len(heads(n - 3)))
                for h in heads(n - 3):
                    v_values(h, sm[h][0], sm[h][1], gate)
            return {2 * (n - 24): ys for n, ys in dead.items() if n >= 24}

        b_plan = {2: [('l', 3, 3)], 5: [('l', 4, 3)], 7: [('s', 3, 1)], 9: [('l', 5, 3), ('v', 0, 2)],
                  10: [('s', 4, 1)], 12: [('l', 6, 3), ('v', 1, 2)], 14: [('s', 5, 1), ('v', 2, 2)],
                  16: [('l', 7, 3)], 17: [('s', 6, 1), ('v', 3, 2)], 20: [('v', 4, 2)], 21: [('s', 7, 1)],
                  22: [('v', 5, 2)], 25: [('v', 6, 2)], 28: [('v', 7, 2)]}

        def step(s, odd):
            brow = pl.multiple_of((s - odd) * SEG, BM)
            dead = b_project(s, brow) if odd else {}
            early = range(3) if odd else []
            lm = {}
            ticks = []

            lhs = jnp.concatenate([memb[...], xar[pl.ds(pl.multiple_of(s * XR, 8), XR), :]], axis=0)
            slot = _mod(s, NS) * NG
            planes = [slot]
            for i in range(3):
                g = PRE // 8 + 3 * s + i
                planes.append(_mod(g >> 2, NS) * NG + 1 + (g & 3))
            qgroups = (0, 1, 2, 3, 4) if odd else (0, 2, 3, 4)
            orows = (32, 48, 56, 64, 72) if odd else (0, 8, 16, 24)
            nrow = 48 if odd else 32

            def proj(h, t):
                n = 3 * h + t
                p = h // 2
                r32 = _dot(tie_lhs(lhs, dead.get(n)), _unpack(wa[t * H + h]))
                for i in early:
                    if n == 7 + 2 * i:
                        r32 = jnp.concatenate([tie(r32[0:8], nil(lm[i][1])), r32[8:]], axis=0)
                ticks.extend(_vregs(r32))
                if n == 4 and odd:
                    gate = make_gate(list(ticks), 64 * len(early))
                    for i in early:
                        lm[i] = b_logits(brow, i, gate)
                for i in early:
                    if n == 9 + 2 * i:
                        b_softmax(i, lm[i][0], lm[i][1], make_gate(ticks[-8:], 16))
                r = r32.astype(BF)
                ro = (p // NB) * 16 + (h % 2) * 8
                for i in range(4):
                    rings[p % NB][t, planes[i], ro:ro + 8, :] = r[8 * i:8 * i + 8]

            probs = {}

            def pair(t, p):
                ro = (p // NB) * 16
                return rings[p % NB][t, pl.ds(slot, NG), ro:ro + 16, :].reshape(PAIR, E)

            def qrows(x):
                return jnp.concatenate([x[16 * i:16 * i + 16] for i in qgroups], axis=0)

            def scores(p):
                sc = lax.dot_general(qrows(pair(0, p)), pair(1, p), (((1,), (1,)), ((), ())),
                                     preferred_element_type=F32)
                fl = qrows(fill[...])
                sc = jnp.where(fl == 0.0, sc, fl)
                e = jnp.exp2((sc - jnp.max(sc, axis=1, keepdims=True)) * (a_scale * LOG2E))
                probs[p] = (e * _rcp(jnp.sum(e, axis=1, keepdims=True))).astype(BF)

            def values(p):
                o = _dot(probs.pop(p), pair(2, p)).astype(BF)
                for k, row in enumerate(orows):
                    for hh in range(2):
                        o_store(2 * p + hh, row, o[16 * k + 8 * hh:16 * k + 8 * hh + 8])

            after = {}
            for p in range(H // 2):
                after[2 * p + 2] = functools.partial(scores, p)
                after[2 * p + 5] = functools.partial(values, p)
            assert 2 * (SPLIT // 2 - 1) + 5 < H

            for h in range(H):
                for t in range(3):
                    proj(h, t)
                if h in after:
                    after[h]()

            oticks = []
            odead = {}
            count = [0]

            def out_dot(l, w, prev):
                n = count[0]
                count[0] += 1
                r = _dot(tie_lhs(l, odead.get(n)), _unpack(w))
                r = r if prev is None else prev + r
                oticks.extend(_vregs(r))
                for stage, i, span in (b_plan.get(n, []) if odd else []):
                    tk = oticks[-6 * span:]
                    if stage == 'l':
                        lm[i] = b_logits(brow, i, make_gate(tk, 64))
                        odead.setdefault(n + 7, []).append(lm[i][1])
                    elif stage == 's':
                        b_softmax(i, lm[i][0], lm[i][1], make_gate(tk, 16))
                    else:
                        b_values(i, make_gate(tk, 64))
                return r

            ks = 3 if odd else 1
            kw = SPLIT * E // ks
            l1 = ola[orows[0]:orows[0] + nrow, :]
            for j in range(8):
                r = None
                for k in range(ks):
                    r = out_dot(l1[:, k * kw:(k + 1) * kw], woa[j, k * kw // 2:(k + 1) * kw // 2, :], r)
                acc[j, 0:nrow, :] = r
                if H + j in after:
                    after[H + j]()
            l2 = olb[orows[0]:orows[0] + nrow, :]
            for j in range(8):
                res = out_dot(l2, woa[j, SPLIT * E // 2:, :], acc[j, 0:nrow, :]).astype(BF)
                cols = slice(j * 128, (j + 1) * 128)
                memb[:, cols] = res[0:MEM]
                if odd:
                    outa[pl.ds(brow, 8), cols] = res[8:16]
                    outa[pl.ds(brow + SEG, SEG), cols] = res[16:]
                else:
                    outa[pl.ds(brow + 8, XR), cols] = res[8:]
            if odd:
                out_copy(outa, brow, 0, D, 0).start()
                b_out(brow)

        def steps(i, carry):
            for u in range(U):
                step(i * U + u, u % 2)
            return carry

        lax.fori_loop(0, NSEG // U, steps, 0)

        pltpu.make_async_copy(outb, out.at[:, pl.ds(D, D)], sem_out.at[1]).wait()
        pltpu.make_async_copy(outa, out.at[:, pl.ds(0, D)], sem_out.at[0]).wait()

    pl.run_scoped(
        phase2,
        vm((PAIR, SPLIT * E), BF),
        vm((PAIR, (H - SPLIT) * E), BF),
        vm((S, D), BF),
        vm((S, D), BF),
    )


@jax.jit
def _run(A_x, A_mem0, A_Wq, A_Wk, A_Wv, A_Wo, B_x, B_wqkv, B_wo):
    assert A_x.shape == (1, S, D) and A_mem0.shape == (1, MEM, D)
    assert A_Wq.shape == (D, H, E) and A_Wo.shape == (H, E, D)
    assert B_x.shape == (1, S, D) and B_wqkv.shape == (D, 3 * D) and B_wo.shape == (D, D)
    vm = pltpu.VMEM
    dma = pltpu.SemaphoreType.DMA
    scratch = [
        vm((NSEG * XR, D), BF),
        vm((S, D), BF),
        vm((MEM, D), BF),
        vm((3 * H, D // 2, E), U32),
        vm((8, H * E // 2, 128), U32),
        vm((24, D // 2, 128), U32),
        vm((8, D // 2, 128), U32),
    ] + [vm((3, NS * NG, 64, E), BF)] * NB + [
        vm((8, 48, 128), F32),
        vm((PAIR, PAIR), F32),
        vm((8, BM, 128), F32),
        vm((8, HIST + BM, 128), F32),
        vm((8, HIST + BM, 128), F32),
        vm((WIN, BM, 128), F32),
        vm((BM, D), BF),
        vm((8, 128), U32),
        dma((NSEM,)), dma((2,)),
    ]
    out = pl.pallas_call(
        _kernel,
        out_shape=jax.ShapeDtypeStruct((S, 2 * D), BF),
        in_specs=[pl.BlockSpec(memory_space=pl.ANY)] * 9,
        out_specs=pl.BlockSpec(memory_space=pl.ANY),
        scratch_shapes=scratch,
        compiler_params=pltpu.CompilerParams(vmem_limit_bytes=120 * 1024 * 1024,
                                             disable_bounds_checks=True,
                                             disable_semaphore_checks=True),
    )(A_x.reshape(S, D), A_mem0.reshape(MEM, D), A_Wq, A_Wk, A_Wv, A_Wo.reshape(8, 512, D),
      B_x.reshape(S, D), B_wqkv, B_wo)
    return out.reshape(1, S, 2 * D)


def pallas_concat_heads__memory_aug_recurrent_mem_tr__sliding_local_dilated__prompt_kernel(
    A_x: jax.Array,
    A_mem0: jax.Array,
    A_Wq: jax.Array,
    A_Wk: jax.Array,
    A_Wv: jax.Array,
    A_Wo: jax.Array,
    A_seg_len,
    B_x: jax.Array,
    B_wqkv: jax.Array,
    B_wo: jax.Array,
):
    if isinstance(A_seg_len, int):
        assert A_seg_len == SEG
    return _run(A_x, A_mem0, A_Wq, A_Wk, A_Wv, A_Wo, B_x, B_wqkv, B_wo)
```

```python
import functools

import jax
import jax.numpy as jnp
from jax import lax
import jax.experimental.pallas as pl
import jax.experimental.pallas.tpu as pltpu

BF = jnp.bfloat16
F32 = jnp.float32
U32 = jnp.uint32

S = 2048
D = 1024
H = 32
E = 128
MEM = 8
SEG = 32
L = MEM + SEG
NG = L // 8
NSEG = S // SEG
WIN = 8
DIL = 2
NEG = -1000000000.0
LOG2E = 1.4426950408889634

PAIR = 2 * L
SPLIT = 24
U = 4
BM = 2 * SEG
FRONT = 32
VGROUPS = (1, 2)
VHEADS = 28

NCH = 12
RB = S // 4
MB = 128
NKP = 4
KP = D // NKP
NQ = 6
OW0 = 3
OA0 = NCH - 8
NTW = 4
WROWS = 3 * 4 * D

SEM_MEM, SEM_X, SEM_B0, SEM_XB, SEM_B, SEM_W, SEM_WOB, SEM_WOA, SEM_XA, NSEM = (
    0, 1, 5, 9, 13, 16, 26, 34, 35, 36)


def _rcp(d):
    r = pl.reciprocal(d, approx=True)
    return r * (2.0 - d * r)


def _dot(a, b):
    return jnp.dot(a, b, preferred_element_type=F32)


def _unpack(w):
    return pltpu.bitcast(w, BF)


def _lo_hi(a, b):
    lo = (a & U32(0xFFFF)) | (b << 16)
    hi = (a >> 16) | (b & U32(0xFFFF0000))
    return lo, hi


def _vregs(x):
    return [x[i:i + 8] for i in range(0, x.shape[0], 8)]


def _kernel(xa, mem0, wq, wk, wv, wo, xb, wqkv, wob, out,
            xaa, memb, wa, woa, wobp, bq, fill, pb, ob, zero, sem, sem_out):
    wsrc = (wq, wk, wv)
    a_scale = E ** -0.5
    b_scale = (D // H) ** -0.5

    xa_copy = pltpu.make_async_copy(xa, xaa, sem.at[SEM_XA])
    mem_copy = pltpu.make_async_copy(mem0, memb, sem.at[SEM_MEM])

    def nil(y):
        return pltpu.bitcast(y, U32) & zero[...]

    def tie_lhs(x, ys):
        if not ys:
            return x
        t = pltpu.bitcast(x[0:16, 0:128], U32)
        for y in ys:
            t = t | nil(y)
        top = jnp.concatenate([pltpu.bitcast(t, BF), x[0:16, 128:]], axis=1)
        return jnp.concatenate([top, x[16:]], axis=0)

    def make_gate(ticks, n):
        cnt = [0]
        cache = {}

        def gate(x):
            k = cnt[0] * len(ticks) // n
            cnt[0] += 1
            if k not in cache:
                cache[k] = nil(ticks[k])
            return pltpu.bitcast(pltpu.bitcast(x, U32) | cache[k], F32)
        return gate

    def b_logits(row, i, gate):
        q = [bq[cc, pl.ds(row + (FRONT + 8 * i), 8), :] for cc in range(8)]
        pos = row + 8 * i + lax.broadcasted_iota(jnp.int32, (8, 128), 0)
        logits = []
        for w in range(WIN):
            lo = FRONT + 8 * i - DIL * w
            t = None
            for cc in range(8):
                x = gate(bq[8 + cc, pl.ds(row + lo, 8), :]) * q[cc]
                t = x if t is None else t + x
            t = t + pltpu.roll(t, 64, 1)
            t = t + pltpu.roll(t, 32, 1)
            if 8 * i < DIL * w:
                t = jnp.where(pos >= DIL * w, t, NEG / b_scale)
            logits.append(t)
        return logits, functools.reduce(jnp.maximum, logits)

    def b_softmax(i, logits, m, gate):
        ex = [jnp.exp2((gate(t) - m) * (b_scale * LOG2E)) for t in logits]
        r = _rcp(functools.reduce(lambda a, b: a + b, ex))
        for w in range(WIN):
            pb[w, 8 * i:8 * i + 8, :] = gate(ex[w]) * r

    def b_values(row, i, gate, slot):
        p = [pb[w, 8 * i:8 * i + 8, :] for w in range(WIN)]
        for cc in range(8):
            t = None
            for w in range(WIN):
                lo = FRONT + 8 * i - DIL * w
                x = gate(bq[16 + cc, pl.ds(row + lo, 8), :]) * p[w]
                t = x if t is None else t + x
            ob[slot, 8 * i:8 * i + 8, cc * 128:(cc + 1) * 128] = t.astype(BF)

    def phase1(xbb, wst, bst, woast, wb, wobst, tw, tb, tob):
        def st(i):
            return i if isinstance(i, int) else 0

        def w_copies(i):
            lo, hi = 256 * NQ * i, 256 * NQ * (i + 1)
            cps = []
            while lo < hi:
                c = lo // D
                n = min(hi, (c + 1) * D) - lo
                cps.append(pltpu.make_async_copy(
                    wsrc[c // 4].at[pl.ds(lo - c * D, n), pl.ds((c % 4) * 8, 8), :], wst.at[pl.ds(lo, n)],
                    sem.at[SEM_W + i]))
                lo += n
            return cps

        def w_wait(i):
            v = wst.at[pl.ds(pl.multiple_of(256 * NQ * i, 256), 256 * NQ)]
            pltpu.make_async_copy(v, v, sem.at[SEM_W + i]).wait()

        def b0_copy(q):
            lo = q * KP if isinstance(q, int) else pl.multiple_of(q * KP, KP)
            return pltpu.make_async_copy(
                wqkv.at[pl.ds(st(q) * KP, KP), pl.ds(0, D)], bst.at[0, pl.ds(lo, KP)], sem.at[SEM_B0 + q])

        def b_copy(p):
            return pltpu.make_async_copy(wqkv.at[:, pl.ds(st(p) * D, D)], bst.at[p], sem.at[SEM_B + p])

        def x0_copy(q):
            return pltpu.make_async_copy(
                xb.at[pl.ds(0, RB), pl.ds(st(q) * KP, KP)], xbb.at[0, q], sem.at[SEM_X + q])

        def xb_copies(b):
            return [pltpu.make_async_copy(
                xb.at[pl.ds(b * RB, RB), pl.ds(q * KP, KP)], xbb.at[b, q], sem.at[SEM_XB + b])
                for q in range(NKP)]

        def xb_wait(b):
            pltpu.make_async_copy(xbb.at[b], xbb.at[b], sem.at[SEM_XB + b]).wait()

        def wob_copy(j):
            return pltpu.make_async_copy(
                wob.at[:, pl.ds(st(j) * 128, 128)], wobst.at[j], sem.at[SEM_WOB + j])

        woa_copy = pltpu.make_async_copy(wo, woast, sem.at[SEM_WOA])

        for q in range(NKP):
            b0_copy(q).start()
            x0_copy(q).start()
        for c in range(1, NCH):
            if c < 4:
                for cp in xb_copies(c):
                    cp.start()
            if OW0 <= c < NCH - 1:
                for cp in w_copies(c - OW0):
                    cp.start()
            if c in (3, 7):
                b_copy(c // 4 + 1).start()
            if c >= OA0:
                wob_copy(c - OA0).start()
        woa_copy.start()
        mem_copy.start()
        xa_copy.start()

        def zero_fill(i, carry):
            r = pl.multiple_of(i * 16, 16)
            wst[pl.ds(WROWS + r, 16)] = jnp.zeros((16, 8, E), BF)
            wobst[8, pl.ds(4 * r, 64), :] = jnp.zeros((64, 128), BF)
            return carry

        lax.fori_loop(0, 16, zero_fill, 0)

        ri = lax.broadcasted_iota(jnp.int32, (PAIR, PAIR), 0)
        ci = lax.broadcasted_iota(jnp.int32, (PAIR, PAIR), 1)
        rb = (ri >> 3) & 1
        cb = (ci >> 3) & 1
        rl = ((ri >> 4) << 3) | (ri & 7)
        cl = ((ci >> 4) << 3) | (ci & 7)
        allowed = (rl < MEM) | (rl >= cl)
        fill[...] = jnp.where(rb == cb, jnp.where(allowed, 0.0, NEG / a_scale), -jnp.inf).astype(F32)
        bq[8:24, FRONT - 16:FRONT, :] = jnp.zeros((16, 16, 128), F32)
        zero[...] = jnp.zeros(zero.shape, U32)

        def zero_acc(i, carry):
            for u in range(32):
                row = FRONT + (u // 8) * MB + pl.multiple_of(i * 8, 8)
                bq[u % 8, pl.ds(row, 8), :] = jnp.zeros((8, E), F32)
            return carry

        lax.fori_loop(0, 16, zero_acc, 0)

        def gated(x, gate):
            return jnp.concatenate([v | gate() for v in _vregs(x)], axis=0) if gate else x

        def relayout1(src, blk, slot, gate):
            v = wst[pl.ds(src + blk * 16, 16)]
            v = pltpu.bitcast(v.reshape(128, 128), U32)
            for dp in range(8):
                tw[slot, 9 * dp:9 * dp + 8, :] = v[8 * dp:8 * dp + 8] | gate()

        def relayout2(base, row0, blk, slot, gate):
            row = row0 + blk * 8
            for j in range(4):
                g = gate()
                a = tw[slot, pl.ds(j, 8, stride=9), :] | g
                b = tw[slot, pl.ds(4 + j, 8, stride=9), :] | g
                lo, hi = _lo_hi(a, b)
                wa[base + 2 * j, pl.ds(row, 8), :] = lo
                wa[base + 2 * j + 1, pl.ds(row, 8), :] = hi

        def relayout_jobs(pieces):
            items = [(p, blk) for p in pieces for blk in range(16)]
            jobs = []
            for k in range(len(items) + 1):
                if k < len(items):
                    (src, _, _), blk = items[k]
                    jobs.append((8, functools.partial(relayout1, src, blk, k % NTW)))
                if k > 0:
                    (_, base, row0), blk = items[k - 1]
                    jobs.append((4, functools.partial(relayout2, base, row0, blk, (k - 1) % NTW)))
            return jobs

        def b_prep1(src, row, e, cc, gate=None):
            x = pltpu.bitcast(bst[src, pl.ds(row, 256), cc * 128:(cc + 1) * 128], U32)
            x = gated(x, gate).T
            for hl in range(4):
                h = 4 * cc + hl
                tb[e, 33 * h:33 * h + 32, :] = x[32 * hl:32 * hl + 32]

        def b_prep2(base, row, e, cc, gate=None):
            y = jnp.concatenate(
                [tb[e, pl.ds(4 * cc + dl + 33 * 8 * g, 8, stride=33), :] for dl in range(4) for g in range(4)],
                axis=0)
            wb[base + cc, pl.ds(row, 128), :] = gated(y, gate).T

        def wob_prep1(src, g, gate):
            v = pltpu.bitcast(wobst[src, g * 512:(g + 1) * 512, :], U32)
            v = gated(v, gate)
            for hp in range(8):
                tob[g, 33 * hp:33 * hp + 32, :] = v[32 * hp:32 * hp + 32]

        def wob_prep2(j, g, gate):
            for dp in range(16):
                z = gate()
                lo, hi = _lo_hi(tob[g, pl.ds(dp, 8, stride=33), :] | z,
                                tob[g, pl.ds(16 + dp, 8, stride=33), :] | z)
                wobp[j, (2 * dp) * 16 + 8 * g:(2 * dp) * 16 + 8 * g + 8, :] = lo
                wobp[j, (2 * dp + 1) * 16 + 8 * g:(2 * dp + 1) * 16 + 8 * g + 8, :] = hi

        def wob_jobs(src, j):
            return ([(32, functools.partial(wob_prep1, src, g)) for g in range(2)]
                    + [(16, functools.partial(wob_prep2, j, g)) for g in range(2)])

        def woa_prep(j, q, gate):
            v = pltpu.bitcast(woast[j, :, q * 128:(q + 1) * 128], U32)
            woa[q, j * 256:(j + 1) * 256, :] = gated(v, gate)

        def run_chunk(b, base, hook=None):
            ticks = []
            row = b * RB if isinstance(b, int) else pl.multiple_of(b * RB, RB)
            dead = {}
            for u in range(16):
                cc, mb = u % 8, u // 8
                rows = slice(mb * 2 * MB, (mb + 1) * 2 * MB)
                lhs = jnp.concatenate([xbb[b, q, rows, :] for q in range(NKP)], axis=1)
                lhs = tie_lhs(lhs, dead.get(2 * u, []) + dead.get(2 * u + 1, []))
                r1 = _dot(lhs[:, :D // 2], _unpack(wb[base + cc, :D // 4, :]))
                r2 = r1 + _dot(lhs[:, D // 2:], _unpack(wb[base + cc, D // 4:, :]))
                bq[base + cc, pl.ds(row + (FRONT + mb * 2 * MB), 2 * MB), :] = r2
                for k, r in enumerate((r1, r2)):
                    ticks += _vregs(r)[::2]
                    if hook:
                        hook(2 * u + k, ticks, dead)
            return ticks

        def run_piece(q, wrow, row0):
            ticks = []
            for u in range(16):
                cc, mb = u % 8, u // 8
                r = _dot(xbb[0, q, pl.ds(row0 + mb * MB, MB), :], _unpack(wb[cc, pl.ds(wrow, KP // 2), :]))
                r = r + bq[cc, pl.ds(row0 + (FRONT + mb * MB), MB), :]
                bq[cc, pl.ds(row0 + (FRONT + mb * MB), MB), :] = r
                ticks += _vregs(r)
            return ticks

        def run_jobs(ticks, spare, jobs, free=0):
            ticks = ticks[:len(ticks) - 16 * spare]
            total = sum(n for n, _ in jobs)
            z = zero[...]
            cache = {}
            cnt = [0]

            def gate():
                k = (cnt[0] - free) * len(ticks) // (total - free)
                cnt[0] += 1
                if k < 0:
                    return z
                if k not in cache:
                    cache[k] = pltpu.bitcast(ticks[k], U32) & z
                return cache[k]

            for _, fn in jobs:
                fn(gate=gate)

        def interleave(*lists):
            items = []
            for l in lists:
                items += [((i + 0.5) / len(l), x) for i, x in enumerate(l)]
            items.sort(key=lambda z: z[0])
            return [x for _, x in items]

        def piece(q, carry):
            b0_copy(q + 1).wait()
            x0_copy(q + 1).wait()
            wrow = pl.multiple_of(q * (KP // 2), KP // 2)
            ticks = run_piece(q, wrow, 256)
            run_jobs(ticks, 4,
                     [(16, functools.partial(b_prep1, 0, 2 * wrow + KP, 0, cc)) for cc in range(8)]
                     + [(16, functools.partial(b_prep2, 0, wrow + KP // 2, 0, cc)) for cc in range(8)],
                     free=60)
            run_piece(q + 1, wrow + KP // 2, 0)
            return carry

        def ends(k, carry):
            run_piece(k * (NKP - 1), pl.multiple_of(k * ((NKP - 1) * KP // 2), 128),
                      pl.multiple_of(k * 256, 256))

            @pl.when(k == 0)
            def _():
                lax.fori_loop(0, NKP - 1, piece, 0)

            return carry

        def chunk(c, carry):
            @pl.when(c < 4)
            def _():
                xb_wait(c)

            @pl.when(c >= OW0)
            def _():
                w_wait(c - OW0)

            @pl.when((c & 3) == 3)
            def _():
                b_copy((c >> 2) + 1).wait()

            @pl.when(c >= OA0)
            def _():
                wob_copy(c - OA0).wait()

            p8 = (c >> 2) * 8
            ticks = run_chunk(c & 3, p8)
            pieces = []
            for k in range(NQ):
                g = jnp.maximum(NQ * (c - OW0), 0) + k
                src = pl.multiple_of(jnp.where(c >= OW0, g * 256, WROWS), 256)
                pieces.append((src, (g >> 2) * 8, pl.multiple_of((g & 3) * 128, 128)))
            ja = jnp.maximum(c - OA0, 0)
            nxt = (c + 1) >> 2
            run_jobs(ticks, 2, interleave(
                relayout_jobs(pieces),
                wob_jobs(jnp.where(c >= OA0, ja, 8), ja),
                [(16, functools.partial(f, j, row, e % 2, cc))
                 for e in range(4) for f, j, row in ((b_prep1, nxt, e * 256), (b_prep2, p8 + 8, e * 128))
                 for cc in range(8)]))
            return carry

        b0_copy(0).wait()
        for cc in range(8):
            b_prep1(0, 0, 0, cc)
        for cc in range(8):
            b_prep2(0, 0, 0, cc)
        x0_copy(0).wait()
        lax.fori_loop(0, 2, ends, 0)
        lax.fori_loop(1, NCH - 1, chunk, 0)

        wob_copy(7).wait()
        woa_copy.wait()
        lm = {}

        def first_attention(u, ticks, dead):
            for i in range(8):
                if u == 1 + 2 * i:
                    lm[i] = b_logits(0, i, make_gate(ticks[-32:], 64))
                    dead.setdefault(u + 4, []).append(lm[i][1])
                if u == 4 + 2 * i:
                    b_softmax(i, lm[i][0], lm[i][1], make_gate(ticks[-16:], 16))
                if u == 14 + 2 * i:
                    b_values(0, i, make_gate(ticks[-32:], 64), 0)

        ticks = run_chunk(3, 16, first_attention)
        run_jobs(ticks, 2, interleave(
            wob_jobs(7, 7),
            [(32, functools.partial(woa_prep, j, q)) for j in range(8) for q in range(8)]))

    vm = pltpu.VMEM
    pl.run_scoped(
        phase1,
        vm((S // RB, NKP, RB, KP), BF),
        vm((WROWS + 256, 8, E), BF),
        vm((3, D, D), BF),
        vm((8, 512, D), BF),
        vm((32, D // 2, 128), U32),
        vm((9, D, 128), BF),
        vm((NTW, 80, 128), U32),
        vm((2, 33 * H + 40, 128), U32),
        vm((2, 33 * 8 + 32, 128), U32),
    )
    mem_copy.wait()
    xa_copy.wait()

    def phase2(qkv, acc, ola, olb, outa, outb):
        def out_copy(buf, row, c0, nc, half):
            return pltpu.make_async_copy(
                buf.at[pl.ds(row, BM), pl.ds(c0, nc)], out.at[pl.ds(row, BM), pl.ds(half * D + c0, nc)],
                sem_out.at[half])

        b_plan = {1: [('l', 3, 2)], 3: [('l', 4, 2)], 6: [('s', 3, 1), ('l', 5, 2)],
                  8: [('s', 4, 1), ('l', 6, 2)], 11: [('s', 5, 1), ('l', 7, 2)], 13: [('s', 6, 1)],
                  15: [('v', 0, 2)], 16: [('s', 7, 1)], 17: [('v', 1, 2)], 19: [('v', 2, 2)],
                  21: [('v', 3, 2)], 23: [('v', 4, 2)], 25: [('v', 5, 2)], 27: [('v', 6, 2)],
                  30: [('v', 7, 2)]}
        b_early = 3
        b_ticks = []

        def step(s, odd, slot_b):
            next_row = pl.multiple_of(jnp.minimum((s + 1) * SEG, S - BM), BM) if odd else None
            row = pl.multiple_of((s - odd) * SEG, BM)
            lhs = jnp.concatenate([memb[...], xaa[pl.ds(row + odd * 40, 24 if odd else 40), :]], axis=0)
            planes = (5, 7, 8, 9) if odd else (0, 1, 2, 3, 4, 6)
            plane0 = 5 * odd
            orows = (32, 48, 56, 64, 72) if odd else (0, 40, 8, 16, 24)
            nrow = 48 if odd else 32
            ticks = []
            tpd = len(planes)
            dead = {}
            lm = {}

            def mxu_groups(p):
                return [i for i in range(NG) if odd or 2 * p >= VHEADS or i not in VGROUPS]

            def proj(h, t):
                r32 = _dot(tie_lhs(lhs, dead.get(3 * h + t)), _unpack(wa[t * H + h]))
                ticks.extend(_vregs(r32))
                r = r32.astype(BF)
                for i, pn in enumerate(planes):
                    qkv[t, pn, h * 8:h * 8 + 8, :] = r[8 * i:8 * i + 8]

            def o_store(h, i, o):
                ol, hi = (ola, h) if h < SPLIT else (olb, h - SPLIT)
                ol[orows[i]:orows[i] + 8, hi * E:(hi + 1) * E] = o

            probs = {}

            def pair(t, p, groups=range(NG)):
                return jnp.concatenate([qkv[t, plane0 + i, 16 * p:16 * p + 16, :] for i in groups], axis=0)

            def scores(p, n):
                groups = mxu_groups(p)
                y = nil(ticks[(6 * p + 6) * tpd - 1])
                k = jnp.concatenate([v | y for v in _vregs(pltpu.bitcast(pair(1, p), U32))], axis=0)
                sc = lax.dot_general(pair(0, p, groups), _unpack(k), (((1,), (1,)), ((), ())),
                                     preferred_element_type=F32)
                fl = jnp.concatenate([fill[16 * i:16 * i + 16, :] for i in groups], axis=0)
                sc = jnp.where(fl == 0.0, sc, fl)
                e = jnp.exp2((sc - jnp.max(sc, axis=1, keepdims=True)) * (a_scale * LOG2E))
                probs[p] = (e * _rcp(jnp.sum(e, axis=1, keepdims=True))).astype(BF)

            def values(p, n):
                o = _dot(probs.pop(p), pair(2, p)).astype(BF)
                for k, i in enumerate(mxu_groups(p)):
                    for hh in range(2):
                        o_store(2 * p + hh, i, o[16 * k + 8 * hh:16 * k + 8 * hh + 8])

            vstate = {}
            nkg = max(VGROUPS) + 1

            def group(t, h, i):
                return qkv[t, plane0 + i, h * 8:h * 8 + 8, :].astype(F32)

            def v_scores(h, n):
                gate = make_gate(ticks[-3 * tpd:], nkg)
                sub = lax.broadcasted_iota(jnp.int32, (8, 1), 0)
                q = {i: group(0, h, i) * (a_scale * LOG2E) for i in VGROUPS}
                sc = {i: [] for i in VGROUPS}
                for kg in range(nkg):
                    k = gate(group(1, h, kg))
                    for j in range(8):
                        kj = jnp.broadcast_to(k[j:j + 1, :], (8, E))
                        for i in VGROUPS:
                            if kg <= i:
                                x = jnp.sum(kj * q[i], axis=1, keepdims=True)
                                if kg == i and j > 0:
                                    x = jnp.where(sub >= j, x, NEG * LOG2E)
                                sc[i].append(jnp.broadcast_to(x, (8, E)))
                m = {i: functools.reduce(jnp.maximum, sc[i]) for i in VGROUPS}
                dead.setdefault(n + 5, []).extend(m.values())
                vstate[h] = (sc, m)

            def v_values(h, n):
                gate = make_gate(ticks[-3 * tpd:], sum(i + 1 for i in VGROUPS))
                sc, m = vstate.pop(h)
                den = {}
                o = {}
                for kg in range(nkg):
                    v = group(2, h, kg)
                    mg = {i: gate(m[i]) for i in VGROUPS if kg <= i}
                    for j in range(8):
                        vj = jnp.broadcast_to(v[j:j + 1, :], (8, E))
                        for i in mg:
                            e = jnp.exp2(sc[i][8 * kg + j] - mg[i])
                            den[i] = den[i] + e if i in den else e
                            x = e * vj
                            o[i] = o[i] + x if i in o else x
                for i in VGROUPS:
                    o_store(h, i, (o[i] * _rcp(den[i])).astype(BF))

            def early_logits(_, n):
                gate = make_gate(b_ticks + ticks, 64 * b_early)
                for i in range(b_early):
                    lm[i] = b_logits(next_row, i, gate)
                    dead.setdefault(6 + 2 * i, []).append(lm[i][1])

            def early_softmax(i, n):
                b_softmax(i, lm[i][0], lm[i][1], make_gate(ticks[-8:], 16))

            events = {}

            def at(n, f, a):
                events.setdefault(n, []).append(functools.partial(f, a, n))

            for p in range(H // 2):
                at(6 * p + 8, scores, p)
                at(6 * p + (17 if odd else 15), values, p)
            if odd:
                at(0, early_logits, 0)
                for i in range(b_early):
                    at(4 + 2 * i, early_softmax, i)
            else:
                for h in range(VHEADS):
                    at(3 * h + 5, v_scores, h)
                    at(3 * h + 10, v_values, h)
            assert 6 * (SPLIT // 2 - 1) + 17 < 3 * H and 3 * (VHEADS - 1) + 10 < 3 * H - 1

            for h in range(H):
                for t in range(3):
                    proj(h, t)
                    for f in events.get(3 * h + t, []):
                        f()

            oticks = []
            odead = {}
            count = [0]

            def out_dot(l, k0, k1, j, prev):
                n = count[0]
                count[0] += 1
                r = _dot(tie_lhs(l, odead.get(n)), _unpack(woa[j, k0 // 2:k1 // 2, :]))
                r = r if prev is None else prev + r
                oticks.extend(_vregs(r))
                for stage, i, span in (b_plan.get(n, []) if odd else []):
                    tk = oticks[-6 * span:]
                    if stage == 'l':
                        lm[i] = b_logits(next_row, i, make_gate(tk, 64))
                        odead.setdefault(n + 7, []).append(lm[i][1])
                    elif stage == 's':
                        b_softmax(i, lm[i][0], lm[i][1], make_gate(tk, 16))
                    else:
                        b_values(next_row, i, make_gate(tk, 64), 1 - slot_b)
                return r

            ks = 3 if odd else 1
            kw = SPLIT * E // ks
            per = 3 if odd else 2
            l1 = ola[orows[0]:orows[0] + nrow, :]
            for j in range(8):
                r = None
                for k in range(ks):
                    r = out_dot(l1[:, k * kw:(k + 1) * kw], k * kw, (k + 1) * kw, j, r)
                acc[j, 0:nrow, :] = r
                for n in range(3 * H + per * j, 3 * H + per * (j + 1)):
                    for f in events.get(n, []):
                        f()
            assert max(events) < 3 * H + 8 * per
            l2 = olb[orows[0]:orows[0] + nrow, :]
            for j in range(8):
                res = out_dot(l2, SPLIT * E, H * E, j, acc[j, 0:nrow, :]).astype(BF)
                cols = slice(j * 128, (j + 1) * 128)
                memb[:, cols] = res[0:MEM]
                if odd:
                    outa[pl.ds(row, 8), cols] = res[8:16]
                    outa[pl.ds(row + SEG, SEG), cols] = res[16:]
                else:
                    outa[pl.ds(row + 8, 24), cols] = res[8:]
            if odd:
                out_copy(outa, row, 0, D, 0).start()

            o = ob[slot_b]
            del b_ticks[:]
            for j in range(4 * odd, 4 * odd + 4):
                r = _dot(o, _unpack(wobp[j]))
                b_ticks.extend(_vregs(r))
                outb[pl.ds(row, BM), j * 128:(j + 1) * 128] = r.astype(BF)
                if j % 2 == 1:
                    out_copy(outb, row, (j - 1) * 128, 256, 1).start()

        def steps(i, carry):
            for u in range(U):
                step(i * U + u, u % 2, (u // 2) % 2)
            return carry

        lax.fori_loop(0, NSEG // U, steps, 0)

        pltpu.make_async_copy(outb, out.at[:, pl.ds(D, D)], sem_out.at[1]).wait()
        pltpu.make_async_copy(outa, out.at[:, pl.ds(0, D)], sem_out.at[0]).wait()

    pl.run_scoped(
        phase2,
        vm((3, 2 * NG, H * 8, E), BF),
        vm((8, 48, 128), F32),
        vm((PAIR, SPLIT * E), BF),
        vm((PAIR, (H - SPLIT) * E), BF),
        vm((S, D), BF),
        vm((S, D), BF),
    )


@jax.jit
def _run(A_x, A_mem0, A_Wq, A_Wk, A_Wv, A_Wo, B_x, B_wqkv, B_wo):
    assert A_x.shape == (1, S, D) and A_mem0.shape == (1, MEM, D)
    assert A_Wq.shape == (D, H, E) and A_Wo.shape == (H, E, D)
    assert B_x.shape == (1, S, D) and B_wqkv.shape == (D, 3 * D) and B_wo.shape == (D, D)
    vm = pltpu.VMEM
    dma = pltpu.SemaphoreType.DMA
    scratch = [
        vm((S, D), BF),
        vm((MEM, D), BF),
        vm((3 * H, D // 2, E), U32),
        vm((8, H * E // 2, 128), U32),
        vm((8, D // 2, 128), U32),
        vm((24, S + FRONT, 128), F32),
        vm((PAIR, PAIR), F32),
        vm((WIN, BM, 128), F32),
        vm((2, BM, D), BF),
        vm((8, 128), U32),
        dma((NSEM,)), dma((2,)),
    ]
    out = pl.pallas_call(
        _kernel,
        out_shape=jax.ShapeDtypeStruct((S, 2 * D), BF),
        in_specs=[pl.BlockSpec(memory_space=pl.ANY)] * 9,
        out_specs=pl.BlockSpec(memory_space=pl.ANY),
        scratch_shapes=scratch,
        compiler_params=pltpu.CompilerParams(vmem_limit_bytes=120 * 1024 * 1024,
                                             disable_bounds_checks=True,
                                             disable_semaphore_checks=True),
    )(A_x.reshape(S, D), A_mem0.reshape(MEM, D), A_Wq, A_Wk, A_Wv, A_Wo.reshape(8, 512, D),
      B_x.reshape(S, D), B_wqkv, B_wo)
    return out.reshape(1, S, 2 * D)


def pallas_concat_heads__memory_aug_recurrent_mem_tr__sliding_local_dilated__prompt_kernel(
    A_x: jax.Array,
    A_mem0: jax.Array,
    A_Wq: jax.Array,
    A_Wk: jax.Array,
    A_Wv: jax.Array,
    A_Wo: jax.Array,
    A_seg_len,
    B_x: jax.Array,
    B_wqkv: jax.Array,
    B_wo: jax.Array,
):
    if isinstance(A_seg_len, int):
        assert A_seg_len == SEG
    return _run(A_x, A_mem0, A_Wq, A_Wk, A_Wv, A_Wo, B_x, B_wqkv, B_wo)
```

```python
import functools

import jax
import jax.numpy as jnp
from jax import lax
import jax.experimental.pallas as pl
import jax.experimental.pallas.tpu as pltpu

BF = jnp.bfloat16
F32 = jnp.float32
U32 = jnp.uint32

S = 2048
D = 1024
H = 32
E = 128
MEM = 8
SEG = 32
L = MEM + SEG
NG = L // 8
NSEG = S // SEG
WIN = 8
DIL = 2
NEG = -1000000000.0
LOG2E = 1.4426950408889634

PAIR = 2 * L
SPLIT = 24
U = 4
BM = 2 * SEG
FRONT = 32
VH_EVEN = 28
VH_ODD = 16

NCH = 12
RB = S // 4
MB = 128
NKP = 4
KP = D // NKP
NQ = 6
OW0 = 3
OA0 = NCH - 8
NTW = 4
WROWS = 3 * 4 * D

SEM_MEM, SEM_X, SEM_B0, SEM_XB, SEM_B, SEM_W, SEM_WOB, SEM_WOA, SEM_XA, NSEM = (
    0, 1, 5, 9, 13, 16, 26, 34, 35, 36)


def _rcp(d):
    r = pl.reciprocal(d, approx=True)
    return r * (2.0 - d * r)


def _dot(a, b):
    return jnp.dot(a, b, preferred_element_type=F32)


def _unpack(w):
    return pltpu.bitcast(w, BF)


def _lo_hi(a, b):
    lo = (a & U32(0xFFFF)) | (b << 16)
    hi = (a >> 16) | (b & U32(0xFFFF0000))
    return lo, hi


def _vregs(x):
    return [x[i:i + 8] for i in range(0, x.shape[0], 8)]


def _kernel(xa, mem0, wq, wk, wv, wo, xb, wqkv, wob, out,
            xaa, memb, wa, woa, wobp, bq, fill, pb, ob, zero, sem, sem_out):
    wsrc = (wq, wk, wv)
    a_scale = E ** -0.5
    b_scale = (D // H) ** -0.5

    xa_copy = pltpu.make_async_copy(xa, xaa, sem.at[SEM_XA])
    mem_copy = pltpu.make_async_copy(mem0, memb, sem.at[SEM_MEM])

    def nil(y):
        return pltpu.bitcast(y, U32) & zero[...]

    def tie_lhs(x, ys):
        if not ys:
            return x
        t = pltpu.bitcast(x[0:16, 0:128], U32)
        for y in ys:
            t = t | nil(y)
        top = jnp.concatenate([pltpu.bitcast(t, BF), x[0:16, 128:]], axis=1)
        return jnp.concatenate([top, x[16:]], axis=0)

    def make_gate(ticks, n):
        cnt = [0]
        cache = {}

        def gate(x):
            k = cnt[0] * len(ticks) // n
            cnt[0] += 1
            if k not in cache:
                cache[k] = nil(ticks[k])
            return pltpu.bitcast(pltpu.bitcast(x, U32) | cache[k], F32)
        return gate

    def b_logits(row, i, gate):
        q = [bq[cc, pl.ds(row + (FRONT + 8 * i), 8), :] for cc in range(8)]
        pos = row + 8 * i + lax.broadcasted_iota(jnp.int32, (8, 128), 0)
        logits = []
        for w in range(WIN):
            lo = FRONT + 8 * i - DIL * w
            t = None
            for cc in range(8):
                x = gate(bq[8 + cc, pl.ds(row + lo, 8), :]) * q[cc]
                t = x if t is None else t + x
            t = t + pltpu.roll(t, 64, 1)
            t = t + pltpu.roll(t, 32, 1)
            if 8 * i < DIL * w:
                t = jnp.where(pos >= DIL * w, t, NEG / b_scale)
            logits.append(t)
        return logits, functools.reduce(jnp.maximum, logits)

    def b_softmax(i, logits, m, gate):
        ex = [jnp.exp2((gate(t) - m) * (b_scale * LOG2E)) for t in logits]
        r = _rcp(functools.reduce(lambda a, b: a + b, ex))
        for w in range(WIN):
            pb[w, 8 * i:8 * i + 8, :] = gate(ex[w]) * r

    def b_values(row, i, gate, slot):
        p = [pb[w, 8 * i:8 * i + 8, :] for w in range(WIN)]
        for cc in range(8):
            t = None
            for w in range(WIN):
                lo = FRONT + 8 * i - DIL * w
                x = gate(bq[16 + cc, pl.ds(row + lo, 8), :]) * p[w]
                t = x if t is None else t + x
            ob[slot, 8 * i:8 * i + 8, cc * 128:(cc + 1) * 128] = t.astype(BF)

    def phase1(xbb, wst, bst, woast, wb, wobst, tw, tb, tob):
        def st(i):
            return i if isinstance(i, int) else 0

        def w_copies(i):
            lo, hi = 256 * NQ * i, 256 * NQ * (i + 1)
            cps = []
            while lo < hi:
                c = lo // D
                n = min(hi, (c + 1) * D) - lo
                cps.append(pltpu.make_async_copy(
                    wsrc[c // 4].at[pl.ds(lo - c * D, n), pl.ds((c % 4) * 8, 8), :], wst.at[pl.ds(lo, n)],
                    sem.at[SEM_W + i]))
                lo += n
            return cps

        def w_wait(i):
            v = wst.at[pl.ds(pl.multiple_of(256 * NQ * i, 256), 256 * NQ)]
            pltpu.make_async_copy(v, v, sem.at[SEM_W + i]).wait()

        def b0_copy(q):
            lo = q * KP if isinstance(q, int) else pl.multiple_of(q * KP, KP)
            return pltpu.make_async_copy(
                wqkv.at[pl.ds(st(q) * KP, KP), pl.ds(0, D)], bst.at[0, pl.ds(lo, KP)], sem.at[SEM_B0 + q])

        def b_copy(p):
            return pltpu.make_async_copy(wqkv.at[:, pl.ds(st(p) * D, D)], bst.at[p], sem.at[SEM_B + p])

        def x0_copy(q):
            return pltpu.make_async_copy(
                xb.at[pl.ds(0, RB), pl.ds(st(q) * KP, KP)], xbb.at[0, q], sem.at[SEM_X + q])

        def xb_copies(b):
            return [pltpu.make_async_copy(
                xb.at[pl.ds(b * RB, RB), pl.ds(q * KP, KP)], xbb.at[b, q], sem.at[SEM_XB + b])
                for q in range(NKP)]

        def xb_wait(b):
            pltpu.make_async_copy(xbb.at[b], xbb.at[b], sem.at[SEM_XB + b]).wait()

        def wob_copy(j):
            return pltpu.make_async_copy(
                wob.at[:, pl.ds(st(j) * 128, 128)], wobst.at[j], sem.at[SEM_WOB + j])

        woa_copy = pltpu.make_async_copy(wo, woast, sem.at[SEM_WOA])

        for q in range(NKP):
            b0_copy(q).start()
            x0_copy(q).start()
        for c in range(1, NCH):
            if c < 4:
                for cp in xb_copies(c):
                    cp.start()
            if OW0 <= c < NCH - 1:
                for cp in w_copies(c - OW0):
                    cp.start()
            if c in (3, 7):
                b_copy(c // 4 + 1).start()
            if c >= OA0:
                wob_copy(c - OA0).start()
        woa_copy.start()
        mem_copy.start()
        xa_copy.start()

        def zero_fill(i, carry):
            r = pl.multiple_of(i * 16, 16)
            wst[pl.ds(WROWS + r, 16)] = jnp.zeros((16, 8, E), BF)
            wobst[8, pl.ds(4 * r, 64), :] = jnp.zeros((64, 128), BF)
            return carry

        lax.fori_loop(0, 16, zero_fill, 0)

        ri = lax.broadcasted_iota(jnp.int32, (PAIR, PAIR), 0)
        ci = lax.broadcasted_iota(jnp.int32, (PAIR, PAIR), 1)
        rb = (ri >> 3) & 1
        cb = (ci >> 3) & 1
        rl = ((ri >> 4) << 3) | (ri & 7)
        cl = ((ci >> 4) << 3) | (ci & 7)
        allowed = (rl < MEM) | (rl >= cl)
        fill[...] = jnp.where(rb == cb, jnp.where(allowed, 0.0, NEG / a_scale), -jnp.inf).astype(F32)
        bq[8:24, FRONT - 16:FRONT, :] = jnp.zeros((16, 16, 128), F32)
        zero[...] = jnp.zeros(zero.shape, U32)

        def zero_acc(i, carry):
            for u in range(32):
                row = FRONT + (u // 8) * MB + pl.multiple_of(i * 8, 8)
                bq[u % 8, pl.ds(row, 8), :] = jnp.zeros((8, E), F32)
            return carry

        lax.fori_loop(0, 16, zero_acc, 0)

        def gated(x, gate):
            return jnp.concatenate([v | gate() for v in _vregs(x)], axis=0) if gate else x

        def relayout1(src, blk, slot, gate):
            v = wst[pl.ds(src + blk * 16, 16)]
            v = pltpu.bitcast(v.reshape(128, 128), U32)
            for dp in range(8):
                tw[slot, 9 * dp:9 * dp + 8, :] = v[8 * dp:8 * dp + 8] | gate()

        def relayout2(base, row0, blk, slot, gate):
            row = row0 + blk * 8
            for j in range(4):
                g = gate()
                a = tw[slot, pl.ds(j, 8, stride=9), :] | g
                b = tw[slot, pl.ds(4 + j, 8, stride=9), :] | g
                lo, hi = _lo_hi(a, b)
                wa[base + 2 * j, pl.ds(row, 8), :] = lo
                wa[base + 2 * j + 1, pl.ds(row, 8), :] = hi

        def relayout_jobs(pieces):
            items = [(p, blk) for p in pieces for blk in range(16)]
            jobs = []
            for k in range(len(items) + 1):
                if k < len(items):
                    (src, _, _), blk = items[k]
                    jobs.append((8, functools.partial(relayout1, src, blk, k % NTW)))
                if k > 0:
                    (_, base, row0), blk = items[k - 1]
                    jobs.append((4, functools.partial(relayout2, base, row0, blk, (k - 1) % NTW)))
            return jobs

        def b_prep1(src, row, e, cc, gate=None):
            x = pltpu.bitcast(bst[src, pl.ds(row, 256), cc * 128:(cc + 1) * 128], U32)
            x = gated(x, gate).T
            for hl in range(4):
                h = 4 * cc + hl
                tb[e, 33 * h:33 * h + 32, :] = x[32 * hl:32 * hl + 32]

        def b_prep2(base, row, e, cc, gate=None):
            y = jnp.concatenate(
                [tb[e, pl.ds(4 * cc + dl + 33 * 8 * g, 8, stride=33), :] for dl in range(4) for g in range(4)],
                axis=0)
            wb[base + cc, pl.ds(row, 128), :] = gated(y, gate).T

        def wob_prep1(src, g, gate):
            v = pltpu.bitcast(wobst[src, g * 512:(g + 1) * 512, :], U32)
            v = gated(v, gate)
            for hp in range(8):
                tob[g, 33 * hp:33 * hp + 32, :] = v[32 * hp:32 * hp + 32]

        def wob_prep2(j, g, gate):
            for dp in range(16):
                z = gate()
                lo, hi = _lo_hi(tob[g, pl.ds(dp, 8, stride=33), :] | z,
                                tob[g, pl.ds(16 + dp, 8, stride=33), :] | z)
                wobp[j, (2 * dp) * 16 + 8 * g:(2 * dp) * 16 + 8 * g + 8, :] = lo
                wobp[j, (2 * dp + 1) * 16 + 8 * g:(2 * dp + 1) * 16 + 8 * g + 8, :] = hi

        def wob_jobs(src, j):
            return ([(32, functools.partial(wob_prep1, src, g)) for g in range(2)]
                    + [(16, functools.partial(wob_prep2, j, g)) for g in range(2)])

        def woa_prep(j, q, gate):
            v = pltpu.bitcast(woast[j, :, q * 128:(q + 1) * 128], U32)
            woa[q, j * 256:(j + 1) * 256, :] = gated(v, gate)

        def run_chunk(b, base, hook=None):
            ticks = []
            row = b * RB if isinstance(b, int) else pl.multiple_of(b * RB, RB)
            dead = {}
            for u in range(16):
                cc, mb = u % 8, u // 8
                rows = slice(mb * 2 * MB, (mb + 1) * 2 * MB)
                lhs = jnp.concatenate([xbb[b, q, rows, :] for q in range(NKP)], axis=1)
                lhs = tie_lhs(lhs, dead.get(2 * u, []) + dead.get(2 * u + 1, []))
                r1 = _dot(lhs[:, :D // 2], _unpack(wb[base + cc, :D // 4, :]))
                r2 = r1 + _dot(lhs[:, D // 2:], _unpack(wb[base + cc, D // 4:, :]))
                bq[base + cc, pl.ds(row + (FRONT + mb * 2 * MB), 2 * MB), :] = r2
                for k, r in enumerate((r1, r2)):
                    ticks += _vregs(r)[::2]
                    if hook:
                        hook(2 * u + k, ticks, dead)
            return ticks

        def run_piece(q, wrow, row0):
            ticks = []
            for u in range(16):
                cc, mb = u % 8, u // 8
                r = _dot(xbb[0, q, pl.ds(row0 + mb * MB, MB), :], _unpack(wb[cc, pl.ds(wrow, KP // 2), :]))
                r = r + bq[cc, pl.ds(row0 + (FRONT + mb * MB), MB), :]
                bq[cc, pl.ds(row0 + (FRONT + mb * MB), MB), :] = r
                ticks += _vregs(r)
            return ticks

        def run_jobs(ticks, spare, jobs, free=0):
            ticks = ticks[:len(ticks) - 16 * spare]
            total = sum(n for n, _ in jobs)
            z = zero[...]
            cache = {}
            cnt = [0]

            def gate():
                k = (cnt[0] - free) * len(ticks) // (total - free)
                cnt[0] += 1
                if k < 0:
                    return z
                if k not in cache:
                    cache[k] = pltpu.bitcast(ticks[k], U32) & z
                return cache[k]

            for _, fn in jobs:
                fn(gate=gate)

        def interleave(*lists):
            items = []
            for l in lists:
                items += [((i + 0.5) / len(l), x) for i, x in enumerate(l)]
            items.sort(key=lambda z: z[0])
            return [x for _, x in items]

        def piece(q, carry):
            b0_copy(q + 1).wait()
            x0_copy(q + 1).wait()
            wrow = pl.multiple_of(q * (KP // 2), KP // 2)
            ticks = run_piece(q, wrow, 256)
            run_jobs(ticks, 4,
                     [(16, functools.partial(b_prep1, 0, 2 * wrow + KP, 0, cc)) for cc in range(8)]
                     + [(16, functools.partial(b_prep2, 0, wrow + KP // 2, 0, cc)) for cc in range(8)],
                     free=60)
            run_piece(q + 1, wrow + KP // 2, 0)
            return carry

        def ends(k, carry):
            run_piece(k * (NKP - 1), pl.multiple_of(k * ((NKP - 1) * KP // 2), 128),
                      pl.multiple_of(k * 256, 256))

            @pl.when(k == 0)
            def _():
                lax.fori_loop(0, NKP - 1, piece, 0)

            return carry

        def chunk(c, carry):
            @pl.when(c < 4)
            def _():
                xb_wait(c)

            @pl.when(c >= OW0)
            def _():
                w_wait(c - OW0)

            @pl.when((c & 3) == 3)
            def _():
                b_copy((c >> 2) + 1).wait()

            @pl.when(c >= OA0)
            def _():
                wob_copy(c - OA0).wait()

            p8 = (c >> 2) * 8
            ticks = run_chunk(c & 3, p8)
            pieces = []
            for k in range(NQ):
                g = jnp.maximum(NQ * (c - OW0), 0) + k
                src = pl.multiple_of(jnp.where(c >= OW0, g * 256, WROWS), 256)
                pieces.append((src, (g >> 2) * 8, pl.multiple_of((g & 3) * 128, 128)))
            ja = jnp.maximum(c - OA0, 0)
            nxt = (c + 1) >> 2
            run_jobs(ticks, 2, interleave(
                relayout_jobs(pieces),
                wob_jobs(jnp.where(c >= OA0, ja, 8), ja),
                [(16, functools.partial(f, j, row, e % 2, cc))
                 for e in range(4) for f, j, row in ((b_prep1, nxt, e * 256), (b_prep2, p8 + 8, e * 128))
                 for cc in range(8)]))
            return carry

        b0_copy(0).wait()
        for cc in range(8):
            b_prep1(0, 0, 0, cc)
        for cc in range(8):
            b_prep2(0, 0, 0, cc)
        x0_copy(0).wait()
        lax.fori_loop(0, 2, ends, 0)
        lax.fori_loop(1, NCH - 1, chunk, 0)

        wob_copy(7).wait()
        woa_copy.wait()
        lm = {}

        def first_attention(u, ticks, dead):
            for i in range(8):
                if u == 1 + 2 * i:
                    lm[i] = b_logits(0, i, make_gate(ticks[-32:], 64))
                    dead.setdefault(u + 4, []).append(lm[i][1])
                if u == 4 + 2 * i:
                    b_softmax(i, lm[i][0], lm[i][1], make_gate(ticks[-16:], 16))
                if u == 22 + 2 * i and i < 4:
                    b_values(0, i, make_gate(ticks[-32:], 64), 0)

        ticks = run_chunk(3, 16, first_attention)
        run_jobs(ticks, 2, interleave(
            wob_jobs(7, 7),
            [(32, functools.partial(woa_prep, j, q)) for j in range(8) for q in range(8)]))

    vm = pltpu.VMEM
    pl.run_scoped(
        phase1,
        vm((S // RB, NKP, RB, KP), BF),
        vm((WROWS + 256, 8, E), BF),
        vm((3, D, D), BF),
        vm((8, 512, D), BF),
        vm((32, D // 2, 128), U32),
        vm((9, D, 128), BF),
        vm((NTW, 80, 128), U32),
        vm((2, 33 * H + 40, 128), U32),
        vm((2, 33 * 8 + 32, 128), U32),
    )
    mem_copy.wait()
    xa_copy.wait()

    def phase2(qkv, acc, ola, olb, outa, outb):
        def out_copy(buf, row, c0, nc, half):
            return pltpu.make_async_copy(
                buf.at[pl.ds(row, BM), pl.ds(c0, nc)], out.at[pl.ds(row, BM), pl.ds(half * D + c0, nc)],
                sem_out.at[half])

        b_plan = {4: ('v', 0, 5), 9: ('v', 1, 5), 14: ('v', 2, 5), 19: ('v', 3, 5),
                  21: ('l', 4, 2), 23: ('l', 5, 2), 25: ('l', 6, 2), 27: ('l', 7, 2)}
        b_ticks = []

        def step(s, odd, slot_b):
            next_row = pl.multiple_of(jnp.minimum((s + 1) * SEG, S - BM), BM) if odd else None
            row = pl.multiple_of((s - odd) * SEG, BM)
            lhs = jnp.concatenate([memb[...], xaa[pl.ds(row + odd * 40, 24 if odd else 40), :]], axis=0)
            planes = (5, 7, 8, 9) if odd else (0, 1, 2, 3, 4, 6)
            plane0 = 5 * odd
            orows = (32, 48, 56, 64, 72) if odd else (0, 40, 8, 16, 24)
            nrow = 48 if odd else 32
            ticks = []
            tpd = len(planes)
            dead = {}
            lm = {}

            vgroups = (1,) if odd else (1, 2)

            def mxu_groups(p):
                vec = 2 * p >= VH_ODD if odd else 2 * p < VH_EVEN
                return [i for i in range(NG) if not (vec and i in vgroups)]

            def proj(h, t):
                r32 = _dot(tie_lhs(lhs, dead.get(3 * h + t)), _unpack(wa[t * H + h]))
                ticks.extend(_vregs(r32))
                r = r32.astype(BF)
                for i, pn in enumerate(planes):
                    qkv[t, pn, h * 8:h * 8 + 8, :] = r[8 * i:8 * i + 8]

            def o_store(h, i, o):
                ol, hi = (ola, h) if h < SPLIT else (olb, h - SPLIT)
                ol[orows[i]:orows[i] + 8, hi * E:(hi + 1) * E] = o

            probs = {}

            def pair(t, p, groups=range(NG)):
                return jnp.concatenate([qkv[t, plane0 + i, 16 * p:16 * p + 16, :] for i in groups], axis=0)

            def scores(p, n):
                groups = mxu_groups(p)
                y = nil(ticks[(6 * p + 6) * tpd - 1])
                k = jnp.concatenate([v | y for v in _vregs(pltpu.bitcast(pair(1, p), U32))], axis=0)
                sc = lax.dot_general(pair(0, p, groups), _unpack(k), (((1,), (1,)), ((), ())),
                                     preferred_element_type=F32)
                fl = jnp.concatenate([fill[16 * i:16 * i + 16, :] for i in groups], axis=0)
                sc = jnp.where(fl == 0.0, sc, fl)
                e = jnp.exp2((sc - jnp.max(sc, axis=1, keepdims=True)) * (a_scale * LOG2E))
                probs[p] = (e * _rcp(jnp.sum(e, axis=1, keepdims=True))).astype(BF)

            def values(p, n):
                o = _dot(probs.pop(p), pair(2, p)).astype(BF)
                for k, i in enumerate(mxu_groups(p)):
                    for hh in range(2):
                        o_store(2 * p + hh, i, o[16 * k + 8 * hh:16 * k + 8 * hh + 8])

            vstate = {}
            nkg = max(vgroups) + 1

            def group(t, h, i):
                return qkv[t, plane0 + i, h * 8:h * 8 + 8, :].astype(F32)

            def v_scores(h, tk):
                gate = make_gate(tk, nkg)
                sub = lax.broadcasted_iota(jnp.int32, (8, 1), 0)
                q = {i: group(0, h, i) * (a_scale * LOG2E) for i in vgroups}
                sc = {i: [] for i in vgroups}
                for kg in range(nkg):
                    k = gate(group(1, h, kg))
                    for j in range(8):
                        kj = jnp.broadcast_to(k[j:j + 1, :], (8, E))
                        for i in vgroups:
                            if kg <= i:
                                x = jnp.sum(kj * q[i], axis=1, keepdims=True)
                                if kg == i and j > 0:
                                    x = jnp.where(sub >= j, x, NEG * LOG2E)
                                sc[i].append(jnp.broadcast_to(x, (8, E)))
                m = {i: functools.reduce(jnp.maximum, sc[i]) for i in vgroups}
                vstate[h] = (sc, m)
                return list(m.values())

            def v_values(h, tk):
                gate = make_gate(tk, sum(i + 1 for i in vgroups))
                sc, m = vstate.pop(h)
                den = {}
                o = {}
                for kg in range(nkg):
                    v = group(2, h, kg)
                    mg = {i: gate(m[i]) for i in vgroups if kg <= i}
                    for j in range(8):
                        vj = jnp.broadcast_to(v[j:j + 1, :], (8, E))
                        for i in mg:
                            e = jnp.exp2(sc[i][8 * kg + j] - mg[i])
                            den[i] = den[i] + e if i in den else e
                            x = e * vj
                            o[i] = o[i] + x if i in o else x
                for i in vgroups:
                    o_store(h, i, (o[i] * _rcp(den[i])).astype(BF))

            def even_scores(h, n):
                dead.setdefault(n + 5, []).extend(v_scores(h, ticks[-3 * tpd:]))

            def even_values(h, n):
                v_values(h, ticks[-3 * tpd:])

            def late_b_values(i, n):
                b_values(row, i, make_gate(ticks[-2 * tpd:], 64), slot_b)

            def early_logits(_, n):
                gate = make_gate(b_ticks + ticks, 64 * 4)
                for i in range(4):
                    lm[i] = b_logits(next_row, i, gate)
                    dead.setdefault(7 + 2 * i, []).append(lm[i][1])

            def early_softmax(i, n):
                b_softmax(i, lm[i][0], lm[i][1], make_gate(ticks[-8:], 16))

            events = {}

            def at(n, f, a):
                events.setdefault(n, []).append(functools.partial(f, a, n))

            for p in range(H // 2):
                at(6 * p + 8, scores, p)
                at(6 * p + (16 if odd else 15), values, p)
            if odd:
                at(2, early_logits, 0)
                for i in range(4):
                    at(5 + 2 * i, early_softmax, i)
            else:
                for h in range(VH_EVEN):
                    at(3 * h + 5, even_scores, h)
                    at(3 * h + 10, even_values, h)
                for i in range(4):
                    at(1 + 2 * i, late_b_values, 4 + i)
            assert 6 * (SPLIT // 2 - 1) + 16 < 3 * H and 3 * (VH_EVEN - 1) + 10 < 3 * H - 1

            for h in range(H):
                for t in range(3):
                    proj(h, t)
                    for f in events.get(3 * h + t, []):
                        f()

            oticks = []
            odead = {}
            count = [0]

            def staged_dot(l, w, prev=None):
                n = count[0]
                count[0] += 1
                r = _dot(tie_lhs(l, odead.get(n)), _unpack(w))
                r = r if prev is None else prev + r
                oticks.extend(_vregs(r))
                if odd and b_plan.get(n - 6, 'v')[0] == 'l':
                    i = b_plan[n - 6][1]
                    b_softmax(i, lm[i][0], lm[i][1], make_gate(oticks[-6:], 16))
                if odd and n in b_plan:
                    stage, i, span = b_plan[n]
                    gate = make_gate(oticks[-6 * span:], 64)
                    if stage == 'l':
                        lm[i] = b_logits(next_row, i, gate)
                        odead.setdefault(n + 8, []).append(lm[i][1])
                    else:
                        b_values(next_row, i, gate, 1 - slot_b)
                return r

            if odd:
                for k in range(SPLIT // 8):
                    assert all(h >= 8 * (k + 1) for h in vstate) and VH_ODD + 8 * k >= 8 * (k + 1)
                    lk = ola[orows[0]:orows[0] + nrow, k * D:(k + 1) * D]
                    for j in range(8):
                        n = 8 * k + j
                        acc[j, 0:nrow, :] = staged_dot(lk, woa[j, k * D // 2:(k + 1) * D // 2, :],
                                                       acc[j, 0:nrow, :] if k else None)
                        if VH_ODD + n < H:
                            odead.setdefault(n + 5, []).extend(v_scores(VH_ODD + n, oticks[-6:]))
                        if VH_ODD <= VH_ODD + n - 5 < H:
                            v_values(VH_ODD + n - 5, oticks[-6:])
                        for f in events.get(3 * H + n, []):
                            f()
            else:
                l1 = ola[orows[0]:orows[0] + nrow, :]
                for j in range(8):
                    acc[j, 0:nrow, :] = staged_dot(l1, woa[j, :SPLIT * E // 2, :])
                    for n in range(3 * H + 2 * j, 3 * H + 2 * j + 2):
                        for f in events.get(n, []):
                            f()
            assert max(events) < 3 * H + 16 and not vstate and not probs
            l2 = olb[orows[0]:orows[0] + nrow, :]
            for j in range(8):
                res = staged_dot(l2, woa[j, SPLIT * E // 2:, :], acc[j, 0:nrow, :]).astype(BF)
                cols = slice(j * 128, (j + 1) * 128)
                memb[:, cols] = res[0:MEM]
                if odd:
                    outa[pl.ds(row, 8), cols] = res[8:16]
                    outa[pl.ds(row + SEG, SEG), cols] = res[16:]
                else:
                    outa[pl.ds(row + 8, 24), cols] = res[8:]
            if odd:
                out_copy(outa, row, 0, D, 0).start()

            o = ob[slot_b]
            del b_ticks[:]
            for j in range(4 * odd, 4 * odd + 4):
                r = staged_dot(o, wobp[j])
                b_ticks.extend(_vregs(r))
                outb[pl.ds(row, BM), j * 128:(j + 1) * 128] = r.astype(BF)
                if j % 2 == 1:
                    out_copy(outb, row, (j - 1) * 128, 256, 1).start()

        def steps(i, carry):
            for u in range(U):
                step(i * U + u, u % 2, (u // 2) % 2)
            return carry

        lax.fori_loop(0, NSEG // U, steps, 0)

        pltpu.make_async_copy(outb, out.at[:, pl.ds(D, D)], sem_out.at[1]).wait()
        pltpu.make_async_copy(outa, out.at[:, pl.ds(0, D)], sem_out.at[0]).wait()

    pl.run_scoped(
        phase2,
        vm((3, 2 * NG, H * 8, E), BF),
        vm((8, 48, 128), F32),
        vm((PAIR, SPLIT * E), BF),
        vm((PAIR, (H - SPLIT) * E), BF),
        vm((S, D), BF),
        vm((S, D), BF),
    )


@jax.jit
def _run(A_x, A_mem0, A_Wq, A_Wk, A_Wv, A_Wo, B_x, B_wqkv, B_wo):
    assert A_x.shape == (1, S, D) and A_mem0.shape == (1, MEM, D)
    assert A_Wq.shape == (D, H, E) and A_Wo.shape == (H, E, D)
    assert B_x.shape == (1, S, D) and B_wqkv.shape == (D, 3 * D) and B_wo.shape == (D, D)
    vm = pltpu.VMEM
    dma = pltpu.SemaphoreType.DMA
    scratch = [
        vm((S, D), BF),
        vm((MEM, D), BF),
        vm((3 * H, D // 2, E), U32),
        vm((8, H * E // 2, 128), U32),
        vm((8, D // 2, 128), U32),
        vm((24, S + FRONT, 128), F32),
        vm((PAIR, PAIR), F32),
        vm((WIN, BM, 128), F32),
        vm((2, BM, D), BF),
        vm((8, 128), U32),
        dma((NSEM,)), dma((2,)),
    ]
    out = pl.pallas_call(
        _kernel,
        out_shape=jax.ShapeDtypeStruct((S, 2 * D), BF),
        in_specs=[pl.BlockSpec(memory_space=pl.ANY)] * 9,
        out_specs=pl.BlockSpec(memory_space=pl.ANY),
        scratch_shapes=scratch,
        compiler_params=pltpu.CompilerParams(vmem_limit_bytes=120 * 1024 * 1024,
                                             disable_bounds_checks=True,
                                             disable_semaphore_checks=True),
    )(A_x.reshape(S, D), A_mem0.reshape(MEM, D), A_Wq, A_Wk, A_Wv, A_Wo.reshape(8, 512, D),
      B_x.reshape(S, D), B_wqkv, B_wo)
    return out.reshape(1, S, 2 * D)


def pallas_concat_heads__memory_aug_recurrent_mem_tr__sliding_local_dilated__prompt_kernel(
    A_x: jax.Array,
    A_mem0: jax.Array,
    A_Wq: jax.Array,
    A_Wk: jax.Array,
    A_Wv: jax.Array,
    A_Wo: jax.Array,
    A_seg_len,
    B_x: jax.Array,
    B_wqkv: jax.Array,
    B_wo: jax.Array,
):
    if isinstance(A_seg_len, int):
        assert A_seg_len == SEG
    return _run(A_x, A_mem0, A_Wq, A_Wk, A_Wv, A_Wo, B_x, B_wqkv, B_wo)
```

```python
import functools

import jax
import jax.numpy as jnp
from jax import lax
import jax.experimental.pallas as pl
import jax.experimental.pallas.tpu as pltpu

BF = jnp.bfloat16
F32 = jnp.float32
U32 = jnp.uint32

S = 2048
D = 1024
H = 32
E = 128
MEM = 8
SEG = 32
L = MEM + SEG
NG = L // 8
NSEG = S // SEG
WIN = 8
DIL = 2
NEG = -1000000000.0
LOG2E = 1.4426950408889634

PAIR = 2 * L
SPLIT = 24
U = 4
BM = 2 * SEG
FRONT = 32
VH_EVEN = 28
VH_ODD = 16

NCH = 12
RB = S // 4
MB = 128
NKP = 4
KP = D // NKP
NQ = 6
OW0 = 3
OA0 = NCH - 8
NTW = 4
WROWS = 3 * 4 * D

SEM_MEM, SEM_X, SEM_B0, SEM_XB, SEM_B, SEM_W, SEM_WOB, SEM_WOA, SEM_XA, NSEM = (
    0, 1, 5, 9, 13, 16, 26, 34, 35, 36)


def _rcp(d):
    r = pl.reciprocal(d, approx=True)
    return r * (2.0 - d * r)


def _dot(a, b):
    return jnp.dot(a, b, preferred_element_type=F32)


def _unpack(w):
    return pltpu.bitcast(w, BF)


def _lo_hi(a, b):
    lo = (a & U32(0xFFFF)) | (b << 16)
    hi = (a >> 16) | (b & U32(0xFFFF0000))
    return lo, hi


def _vregs(x):
    return [x[i:i + 8] for i in range(0, x.shape[0], 8)]


def _kernel(xa, mem0, wq, wk, wv, wo, xb, wqkv, wob, out,
            xaa, memb, wa, woa, wobp, bq, fill, pb, ob, zero, sem, sem_out):
    wsrc = (wq, wk, wv)
    a_scale = E ** -0.5
    b_scale = (D // H) ** -0.5

    xa_copy = pltpu.make_async_copy(xa, xaa, sem.at[SEM_XA])
    mem_copy = pltpu.make_async_copy(mem0, memb, sem.at[SEM_MEM])

    def nil(y):
        return pltpu.bitcast(y, U32) & zero[...]

    def tie_lhs(x, ys):
        if not ys:
            return x
        t = pltpu.bitcast(x[0:16, 0:128], U32)
        for y in ys:
            t = t | nil(y)
        top = jnp.concatenate([pltpu.bitcast(t, BF), x[0:16, 128:]], axis=1)
        return jnp.concatenate([top, x[16:]], axis=0)

    def make_gate(ticks, n):
        cnt = [0]
        cache = {}

        def gate(x):
            k = cnt[0] * len(ticks) // n
            cnt[0] += 1
            if k not in cache:
                cache[k] = nil(ticks[k])
            return pltpu.bitcast(pltpu.bitcast(x, U32) | cache[k], F32)
        return gate

    def b_logits(row, i, gate):
        q = [bq[cc, pl.ds(row + (FRONT + 8 * i), 8), :] for cc in range(8)]
        pos = row + 8 * i + lax.broadcasted_iota(jnp.int32, (8, 128), 0)
        logits = []
        for w in range(WIN):
            lo = FRONT + 8 * i - DIL * w
            t = None
            for cc in range(8):
                x = bq[8 + cc, pl.ds(row + lo, 8), :]
                x = (gate(x) if cc % 4 == 0 else x) * q[cc]
                t = x if t is None else t + x
            t = t + pltpu.roll(t, 64, 1)
            t = t + pltpu.roll(t, 32, 1)
            if 8 * i < DIL * w:
                t = jnp.where(pos >= DIL * w, t, NEG / b_scale)
            logits.append(t)
        return logits, functools.reduce(jnp.maximum, logits)

    def b_softmax(i, logits, m, gate):
        ex = [jnp.exp2((gate(t) - m) * (b_scale * LOG2E)) for t in logits]
        r = _rcp(functools.reduce(lambda a, b: a + b, ex))
        for w in range(WIN):
            pb[w, 8 * i:8 * i + 8, :] = gate(ex[w]) * r

    def b_values(row, i, gate, slot):
        p = [pb[w, 8 * i:8 * i + 8, :] for w in range(WIN)]
        for cc in range(8):
            t = None
            for w in range(WIN):
                lo = FRONT + 8 * i - DIL * w
                x = bq[16 + cc, pl.ds(row + lo, 8), :]
                x = (gate(x) if w % 4 == 0 else x) * p[w]
                t = x if t is None else t + x
            ob[slot, 8 * i:8 * i + 8, cc * 128:(cc + 1) * 128] = t.astype(BF)

    def phase1(xbb, wst, bst, woast, wb, wobst, tw, tb, tob):
        def st(i):
            return i if isinstance(i, int) else 0

        def w_copies(i):
            lo, hi = 256 * NQ * i, 256 * NQ * (i + 1)
            cps = []
            while lo < hi:
                c = lo // D
                n = min(hi, (c + 1) * D) - lo
                cps.append(pltpu.make_async_copy(
                    wsrc[c // 4].at[pl.ds(lo - c * D, n), pl.ds((c % 4) * 8, 8), :], wst.at[pl.ds(lo, n)],
                    sem.at[SEM_W + i]))
                lo += n
            return cps

        def w_wait(i):
            v = wst.at[pl.ds(pl.multiple_of(256 * NQ * i, 256), 256 * NQ)]
            pltpu.make_async_copy(v, v, sem.at[SEM_W + i]).wait()

        def b0_copy(q):
            lo = q * KP if isinstance(q, int) else pl.multiple_of(q * KP, KP)
            return pltpu.make_async_copy(
                wqkv.at[pl.ds(st(q) * KP, KP), pl.ds(0, D)], bst.at[0, pl.ds(lo, KP)], sem.at[SEM_B0 + q])

        def b_copy(p):
            return pltpu.make_async_copy(wqkv.at[:, pl.ds(st(p) * D, D)], bst.at[p], sem.at[SEM_B + p])

        def x0_copy(q):
            return pltpu.make_async_copy(
                xb.at[pl.ds(0, RB), pl.ds(st(q) * KP, KP)], xbb.at[0, q], sem.at[SEM_X + q])

        def xb_copies(b):
            return [pltpu.make_async_copy(
                xb.at[pl.ds(b * RB, RB), pl.ds(q * KP, KP)], xbb.at[b, q], sem.at[SEM_XB + b])
                for q in range(NKP)]

        def xb_wait(b):
            pltpu.make_async_copy(xbb.at[b], xbb.at[b], sem.at[SEM_XB + b]).wait()

        def wob_copy(j):
            return pltpu.make_async_copy(
                wob.at[:, pl.ds(st(j) * 128, 128)], wobst.at[j], sem.at[SEM_WOB + j])

        woa_copy = pltpu.make_async_copy(wo, woast, sem.at[SEM_WOA])

        for q in range(NKP):
            b0_copy(q).start()
            x0_copy(q).start()
        for c in range(1, NCH):
            if c < 4:
                for cp in xb_copies(c):
                    cp.start()
            if OW0 <= c < NCH - 1:
                for cp in w_copies(c - OW0):
                    cp.start()
            if c in (3, 7):
                b_copy(c // 4 + 1).start()
            if c >= OA0:
                wob_copy(c - OA0).start()
        woa_copy.start()
        mem_copy.start()
        xa_copy.start()

        def zero_fill(i, carry):
            r = pl.multiple_of(i * 16, 16)
            wst[pl.ds(WROWS + r, 16)] = jnp.zeros((16, 8, E), BF)
            wobst[8, pl.ds(4 * r, 64), :] = jnp.zeros((64, 128), BF)
            return carry

        lax.fori_loop(0, 16, zero_fill, 0)

        ri = lax.broadcasted_iota(jnp.int32, (PAIR, PAIR), 0)
        ci = lax.broadcasted_iota(jnp.int32, (PAIR, PAIR), 1)
        rb = (ri >> 3) & 1
        cb = (ci >> 3) & 1
        rl = ((ri >> 4) << 3) | (ri & 7)
        cl = ((ci >> 4) << 3) | (ci & 7)
        allowed = (rl < MEM) | (rl >= cl)
        fill[...] = jnp.where(rb == cb, jnp.where(allowed, 0.0, NEG / a_scale), -jnp.inf).astype(F32)
        bq[8:24, FRONT - 16:FRONT, :] = jnp.zeros((16, 16, 128), F32)
        zero[...] = jnp.zeros(zero.shape, U32)

        def zero_acc(i, carry):
            for u in range(32):
                row = FRONT + (u // 8) * MB + pl.multiple_of(i * 8, 8)
                bq[u % 8, pl.ds(row, 8), :] = jnp.zeros((8, E), F32)
            return carry

        lax.fori_loop(0, 16, zero_acc, 0)

        def gated(x, gate):
            return jnp.concatenate([v | gate() for v in _vregs(x)], axis=0) if gate else x

        def relayout1(src, blk, slot, gate):
            v = wst[pl.ds(src + blk * 16, 16)]
            v = pltpu.bitcast(v.reshape(128, 128), U32)
            for dp in range(8):
                tw[slot, 9 * dp:9 * dp + 8, :] = v[8 * dp:8 * dp + 8] | gate()

        def relayout2(base, row0, blk, slot, gate):
            row = row0 + blk * 8
            for j in range(4):
                g = gate()
                a = tw[slot, pl.ds(j, 8, stride=9), :] | g
                b = tw[slot, pl.ds(4 + j, 8, stride=9), :] | g
                lo, hi = _lo_hi(a, b)
                wa[base + 2 * j, pl.ds(row, 8), :] = lo
                wa[base + 2 * j + 1, pl.ds(row, 8), :] = hi

        def relayout_jobs(pieces):
            items = [(p, blk) for p in pieces for blk in range(16)]
            jobs = []
            for k in range(len(items) + 1):
                if k < len(items):
                    (src, _, _), blk = items[k]
                    jobs.append((8, functools.partial(relayout1, src, blk, k % NTW)))
                if k > 0:
                    (_, base, row0), blk = items[k - 1]
                    jobs.append((4, functools.partial(relayout2, base, row0, blk, (k - 1) % NTW)))
            return jobs

        def b_prep1(src, row, e, cc, gate=None):
            x = pltpu.bitcast(bst[src, pl.ds(row, 256), cc * 128:(cc + 1) * 128], U32)
            x = gated(x, gate).T
            for hl in range(4):
                h = 4 * cc + hl
                tb[e, 33 * h:33 * h + 32, :] = x[32 * hl:32 * hl + 32]

        def b_prep2(base, row, e, cc, gate=None):
            y = jnp.concatenate(
                [tb[e, pl.ds(4 * cc + dl + 33 * 8 * g, 8, stride=33), :] for dl in range(4) for g in range(4)],
                axis=0)
            wb[base + cc, pl.ds(row, 128), :] = gated(y, gate).T

        def wob_prep1(src, g, gate):
            v = pltpu.bitcast(wobst[src, g * 512:(g + 1) * 512, :], U32)
            v = gated(v, gate)
            for hp in range(8):
                tob[g, 33 * hp:33 * hp + 32, :] = v[32 * hp:32 * hp + 32]

        def wob_prep2(j, g, gate):
            for dp in range(16):
                z = gate()
                lo, hi = _lo_hi(tob[g, pl.ds(dp, 8, stride=33), :] | z,
                                tob[g, pl.ds(16 + dp, 8, stride=33), :] | z)
                wobp[j, (2 * dp) * 16 + 8 * g:(2 * dp) * 16 + 8 * g + 8, :] = lo
                wobp[j, (2 * dp + 1) * 16 + 8 * g:(2 * dp + 1) * 16 + 8 * g + 8, :] = hi

        def wob_jobs(src, j):
            return ([(32, functools.partial(wob_prep1, src, g)) for g in range(2)]
                    + [(16, functools.partial(wob_prep2, j, g)) for g in range(2)])

        def woa_prep(j, q, gate):
            v = pltpu.bitcast(woast[j, :, q * 128:(q + 1) * 128], U32)
            woa[q, j * 256:(j + 1) * 256, :] = gated(v, gate)

        def run_chunk(b, base, hook=None):
            ticks = []
            row = b * RB if isinstance(b, int) else pl.multiple_of(b * RB, RB)
            dead = {}
            for u in range(16):
                cc, mb = u % 8, u // 8
                rows = slice(mb * 2 * MB, (mb + 1) * 2 * MB)
                lhs = jnp.concatenate([xbb[b, q, rows, :] for q in range(NKP)], axis=1)
                lhs = tie_lhs(lhs, dead.get(2 * u, []) + dead.get(2 * u + 1, []))
                r1 = _dot(lhs[:, :D // 2], _unpack(wb[base + cc, :D // 4, :]))
                r2 = r1 + _dot(lhs[:, D // 2:], _unpack(wb[base + cc, D // 4:, :]))
                bq[base + cc, pl.ds(row + (FRONT + mb * 2 * MB), 2 * MB), :] = r2
                for k, r in enumerate((r1, r2)):
                    ticks += _vregs(r)[::2]
                    if hook:
                        hook(2 * u + k, ticks, dead)
            return ticks

        def run_piece(q, wrow, row0):
            ticks = []
            for u in range(16):
                cc, mb = u % 8, u // 8
                r = _dot(xbb[0, q, pl.ds(row0 + mb * MB, MB), :], _unpack(wb[cc, pl.ds(wrow, KP // 2), :]))
                r = r + bq[cc, pl.ds(row0 + (FRONT + mb * MB), MB), :]
                bq[cc, pl.ds(row0 + (FRONT + mb * MB), MB), :] = r
                ticks += _vregs(r)
            return ticks

        def run_jobs(ticks, spare, jobs, free=0):
            ticks = ticks[:len(ticks) - 16 * spare]
            total = sum(n for n, _ in jobs)
            z = zero[...]
            cache = {}
            cnt = [0]

            def gate():
                k = (cnt[0] - free) * len(ticks) // (total - free)
                cnt[0] += 1
                if k < 0:
                    return z
                if k not in cache:
                    cache[k] = pltpu.bitcast(ticks[k], U32) & z
                return cache[k]

            for _, fn in jobs:
                fn(gate=gate)

        def interleave(*lists):
            items = []
            for l in lists:
                items += [((i + 0.5) / len(l), x) for i, x in enumerate(l)]
            items.sort(key=lambda z: z[0])
            return [x for _, x in items]

        def piece(q, carry):
            b0_copy(q + 1).wait()
            x0_copy(q + 1).wait()
            wrow = pl.multiple_of(q * (KP // 2), KP // 2)
            ticks = run_piece(q, wrow, 256)
            run_jobs(ticks, 4,
                     [(16, functools.partial(b_prep1, 0, 2 * wrow + KP, 0, cc)) for cc in range(8)]
                     + [(16, functools.partial(b_prep2, 0, wrow + KP // 2, 0, cc)) for cc in range(8)],
                     free=60)
            run_piece(q + 1, wrow + KP // 2, 0)
            return carry

        def ends(k, carry):
            run_piece(k * (NKP - 1), pl.multiple_of(k * ((NKP - 1) * KP // 2), 128),
                      pl.multiple_of(k * 256, 256))

            @pl.when(k == 0)
            def _():
                lax.fori_loop(0, NKP - 1, piece, 0)

            return carry

        def chunk(c, carry):
            @pl.when(c < 4)
            def _():
                xb_wait(c)

            @pl.when(c >= OW0)
            def _():
                w_wait(c - OW0)

            @pl.when((c & 3) == 3)
            def _():
                b_copy((c >> 2) + 1).wait()

            @pl.when(c >= OA0)
            def _():
                wob_copy(c - OA0).wait()

            p8 = (c >> 2) * 8
            ticks = run_chunk(c & 3, p8)
            pieces = []
            for k in range(NQ):
                g = jnp.maximum(NQ * (c - OW0), 0) + k
                src = pl.multiple_of(jnp.where(c >= OW0, g * 256, WROWS), 256)
                pieces.append((src, (g >> 2) * 8, pl.multiple_of((g & 3) * 128, 128)))
            ja = jnp.maximum(c - OA0, 0)
            nxt = (c + 1) >> 2
            run_jobs(ticks, 2, interleave(
                relayout_jobs(pieces),
                wob_jobs(jnp.where(c >= OA0, ja, 8), ja),
                [(16, functools.partial(f, j, row, e % 2, cc))
                 for e in range(4) for f, j, row in ((b_prep1, nxt, e * 256), (b_prep2, p8 + 8, e * 128))
                 for cc in range(8)]))
            return carry

        b0_copy(0).wait()
        for cc in range(8):
            b_prep1(0, 0, 0, cc)
        for cc in range(8):
            b_prep2(0, 0, 0, cc)
        x0_copy(0).wait()
        lax.fori_loop(0, 2, ends, 0)
        lax.fori_loop(1, NCH - 1, chunk, 0)

        wob_copy(7).wait()
        woa_copy.wait()
        lm = {}

        def first_attention(u, ticks, dead):
            for i in range(8):
                if u == 1 + 2 * i:
                    lm[i] = b_logits(0, i, make_gate(ticks[-32:], 16))
                    dead.setdefault(u + 4, []).append(lm[i][1])
                if u == 4 + 2 * i:
                    b_softmax(i, lm[i][0], lm[i][1], make_gate(ticks[-16:], 16))
                if u == 22 + 2 * i and i < 4:
                    b_values(0, i, make_gate(ticks[-32:], 16), 0)

        ticks = run_chunk(3, 16, first_attention)
        run_jobs(ticks, 2, interleave(
            wob_jobs(7, 7),
            [(32, functools.partial(woa_prep, j, q)) for j in range(8) for q in range(8)]))

    vm = pltpu.VMEM
    pl.run_scoped(
        phase1,
        vm((S // RB, NKP, RB, KP), BF),
        vm((WROWS + 256, 8, E), BF),
        vm((3, D, D), BF),
        vm((8, 512, D), BF),
        vm((32, D // 2, 128), U32),
        vm((9, D, 128), BF),
        vm((NTW, 80, 128), U32),
        vm((2, 33 * H + 40, 128), U32),
        vm((2, 33 * 8 + 32, 128), U32),
    )
    mem_copy.wait()
    xa_copy.wait()

    def phase2(qkv, acc, ola, olb, outa, outb):
        def out_copy(buf, row, c0, nc, half):
            return pltpu.make_async_copy(
                buf.at[pl.ds(row, BM), pl.ds(c0, nc)], out.at[pl.ds(row, BM), pl.ds(half * D + c0, nc)],
                sem_out.at[half])

        b_plan = {4: ('v', 0, 5), 9: ('v', 1, 5), 14: ('v', 2, 5), 19: ('v', 3, 5),
                  21: ('l', 4, 2), 23: ('l', 5, 2), 25: ('l', 6, 2), 27: ('l', 7, 2)}
        b_ticks = []

        def step(s, odd, slot_b):
            next_row = pl.multiple_of(jnp.minimum((s + 1) * SEG, S - BM), BM) if odd else None
            row = pl.multiple_of((s - odd) * SEG, BM)
            lhs = jnp.concatenate([memb[...], xaa[pl.ds(row + odd * 40, 24 if odd else 40), :]], axis=0)
            planes = (5, 7, 8, 9) if odd else (0, 1, 2, 3, 4, 6)
            plane0 = 5 * odd
            orows = (32, 48, 56, 64, 72) if odd else (0, 40, 8, 16, 24)
            nrow = 48 if odd else 32
            ticks = []
            tpd = len(planes)
            dead = {}
            lm = {}

            vgroups = (1,) if odd else (1, 2)

            def mxu_groups(p):
                vec = 2 * p >= VH_ODD if odd else 2 * p < VH_EVEN
                return [i for i in range(NG) if not (vec and i in vgroups)]

            def proj(h, t):
                r32 = _dot(tie_lhs(lhs, dead.get(3 * h + t)), _unpack(wa[t * H + h]))
                ticks.extend(_vregs(r32))
                r = r32.astype(BF)
                for i, pn in enumerate(planes):
                    qkv[t, pn, h * 8:h * 8 + 8, :] = r[8 * i:8 * i + 8]

            def o_store(h, i, o):
                ol, hi = (ola, h) if h < SPLIT else (olb, h - SPLIT)
                ol[orows[i]:orows[i] + 8, hi * E:(hi + 1) * E] = o

            probs = {}

            def pair(t, p, groups=range(NG)):
                return jnp.concatenate([qkv[t, plane0 + i, 16 * p:16 * p + 16, :] for i in groups], axis=0)

            def scores(p, n):
                groups = mxu_groups(p)
                y = nil(ticks[(6 * p + 6) * tpd - 1])
                k = jnp.concatenate([v | y for v in _vregs(pltpu.bitcast(pair(1, p), U32))], axis=0)
                sc = lax.dot_general(pair(0, p, groups), _unpack(k), (((1,), (1,)), ((), ())),
                                     preferred_element_type=F32)
                fl = jnp.concatenate([fill[16 * i:16 * i + 16, :] for i in groups], axis=0)
                sc = jnp.where(fl == 0.0, sc, fl)
                e = jnp.exp2((sc - jnp.max(sc, axis=1, keepdims=True)) * (a_scale * LOG2E))
                probs[p] = (e * _rcp(jnp.sum(e, axis=1, keepdims=True))).astype(BF)

            def values(p, n):
                o = _dot(probs.pop(p), pair(2, p)).astype(BF)
                for k, i in enumerate(mxu_groups(p)):
                    for hh in range(2):
                        o_store(2 * p + hh, i, o[16 * k + 8 * hh:16 * k + 8 * hh + 8])

            vstate = {}
            nkg = max(vgroups) + 1

            def group(t, h, i):
                return qkv[t, plane0 + i, h * 8:h * 8 + 8, :].astype(F32)

            def v_scores(h, tk):
                gate = make_gate(tk, nkg)
                sub = lax.broadcasted_iota(jnp.int32, (8, 1), 0)
                q = {i: group(0, h, i) * (a_scale * LOG2E) for i in vgroups}
                sc = {i: [] for i in vgroups}
                for kg in range(nkg):
                    k = gate(group(1, h, kg))
                    for j in range(8):
                        kj = jnp.broadcast_to(k[j:j + 1, :], (8, E))
                        for i in vgroups:
                            if kg <= i:
                                x = jnp.sum(kj * q[i], axis=1, keepdims=True)
                                if kg == i and j > 0:
                                    x = jnp.where(sub >= j, x, NEG * LOG2E)
                                sc[i].append(jnp.broadcast_to(x, (8, E)))
                m = {i: functools.reduce(jnp.maximum, sc[i]) for i in vgroups}
                vstate[h] = (sc, m)
                return list(m.values())

            def v_values(h, tk):
                gate = make_gate(tk, sum(i + 1 for i in vgroups))
                sc, m = vstate.pop(h)
                den = {}
                o = {}
                for kg in range(nkg):
                    v = group(2, h, kg)
                    mg = {i: gate(m[i]) for i in vgroups if kg <= i}
                    for j in range(8):
                        vj = jnp.broadcast_to(v[j:j + 1, :], (8, E))
                        for i in mg:
                            e = jnp.exp2(sc[i][8 * kg + j] - mg[i])
                            den[i] = den[i] + e if i in den else e
                            x = e * vj
                            o[i] = o[i] + x if i in o else x
                for i in vgroups:
                    o_store(h, i, (o[i] * _rcp(den[i])).astype(BF))

            def even_scores(h, n):
                dead.setdefault(n + 5, []).extend(v_scores(h, ticks[-3 * tpd:]))

            def even_values(h, n):
                v_values(h, ticks[-3 * tpd:])

            def late_b_values(i, n):
                b_values(row, i, make_gate(ticks[-2 * tpd:], 16), slot_b)

            def early_logits(_, n):
                gate = make_gate(b_ticks + ticks, 16 * 4)
                for i in range(4):
                    lm[i] = b_logits(next_row, i, gate)
                    dead.setdefault(7 + 2 * i, []).append(lm[i][1])

            def early_softmax(i, n):
                b_softmax(i, lm[i][0], lm[i][1], make_gate(ticks[-8:], 16))

            events = {}

            def at(n, f, a):
                events.setdefault(n, []).append(functools.partial(f, a, n))

            for p in range(H // 2):
                at(6 * p + 8, scores, p)
                at(6 * p + (16 if odd else 15), values, p)
            if odd:
                at(2, early_logits, 0)
                for i in range(4):
                    at(5 + 2 * i, early_softmax, i)
            else:
                for h in range(VH_EVEN):
                    at(3 * h + 5, even_scores, h)
                    at(3 * h + 10, even_values, h)
                for i in range(4):
                    at(1 + 2 * i, late_b_values, 4 + i)
            assert 6 * (SPLIT // 2 - 1) + 16 < 3 * H and 3 * (VH_EVEN - 1) + 10 < 3 * H - 1

            for h in range(H):
                for t in range(3):
                    proj(h, t)
                    for f in events.get(3 * h + t, []):
                        f()

            oticks = []
            odead = {}
            count = [0]

            def staged_dot(l, w, prev=None):
                n = count[0]
                count[0] += 1
                r = _dot(tie_lhs(l, odead.get(n)), _unpack(w))
                r = r if prev is None else prev + r
                oticks.extend(_vregs(r))
                if odd and b_plan.get(n - 6, 'v')[0] == 'l':
                    i = b_plan[n - 6][1]
                    b_softmax(i, lm[i][0], lm[i][1], make_gate(oticks[-6:], 16))
                if odd and n in b_plan:
                    stage, i, span = b_plan[n]
                    gate = make_gate(oticks[-6 * span:], 16)
                    if stage == 'l':
                        lm[i] = b_logits(next_row, i, gate)
                        odead.setdefault(n + 8, []).append(lm[i][1])
                    else:
                        b_values(next_row, i, gate, 1 - slot_b)
                return r

            if odd:
                for k in range(SPLIT // 8):
                    assert all(h >= 8 * (k + 1) for h in vstate) and VH_ODD + 8 * k >= 8 * (k + 1)
                    lk = ola[orows[0]:orows[0] + nrow, k * D:(k + 1) * D]
                    for j in range(8):
                        n = 8 * k + j
                        acc[j, 0:nrow, :] = staged_dot(lk, woa[j, k * D // 2:(k + 1) * D // 2, :],
                                                       acc[j, 0:nrow, :] if k else None)
                        if VH_ODD + n < H:
                            odead.setdefault(n + 5, []).extend(v_scores(VH_ODD + n, oticks[-6:]))
                        if VH_ODD <= VH_ODD + n - 5 < H:
                            v_values(VH_ODD + n - 5, oticks[-6:])
                        for f in events.get(3 * H + n, []):
                            f()
            else:
                l1 = ola[orows[0]:orows[0] + nrow, :]
                for j in range(8):
                    acc[j, 0:nrow, :] = staged_dot(l1, woa[j, :SPLIT * E // 2, :])
                    for n in range(3 * H + 2 * j, 3 * H + 2 * j + 2):
                        for f in events.get(n, []):
                            f()
            assert max(events) < 3 * H + 16 and not vstate and not probs
            l2 = olb[orows[0]:orows[0] + nrow, :]
            for j in range(8):
                res = staged_dot(l2, woa[j, SPLIT * E // 2:, :], acc[j, 0:nrow, :]).astype(BF)
                cols = slice(j * 128, (j + 1) * 128)
                memb[:, cols] = res[0:MEM]
                if odd:
                    outa[pl.ds(row, 8), cols] = res[8:16]
                    outa[pl.ds(row + SEG, SEG), cols] = res[16:]
                else:
                    outa[pl.ds(row + 8, 24), cols] = res[8:]
            if odd:
                out_copy(outa, row, 0, D, 0).start()

            o = ob[slot_b]
            del b_ticks[:]
            for j in range(4 * odd, 4 * odd + 4):
                r = staged_dot(o, wobp[j])
                b_ticks.extend(_vregs(r))
                outb[pl.ds(row, BM), j * 128:(j + 1) * 128] = r.astype(BF)
                if j % 2 == 1:
                    out_copy(outb, row, (j - 1) * 128, 256, 1).start()

        def steps(i, carry):
            for u in range(U):
                step(i * U + u, u % 2, (u // 2) % 2)
            return carry

        lax.fori_loop(0, NSEG // U, steps, 0)

        pltpu.make_async_copy(outb, out.at[:, pl.ds(D, D)], sem_out.at[1]).wait()
        pltpu.make_async_copy(outa, out.at[:, pl.ds(0, D)], sem_out.at[0]).wait()

    pl.run_scoped(
        phase2,
        vm((3, 2 * NG, H * 8, E), BF),
        vm((8, 48, 128), F32),
        vm((PAIR, SPLIT * E), BF),
        vm((PAIR, (H - SPLIT) * E), BF),
        vm((S, D), BF),
        vm((S, D), BF),
    )


@jax.jit
def _run(A_x, A_mem0, A_Wq, A_Wk, A_Wv, A_Wo, B_x, B_wqkv, B_wo):
    assert A_x.shape == (1, S, D) and A_mem0.shape == (1, MEM, D)
    assert A_Wq.shape == (D, H, E) and A_Wo.shape == (H, E, D)
    assert B_x.shape == (1, S, D) and B_wqkv.shape == (D, 3 * D) and B_wo.shape == (D, D)
    vm = pltpu.VMEM
    dma = pltpu.SemaphoreType.DMA
    scratch = [
        vm((S, D), BF),
        vm((MEM, D), BF),
        vm((3 * H, D // 2, E), U32),
        vm((8, H * E // 2, 128), U32),
        vm((8, D // 2, 128), U32),
        vm((24, S + FRONT, 128), F32),
        vm((PAIR, PAIR), F32),
        vm((WIN, BM, 128), F32),
        vm((2, BM, D), BF),
        vm((8, 128), U32),
        dma((NSEM,)), dma((2,)),
    ]
    out = pl.pallas_call(
        _kernel,
        out_shape=jax.ShapeDtypeStruct((S, 2 * D), BF),
        in_specs=[pl.BlockSpec(memory_space=pl.ANY)] * 9,
        out_specs=pl.BlockSpec(memory_space=pl.ANY),
        scratch_shapes=scratch,
        compiler_params=pltpu.CompilerParams(vmem_limit_bytes=120 * 1024 * 1024,
                                             disable_bounds_checks=True,
                                             disable_semaphore_checks=True),
    )(A_x.reshape(S, D), A_mem0.reshape(MEM, D), A_Wq, A_Wk, A_Wv, A_Wo.reshape(8, 512, D),
      B_x.reshape(S, D), B_wqkv, B_wo)
    return out.reshape(1, S, 2 * D)


def pallas_concat_heads__memory_aug_recurrent_mem_tr__sliding_local_dilated__prompt_kernel(
    A_x: jax.Array,
    A_mem0: jax.Array,
    A_Wq: jax.Array,
    A_Wk: jax.Array,
    A_Wv: jax.Array,
    A_Wo: jax.Array,
    A_seg_len,
    B_x: jax.Array,
    B_wqkv: jax.Array,
    B_wo: jax.Array,
):
    if isinstance(A_seg_len, int):
        assert A_seg_len == SEG
    return _run(A_x, A_mem0, A_Wq, A_Wk, A_Wv, A_Wo, B_x, B_wqkv, B_wo)
```
